```python
import jax
import jax.numpy as jnp

def _softmax(x, axis=-1):
    return jax.nn.softmax(x, axis=axis)
def _gelu(x):
    return jax.nn.gelu(x, approximate=True)
def _silu(x):
    return jax.nn.silu(x)
def _sigmoid(x):
    return jax.nn.sigmoid(x)
def _layernorm(x, axis=-1, eps=1e-5):
    m = jnp.mean(x, axis=axis, keepdims=True)
    v = jnp.var(x, axis=axis, keepdims=True)
    return (x - m) / jnp.sqrt(v + eps)
def _scatter_add(tgt, idx, src, axis=0):
    return tgt.at[idx].add(src)
def _segment_sum(src, seg, n):
    return jax.ops.segment_sum(src, seg, n)
class _Rng:
    def __init__(self, key):
        self._k = key
    def _next(self):
        self._k, sub = jax.random.split(self._k)
        return sub
    def normal(self, shape):
        return jax.random.normal(self._next(), shape, dtype=jnp.bfloat16)
    def randint(self, lo, hi, shape):
        return jax.random.randint(self._next(), shape, lo, hi, dtype=jnp.int32)
    def uniform(self, shape, lo=0.0, hi=1.0):
        return jax.random.uniform(self._next(), shape, jnp.bfloat16, lo, hi)
    def permutation(self, n):
        return jax.random.permutation(self._next(), n)


kernel_name = 'sequential_preLN__spectral_gfnet__swiglu_ffn__prompt'

def _fwd_setup_inputs():
    _rng = _Rng(jax.random.key(int.from_bytes(__import__("os").urandom(4), "little")))
    _w = (lambda a: (lambda t: t.astype(jnp.bfloat16) if jnp.issubdtype(t.dtype, jnp.floating) else t)(jnp.asarray(a)))
    def _A_setup():
        B, S, D = 1, 2048, 576
        Df = D // 2 + 1
        return {
            "x": _w((lambda *s: _rng.normal(s) * 0.05)(B, S, D)),
            "w_r": _w((lambda *s: _rng.normal(s) * 0.05)(S, Df) * 0.02),
            "w_i": _w((lambda *s: _rng.normal(s) * 0.05)(S, Df) * 0.02),
        }
    _A_in = _A_setup()

    def _B_setup():
        B, S, D, F = 1, 2048, 576, 4608
        return {
            "x": _w((lambda *s: _rng.normal(s) * 0.05)(B, S, D)),
            "w_gate": _w((lambda *s: _rng.normal(s) * 0.05)(D, F)),
            "w_up": _w((lambda *s: _rng.normal(s) * 0.05)(D, F)),
            "w_down": _w((lambda *s: _rng.normal(s) * 0.05)(F, D)),
        }
    _B_in = _B_setup()

    return {
        "A_x": _A_in["x"],
        "A_w_r": _A_in["w_r"],
        "A_w_i": _A_in["w_i"],
        "B_x": _B_in["x"],
        "B_w_gate": _B_in["w_gate"],
        "B_w_up": _B_in["w_up"],
        "B_w_down": _B_in["w_down"],
    }

def _fwd_reference(A_x, A_w_r, A_w_i, B_x, B_w_gate, B_w_up, B_w_down):
    def _A_ref(x, w_r, w_i):
        B, S, D = x.shape
        X = (lambda x, axes=(-2,-1): jnp.fft.rfft2(x.astype(jnp.float32), axes=axes))(x, axes=(-2, -1))
        W = w_r + 1j * w_i
        X = X * W
        y = (lambda x, s, axes=(-2,-1): jnp.fft.irfft2(x, s=s, axes=axes).astype(jnp.bfloat16))(X, (S, D), axes=(-2, -1))
        return y

    def _B_ref(x, w_gate, w_up, w_down):
        g = _silu(x @ w_gate)
        u = x @ w_up
        return (g * u) @ w_down

    x = A_x
    h = x + _A_ref(_layernorm(x, axis=-1), A_w_r, A_w_i)
    h2 = h + _B_ref(_layernorm(h, axis=-1), B_w_gate, B_w_up, B_w_down)
    return h2


def setup_inputs():
    _inp = _fwd_setup_inputs()
    _gk = jax.random.fold_in(jax.random.key(int.from_bytes(__import__("os").urandom(4), "little")), 2**31 - 1)
    _shapes = [[1, 2048, 576]]
    _dtypes = ['bfloat16']
    _gks = jax.random.split(_gk, len(_shapes))
    _gs = [jax.random.normal(k, s, dtype=jnp.dtype(d)) * 0.05 for k, s, d in zip(_gks, _shapes, _dtypes)]
    _inp["grad_out"] = _gs[0]
    return _inp

def reference(A_x, A_w_r, A_w_i, B_w_gate, B_w_up, B_w_down, B_x, grad_out):
    _const = dict(B_x=B_x)
    def _f(*_d):
        return _fwd_reference(**{'A_x': _d[0], 'A_w_r': _d[1], 'A_w_i': _d[2], 'B_w_gate': _d[3], 'B_w_up': _d[4], 'B_w_down': _d[5], **_const})
    _out, _vjp = jax.vjp(_f, A_x, A_w_r, A_w_i, B_w_gate, B_w_up, B_w_down)
    _grads = _vjp(grad_out)
    _out0 = jnp.asarray(_out)
    return (_out0, *[jnp.asarray(_g) for _g in _grads])
```

```python
import functools
import math

import jax
import jax.numpy as jnp
import ml_dtypes
import numpy as np
from jax import lax
from jax.experimental import pallas as pl
from jax.experimental.pallas import tpu as pltpu

S, D, F = 2048, 576, 4608
KF = D // 2 + 1
KP = 384
R1, R2 = 16, 128
EPS = 1e-5
ST = 512
FT = 512
RC = 256

bf16 = jnp.bfloat16
f32 = jnp.float32
NN = (((1,), (0,)), ((), ()))
NT = (((1,), (1,)), ((), ()))


def _consts():
    d = np.arange(D)[:, None]
    k = np.arange(KF)[None, :]
    ang = 2.0 * np.pi * ((d * k) % D) / D
    fd = np.zeros((D, 2 * KP), np.float64)
    fd[:, :KF] = np.cos(ang)
    fd[:, KP:KP + KF] = -np.sin(ang)
    k1 = np.arange(R1)[:, None, None]
    k2 = np.arange(R2)[None, :, None]
    n2 = np.arange(R2)[None, None, :]
    ang = 2.0 * np.pi * ((n2 * (k1 + R1 * k2)) % S) / S
    gr, gi = np.cos(ang), -np.sin(ang)
    g = np.concatenate([np.concatenate([gr, -gi], 2), np.concatenate([gi, gr], 2)], 1)
    gh = np.ascontiguousarray(g.transpose(0, 2, 1))
    c = np.zeros((1, KP), np.float32)
    c[0, :KF] = 2.0 / (S * D)
    c[0, 0] = c[0, KF - 1] = 1.0 / (S * D)
    cast = lambda a: a.astype(np.float32).astype(ml_dtypes.bfloat16)
    return cast(fd), cast(g), cast(gh), c


_FD, _G, _GH, _C = _consts()


def _dot(a, b, dn=NN):
    return lax.dot_general(a, b, dn, preferred_element_type=f32)


def _fft4(x, sign):
    (ar, ai), (br, bi), (cr, ci), (dr, di) = x
    s0r, s0i, d0r, d0i = ar + cr, ai + ci, ar - cr, ai - ci
    s1r, s1i, d1r, d1i = br + dr, bi + di, br - dr, bi - di
    lo = (d0r + d1i, d0i - d1r)
    hi = (d0r - d1i, d0i + d1r)
    o1, o3 = (lo, hi) if sign < 0 else (hi, lo)
    return [(s0r + s1r, s0i + s1i), o1, (s0r - s1r, s0i - s1i), o3]


def _tw16(v, e, sign):
    r, i = v
    e %= 16
    if e == 0:
        return v
    if e == 4:
        return (i, -r) if sign < 0 else (-i, r)
    c = math.cos(2 * math.pi * e / 16)
    s = sign * math.sin(2 * math.pi * e / 16)
    if e % 2 == 0:
        if c * s > 0:
            return ((r - i) * c, (r + i) * c)
        return ((r + i) * c, (i - r) * c)
    return (r * c - i * s, r * s + i * c)


def _fft16(x, sign):
    cols = [_fft4([x[4 * a + b] for a in range(4)], sign) for b in range(4)]
    out = [None] * 16
    for p in range(4):
        o = _fft4([_tw16(cols[b][p], b * p, sign) for b in range(4)], sign)
        for q in range(4):
            out[p + 4 * q] = o[q]
    return out


def _ln(x):
    xc = x - jnp.mean(x, axis=-1, keepdims=True)
    rstd = 1.0 / jnp.sqrt(jnp.mean(xc * xc, axis=-1, keepdims=True) + EPS)
    return xc * rstd, rstd


def _ln_bwd(dn, n, rstd):
    return rstd * (dn - jnp.mean(dn, axis=-1, keepdims=True)
                   - n * jnp.mean(dn * n, axis=-1, keepdims=True))


def _kernel(x_h, wr_h, wi_h, wg_h, wu_h, wd_h, g_h, fd_h, gm_h, gh_h, c_h,
            out_h, dx_h, dwr_h, dwi_h, dwg_h, dwu_h, dwd_h,
            x_v, g_v, wb_v, wg_v, wu_v, wd_v, fd_v, gm_v, gh_v, c_v,
            wp_v, z_v, t_v, xs_v, zb_v, h_v, hn_v, hnt_v, gt_v,
            wdt_v, p_v, da_v, du_v, acco_v, acch_v, dwg_v, dwu_v, dwd_v, ob_v,
            sin, sout):
    nrc = S // RC
    nj = F // FT

    def rows(i, n):
        return pl.ds(pl.multiple_of(i * n, n), n)

    def cp(src, dst, sem):
        return pltpu.make_async_copy(src, dst, sem)

    x_cp = lambda i: cp(x_h.at[0, rows(i, RC)], x_v.at[rows(i, RC)], sin.at[i])
    fd_cp = cp(fd_h, fd_v, sin.at[nrc])
    early = [cp(gm_h, gm_v, sin.at[nrc + 1]), cp(gh_h, gh_v, sin.at[nrc + 2]),
             cp(c_h, c_v, sin.at[nrc + 3])]
    w_cp = [cp(wr_h, wb_v.at[0], sin.at[nrc + 4]), cp(wi_h, wb_v.at[1], sin.at[nrc + 5])]
    g_cp = cp(g_h.at[0], g_v, sin.at[nrc + 6])
    ffn_cp = [cp(wg_h, wg_v, sin.at[nrc + 7]), cp(wu_h, wu_v, sin.at[nrc + 8]),
              cp(wd_h, wd_v, sin.at[nrc + 9])]

    x_cp(0).start()
    fd_cp.start()
    for i in range(1, nrc):
        x_cp(i).start()
    for c in w_cp + early + [g_cp] + ffn_cp:
        c.start()

    def radix_fwd():
        def body(it, carry):
            r = it // 3
            lre = pl.ds(pl.multiple_of((it % 3) * 128, 128), 128)
            lim = pl.ds(pl.multiple_of((it % 3) * 128 + KP, 128), 128)
            xs = [(z_v[n, rows(r, 8), lre], z_v[n, rows(r, 8), lim]) for n in range(R1)]
            for k, (a, b) in enumerate(_fft16(xs, -1)):
                t_v[k, 0, rows(r, 8), lre] = a
                t_v[k, 1, rows(r, 8), lre] = b
            return carry
        lax.fori_loop(0, 3 * R2 // 8, body, 0)

    def radix_inv():
        def body(it, carry):
            r = it // 3
            lre = pl.ds(pl.multiple_of((it % 3) * 128, 128), 128)
            lim = pl.ds(pl.multiple_of((it % 3) * 128 + KP, 128), 128)
            xs = [(t_v[n, 0, rows(r, 8), lre], t_v[n, 1, rows(r, 8), lre]) for n in range(R1)]
            for k, (a, b) in enumerate(_fft16(xs, 1)):
                z_v[k, rows(r, 8), lre] = a
                z_v[k, rows(r, 8), lim] = b
            return carry
        lax.fori_loop(0, 3 * R2 // 8, body, 0)

    def z_rows(i):
        nb = RC // R2
        return z_v[pl.ds(i * nb, nb)].reshape(RC, 2 * KP)

    def set_z_rows(i, val):
        nb = RC // R2
        z_v[pl.ds(i * nb, nb)] = val.reshape(nb, R2, 2 * KP)

    def filt(k1):
        sl = pl.ds(k1, R2, stride=R1)
        wr = jnp.concatenate([wp_v[0, c, sl, :] for c in range(3)], axis=1)
        wi = jnp.concatenate([wp_v[1, c, sl, :] for c in range(3)], axis=1)
        return wr, wi

    fd_cp.wait()

    def p1(i, carry):
        x_cp(i).wait()
        xn, _ = _ln(x_v[rows(i, RC), :].astype(f32))
        set_z_rows(i, _dot(xn.astype(bf16), fd_v[...]))
        return carry
    lax.fori_loop(0, nrc, p1, 0)

    radix_fwd()

    for c in w_cp + early:
        c.wait()

    def pw(i, carry):
        r = rows(i, RC)
        for a in range(2):
            for c in range(2):
                wp_v[a, c, r, :] = (wb_v[a, r, c * 128:(c + 1) * 128].astype(f32)
                                    * c_v[:, c * 128:(c + 1) * 128])
            wp_v[a, 2, r, :] = jnp.zeros((RC, 128), f32)
            wp_v[a, 2, r, 0:KF - 256] = wb_v[a, r, 256:KF].astype(f32) * c_v[:, 256:KF]
        return carry
    lax.fori_loop(0, nrc, pw, 0)

    def p3(k1, carry):
        xx = _dot(gm_v[k1], t_v[k1].reshape(2 * R2, KP).astype(bf16))
        xs_v[k1] = xx
        xr, xi = xx[:R2], xx[R2:]
        wr, wi = filt(k1)
        yy = jnp.concatenate([xr * wr - xi * wi, xr * wi + xi * wr], axis=0)
        t_v[k1] = _dot(gh_v[k1], yy.astype(bf16)).reshape(2, R2, KP)
        return carry
    lax.fori_loop(0, R1, p3, 0)

    radix_inv()

    g_cp.wait()

    def p5(i, carry):
        r = rows(i, RC)
        h = x_v[r, :].astype(f32) + _dot(z_rows(i).astype(bf16), fd_v[...], NT)
        h_v[r, :] = h
        hn, _ = _ln(h)
        hn_v[r, :] = hn.astype(bf16)
        hnt_v[:, r] = hn.T.astype(bf16)
        gt_v[:, r] = g_v[r, :].astype(f32).T.astype(bf16)
        acco_v[:, r] = jnp.zeros((D, RC), f32)
        acch_v[:, r] = jnp.zeros((D, RC), f32)
        return carry
    lax.fori_loop(0, nrc, p5, 0)

    for c in ffn_cp:
        c.wait()

    def dw_cp(j):
        fs = rows(j, FT)
        return [cp(dwg_v.at[:, fs], dwg_h.at[:, fs], sout.at[3 * j]),
                cp(dwu_v.at[:, fs], dwu_h.at[:, fs], sout.at[3 * j + 1]),
                cp(dwd_v.at[fs], dwd_h.at[fs], sout.at[3 * j + 2])]

    def jbody(j, carry):
        fs = rows(j, FT)
        wdt_v[...] = wd_v[fs, :].astype(f32).T.astype(bf16)

        def ibody(i, carry):
            ss = rows(i, ST)
            hn = hn_v[ss, :]
            a = _dot(hn, wg_v[:, fs])
            u = _dot(hn, wu_v[:, fs])
            dp = _dot(g_v[ss, :], wdt_v[...])
            sg = jax.nn.sigmoid(a)
            sl = a * sg
            p = (sl * u).astype(bf16)
            du = (dp * sl).astype(bf16)
            da = (dp * u * (sg + sl * (1.0 - sg))).astype(bf16)
            p_v[ss, :] = p
            da_v[ss, :] = da
            du_v[ss, :] = du
            acco_v[:, ss] += _dot(wdt_v[...], p, NT)
            acch_v[:, ss] += _dot(wg_v[:, fs], da, NT) + _dot(wu_v[:, fs], du, NT)
            return carry
        lax.fori_loop(0, S // ST, ibody, 0)
        dwg_v[:, fs] = _dot(hnt_v[...], da_v[...]).astype(bf16)
        dwu_v[:, fs] = _dot(hnt_v[...], du_v[...]).astype(bf16)
        dwd_v[fs, :] = _dot(gt_v[...], p_v[...]).T.astype(bf16)
        for c in dw_cp(j):
            c.start()
        return carry
    lax.fori_loop(0, nj, jbody, 0)

    o_cp = cp(ob_v, out_h.at[0], sout.at[3 * nj])

    def p7(i, carry):
        r = rows(i, RC)
        h = h_v[r, :]
        ob_v[r, :] = (h + acco_v[:, r].T).astype(bf16)
        hn, rstd = _ln(h)
        dh = g_v[r, :].astype(f32) + _ln_bwd(acch_v[:, r].T, hn, rstd)
        h_v[r, :] = dh
        set_z_rows(i, _dot(dh.astype(bf16), fd_v[...]))
        return carry
    lax.fori_loop(0, nrc, p7, 0)
    o_cp.start()

    radix_fwd()

    def p9(k1, carry):
        dy = _dot(gm_v[k1], t_v[k1].reshape(2 * R2, KP).astype(bf16))
        dr, di = dy[:R2], dy[R2:]
        wr, wi = filt(k1)
        dxx = jnp.concatenate([dr * wr + di * wi, di * wr - dr * wi], axis=0)
        t_v[k1] = _dot(gh_v[k1], dxx.astype(bf16)).reshape(2, R2, KP)
        xr, xi = xs_v[k1, :R2], xs_v[k1, R2:]
        cc = c_v[...]
        gr = (dr * xr + di * xi) * cc
        gi = (di * xr - dr * xi) * cc
        sl = pl.ds(k1, R2, stride=R1)
        for c in range(3):
            wp_v[0, c, sl, :] = gr[:, c * 128:(c + 1) * 128]
            wp_v[1, c, sl, :] = gi[:, c * 128:(c + 1) * 128]
        return carry
    lax.fori_loop(0, R1, p9, 0)

    def pdw(i, carry):
        r = rows(i, RC)
        for a in range(2):
            for c in range(2):
                wb_v[a, r, c * 128:(c + 1) * 128] = wp_v[a, c, r, :].astype(bf16)
            wb_v[a, r, 256:KF] = wp_v[a, 2, r, 0:KF - 256].astype(bf16)
        return carry
    lax.fori_loop(0, nrc, pdw, 0)
    dw_out = [cp(wb_v.at[0], dwr_h, sout.at[3 * nj + 1]),
              cp(wb_v.at[1], dwi_h, sout.at[3 * nj + 2])]
    for c in dw_out:
        c.start()

    radix_inv()

    dx_cp = lambda i: cp(hn_v.at[rows(i, RC)], dx_h.at[0, rows(i, RC)],
                         sout.at[3 * nj + 3 + i])

    def p11(i, carry):
        r = rows(i, RC)
        dxn = _dot(z_rows(i).astype(bf16), fd_v[...], NT)
        xn, rstd = _ln(x_v[r, :].astype(f32))
        hn_v[r, :] = (h_v[r, :] + _ln_bwd(dxn, xn, rstd)).astype(bf16)
        dx_cp(i).start()
        return carry
    lax.fori_loop(0, nrc, p11, 0)

    for j in range(nj):
        for c in dw_cp(j):
            c.wait()
    o_cp.wait()
    for c in dw_out:
        c.wait()
    for i in range(nrc):
        dx_cp(i).wait()


@jax.jit
def pallas_sequential_preLN__spectral_gfnet__swiglu_ffn__prompt_kernel(
    A_x: jax.Array,
    A_w_r: jax.Array,
    A_w_i: jax.Array,
    B_x: jax.Array,
    B_w_gate: jax.Array,
    B_w_up: jax.Array,
    B_w_down: jax.Array,
    grad_out: jax.Array,
):
    del B_x
    V = pltpu.VMEM
    sds = jax.ShapeDtypeStruct
    any_spec = pl.BlockSpec(memory_space=pl.ANY)
    return tuple(pl.pallas_call(
        _kernel,
        out_shape=[sds((1, S, D), bf16), sds((1, S, D), bf16),
                   sds((S, KF), bf16), sds((S, KF), bf16),
                   sds((D, F), bf16), sds((D, F), bf16), sds((F, D), bf16)],
        in_specs=[any_spec] * 11,
        out_specs=[any_spec] * 7,
        scratch_shapes=[
            V((S, D), bf16), V((S, D), bf16), V((2, S, KF), bf16),
            V((D, F), bf16), V((D, F), bf16), V((F, D), bf16),
            V((D, 2 * KP), bf16), V((R1, 2 * R2, 2 * R2), bf16), V((R1, 2 * R2, 2 * R2), bf16),
            V((1, KP), f32),
            V((2, 3, S, 128), f32), V((R1, R2, 2 * KP), f32), V((R1, 2, R2, KP), f32),
            V((R1, 2 * R2, KP), f32), V((8, 128), f32),
            V((S, D), f32), V((S, D), bf16), V((D, S), bf16), V((D, S), bf16),
            V((D, FT), bf16), V((S, FT), bf16), V((S, FT), bf16), V((S, FT), bf16),
            V((D, S), f32), V((D, S), f32),
            V((D, F), bf16), V((D, F), bf16), V((F, D), bf16), V((S, D), bf16),
            pltpu.SemaphoreType.DMA((S // RC + 10,)),
            pltpu.SemaphoreType.DMA((3 * (F // FT) + 3 + S // RC,)),
        ],
        compiler_params=pltpu.CompilerParams(vmem_limit_bytes=124 * 2**20),
    )(A_x, A_w_r, A_w_i, B_w_gate, B_w_up, B_w_down, grad_out, _FD, _G, _GH, _C))
```

```python
import math

import jax
import jax.numpy as jnp
import ml_dtypes
import numpy as np
from jax import lax
from jax.experimental import pallas as pl
from jax.experimental.pallas import tpu as pltpu

S, D, F = 2048, 576, 4608
KF = D // 2 + 1
KP = 304
R1, R2 = 16, 128
EPS = 1e-5
ST = 512
FT = 512
TC = 256

bf16 = jnp.bfloat16
f32 = jnp.float32
NN = (((1,), (0,)), ((), ()))
NT = (((1,), (1,)), ((), ()))


def _consts():
    d = np.arange(D)[:, None]
    k = np.arange(KF)[None, :]
    ang = 2.0 * np.pi * ((d * k) % D) / D
    fd = np.zeros((D, 2 * KP), np.float64)
    fd[:, :KF] = np.cos(ang)
    fd[:, KP:KP + KF] = -np.sin(ang)
    k1 = np.arange(R1)[:, None, None]
    n2 = np.arange(R2)[None, :, None]
    lane = np.arange(R2)[None, None, :]
    k2 = 8 * (lane % 16) + lane // 16
    ang = 2.0 * np.pi * ((n2 * (k1 + R1 * k2)) % S) / S
    gr, gi = np.cos(ang), -np.sin(ang)
    g = np.concatenate([np.concatenate([gr, gi], 2), np.concatenate([-gi, gr], 2)], 1)
    cast = lambda a: np.ascontiguousarray(a).astype(np.float32).astype(ml_dtypes.bfloat16)
    return cast(fd), cast(fd.T), cast(g)


_FD, _FDT, _G = _consts()


def _dot(a, b, dn=NN):
    return lax.dot_general(a, b, dn, preferred_element_type=f32)


def _fft4(x, sign):
    (ar, ai), (br, bi), (cr, ci), (dr, di) = x
    s0r, s0i, d0r, d0i = ar + cr, ai + ci, ar - cr, ai - ci
    s1r, s1i, d1r, d1i = br + dr, bi + di, br - dr, bi - di
    lo = (d0r + d1i, d0i - d1r)
    hi = (d0r - d1i, d0i + d1r)
    o1, o3 = (lo, hi) if sign < 0 else (hi, lo)
    return [(s0r + s1r, s0i + s1i), o1, (s0r - s1r, s0i - s1i), o3]


def _tw16(v, e, sign):
    r, i = v
    e %= 16
    if e == 0:
        return v
    if e == 4:
        return (i, -r) if sign < 0 else (-i, r)
    c = math.cos(2 * math.pi * e / 16)
    s = sign * math.sin(2 * math.pi * e / 16)
    if e % 2 == 0:
        if c * s > 0:
            return ((r - i) * c, (r + i) * c)
        return ((r + i) * c, (i - r) * c)
    return (r * c - i * s, r * s + i * c)


def _fft16(x, sign):
    cols = [_fft4([x[4 * a + b] for a in range(4)], sign) for b in range(4)]
    out = [None] * 16
    for p in range(4):
        o = _fft4([_tw16(cols[b][p], b * p, sign) for b in range(4)], sign)
        for q in range(4):
            out[p + 4 * q] = o[q]
    return out


def _shuffle16(tiles):
    lane = lax.broadcasted_iota(jnp.int32, tiles[0].shape, 1)
    tiles = list(tiles)
    for d in (8, 4, 2, 1):
        low = (lane & d) == 0
        for t in range(R1):
            if t & d:
                continue
            a, b = tiles[t], tiles[t + d]
            tiles[t] = jnp.where(low, a, pltpu.roll(b, d, 1))
            tiles[t + d] = jnp.where(low, pltpu.roll(a, R2 - d, 1), b)
    return tiles


def _ln(x):
    xc = x - jnp.mean(x, axis=0, keepdims=True)
    rstd = 1.0 / jnp.sqrt(jnp.mean(xc * xc, axis=0, keepdims=True) + EPS)
    return xc * rstd, rstd


def _ln_bwd(dn, n, rstd):
    return rstd * (dn - jnp.mean(dn, axis=0, keepdims=True)
                   - n * jnp.mean(dn * n, axis=0, keepdims=True))


def _kernel(x_h, wr_h, wi_h, wg_h, wu_h, wd_h, g_h, fd_h, fdt_h, gm_h,
            out_h, dx_h, dwr_h, dwi_h, dwg_h, dwu_h, dwd_h,
            x_v, gt_v, wb_v, wg_v, wu_v, wd_v, fd_v, fdt_v, gm_v,
            wp_v, z_v, t_v, xs_v, h_v, hn_v, hnt_v, g_v,
            p_v, da_v, du_v, acco_v, acch_v, dwg_v, dwu_v, dwd_v, ob_v,
            sin, sout):
    ntc = S // TC
    nj = F // FT

    def blk(i, n):
        return pl.ds(pl.multiple_of(i * n, n), n)

    def cp(src, dst, sem):
        return pltpu.make_async_copy(src, dst, sem)

    x_cp = lambda i: cp(x_h.at[:, blk(i, TC)], x_v.at[:, blk(i, TC)], sin.at[i])
    fdt_cp = cp(fdt_h, fdt_v, sin.at[ntc])
    gm_cp = cp(gm_h, gm_v, sin.at[ntc + 1])
    fd_cp = cp(fd_h, fd_v, sin.at[ntc + 2])
    w_cp = [cp(wr_h, wb_v.at[0], sin.at[ntc + 3]), cp(wi_h, wb_v.at[1], sin.at[ntc + 4])]
    g_cp = cp(g_h, gt_v, sin.at[ntc + 5])
    ffn_cp = [cp(wg_h, wg_v, sin.at[ntc + 6]), cp(wu_h, wu_v, sin.at[ntc + 7]),
              cp(wd_h, wd_v, sin.at[ntc + 8])]

    x_cp(0).start()
    fdt_cp.start()
    for i in range(1, ntc):
        x_cp(i).start()
    for c in w_cp + [gm_cp, fd_cp, g_cp] + ffn_cp:
        c.start()

    def scale(row0, n):
        k = row0 + lax.broadcasted_iota(jnp.int32, (n, R2), 0)
        return jnp.where((k == 0) | (k == KF - 1), 1.0 / (S * D), 2.0 / (S * D))

    def radix_fwd():
        def body(r, carry):
            re = blk(r, 8)
            im = pl.ds(pl.multiple_of(r * 8 + KP, 8), 8)
            xs = [(z_v[re, n * R2:(n + 1) * R2], z_v[im, n * R2:(n + 1) * R2])
                  for n in range(R1)]
            for k, (a, b) in enumerate(_fft16(xs, -1)):
                t_v[k, re, 0:R2] = a
                t_v[k, re, R2:2 * R2] = b
            return carry
        lax.fori_loop(0, KP // 8, body, 0)

    def radix_inv():
        def body(r, carry):
            re = blk(r, 8)
            im = pl.ds(pl.multiple_of(r * 8 + KP, 8), 8)
            xs = [(t_v[n, re, 0:R2], t_v[n, re, R2:2 * R2]) for n in range(R1)]
            for k, (a, b) in enumerate(_fft16(xs, 1)):
                z_v[re, k * R2:(k + 1) * R2] = a
                z_v[im, k * R2:(k + 1) * R2] = b
            return carry
        lax.fori_loop(0, KP // 8, body, 0)

    fdt_cp.wait()

    def p1(i, carry):
        x_cp(i).wait()
        xn, _ = _ln(x_v[:, blk(i, TC)].astype(f32))
        z_v[:, blk(i, TC)] = _dot(fdt_v[...], xn.astype(bf16))
        return carry
    lax.fori_loop(0, ntc, p1, 0)

    radix_fwd()

    for c in w_cp:
        c.wait()

    def pw(r, carry):
        rr = blk(r, 16)
        for a in range(2):
            w = pltpu.bitcast(wb_v[a, rr, :], jnp.uint32)
            tiles = _shuffle16([w[:, t * R2:(t + 1) * R2] for t in range(R1)])
            for k in range(R1):
                wp_v[k, rr, a * R2:(a + 1) * R2] = pltpu.bitcast(tiles[k], bf16)
        return carry
    lax.fori_loop(0, (KF - 1) // 16, pw, 0)
    row = lax.broadcasted_iota(jnp.int32, (16, S), 0)
    for a in range(2):
        last = jnp.broadcast_to(wb_v[a, KF - 1:KF, :].astype(f32), (16, S))
        w = pltpu.bitcast(jnp.where(row == 0, last, 0.0).astype(bf16), jnp.uint32)
        tiles = _shuffle16([w[:, t * R2:(t + 1) * R2] for t in range(R1)])
        for k in range(R1):
            wp_v[k, KF - 1:KP, a * R2:(a + 1) * R2] = pltpu.bitcast(tiles[k], bf16)

    gm_cp.wait()

    def p3(k1, carry):
        xx = _dot(t_v[k1].astype(bf16), gm_v[k1])
        cc = scale(0, KP)
        xr, xi = xx[:, :R2] * cc, xx[:, R2:] * cc
        xs_v[k1, :, :R2] = xr
        xs_v[k1, :, R2:] = xi
        wr, wi = wp_v[k1, :, :R2].astype(f32), wp_v[k1, :, R2:].astype(f32)
        yy = jnp.concatenate([xr * wr - xi * wi, xr * wi + xi * wr], axis=1)
        t_v[k1] = _dot(yy.astype(bf16), gm_v[k1], NT)
        return carry
    lax.fori_loop(0, R1, p3, 0)

    radix_inv()

    fd_cp.wait()
    g_cp.wait()

    def p5(i, carry):
        c = blk(i, TC)
        h = x_v[:, c].astype(f32) + _dot(fd_v[...], z_v[:, c].astype(bf16))
        h_v[:, c] = h
        hn, _ = _ln(h)
        hnt_v[:, c] = hn.astype(bf16)
        hn_v[c, :] = hn.T.astype(bf16)
        g_v[c, :] = gt_v[:, c].astype(f32).T.astype(bf16)
        acco_v[:, c] = jnp.zeros((D, TC), f32)
        acch_v[:, c] = jnp.zeros((D, TC), f32)
        return carry
    lax.fori_loop(0, ntc, p5, 0)

    for c in ffn_cp:
        c.wait()

    def dw_cp(j):
        fs = blk(j, FT)
        return [cp(dwg_v.at[:, fs], dwg_h.at[:, fs], sout.at[3 * j]),
                cp(dwu_v.at[:, fs], dwu_h.at[:, fs], sout.at[3 * j + 1]),
                cp(dwd_v.at[:, fs], dwd_h.at[:, fs], sout.at[3 * j + 2])]

    def jbody(j, carry):
        fs = blk(j, FT)

        def ibody(i, carry):
            ss = blk(i, ST)
            hn = hn_v[ss, :]
            a = _dot(hn, wg_v[:, fs])
            u = _dot(hn, wu_v[:, fs])
            dp = _dot(g_v[ss, :], wd_v[:, fs])
            sg = jax.nn.sigmoid(a)
            sl = a * sg
            p = (sl * u).astype(bf16)
            du = (dp * sl).astype(bf16)
            da = (dp * u * (sg + sl * (1.0 - sg))).astype(bf16)
            p_v[ss, :] = p
            da_v[ss, :] = da
            du_v[ss, :] = du
            acco_v[:, ss] += _dot(wd_v[:, fs], p, NT)
            acch_v[:, ss] += _dot(wg_v[:, fs], da, NT) + _dot(wu_v[:, fs], du, NT)
            return carry
        lax.fori_loop(0, S // ST, ibody, 0)
        dwg_v[:, fs] = _dot(hnt_v[...], da_v[...]).astype(bf16)
        dwu_v[:, fs] = _dot(hnt_v[...], du_v[...]).astype(bf16)
        dwd_v[:, fs] = _dot(gt_v[...], p_v[...]).astype(bf16)
        for c in dw_cp(j):
            c.start()
        return carry
    lax.fori_loop(0, nj, jbody, 0)

    o_cp = cp(ob_v, out_h, sout.at[3 * nj])

    def p7(i, carry):
        c = blk(i, TC)
        h = h_v[:, c]
        ob_v[:, c] = (h + acco_v[:, c]).astype(bf16)
        hn, rstd = _ln(h)
        dh = gt_v[:, c].astype(f32) + _ln_bwd(acch_v[:, c], hn, rstd)
        h_v[:, c] = dh
        z_v[:, c] = _dot(fdt_v[...], dh.astype(bf16))
        return carry
    lax.fori_loop(0, ntc, p7, 0)
    o_cp.start()

    radix_fwd()

    def p9(k1, carry):
        dy = _dot(t_v[k1].astype(bf16), gm_v[k1])
        dr, di = dy[:, :R2], dy[:, R2:]
        cc = scale(0, KP)
        wr, wi = wp_v[k1, :, :R2].astype(f32) * cc, wp_v[k1, :, R2:].astype(f32) * cc
        dxx = jnp.concatenate([dr * wr + di * wi, di * wr - dr * wi], axis=1)
        t_v[k1] = _dot(dxx.astype(bf16), gm_v[k1], NT)
        xr, xi = xs_v[k1, :, :R2], xs_v[k1, :, R2:]
        wp_v[k1, :, :R2] = (dr * xr + di * xi).astype(bf16)
        wp_v[k1, :, R2:] = (di * xr - dr * xi).astype(bf16)
        return carry
    lax.fori_loop(0, R1, p9, 0)

    def pdw(r, carry):
        rr = blk(r, 16)
        for a in range(2):
            tiles = _shuffle16([pltpu.bitcast(wp_v[k, rr, a * R2:(a + 1) * R2], jnp.uint32)
                                for k in range(R1)])
            for t in range(R1):
                wb_v[a, rr, t * R2:(t + 1) * R2] = pltpu.bitcast(tiles[t], bf16)
        return carry
    lax.fori_loop(0, (KF - 1) // 16, pdw, 0)
    for a in range(2):
        tiles = _shuffle16([pltpu.bitcast(wp_v[k, KF - 1:KP, a * R2:(a + 1) * R2], jnp.uint32)
                            for k in range(R1)])
        for t in range(R1):
            wb_v[a, KF - 1:KF, t * R2:(t + 1) * R2] = (
                pltpu.bitcast(tiles[t], bf16).astype(f32)[0:1].astype(bf16))
    dw_out = [cp(wb_v.at[0], dwr_h, sout.at[3 * nj + 1]),
              cp(wb_v.at[1], dwi_h, sout.at[3 * nj + 2])]
    for c in dw_out:
        c.start()

    radix_inv()

    dx_cp = lambda i: cp(hnt_v.at[:, blk(i, TC)], dx_h.at[:, blk(i, TC)],
                         sout.at[3 * nj + 3 + i])

    def p11(i, carry):
        c = blk(i, TC)
        dxn = _dot(fd_v[...], z_v[:, c].astype(bf16))
        xn, rstd = _ln(x_v[:, c].astype(f32))
        hnt_v[:, c] = (h_v[:, c] + _ln_bwd(dxn, xn, rstd)).astype(bf16)
        dx_cp(i).start()
        return carry
    lax.fori_loop(0, ntc, p11, 0)

    for j in range(nj):
        for c in dw_cp(j):
            c.wait()
    o_cp.wait()
    for c in dw_out:
        c.wait()
    for i in range(ntc):
        dx_cp(i).wait()


@jax.jit
def pallas_sequential_preLN__spectral_gfnet__swiglu_ffn__prompt_kernel(
    A_x: jax.Array,
    A_w_r: jax.Array,
    A_w_i: jax.Array,
    B_x: jax.Array,
    B_w_gate: jax.Array,
    B_w_up: jax.Array,
    B_w_down: jax.Array,
    grad_out: jax.Array,
):
    del B_x
    V = pltpu.VMEM
    sds = jax.ShapeDtypeStruct
    hbm = pl.BlockSpec(memory_space=pltpu.HBM)
    out, dx, dwr, dwi, dwg, dwu, dwd = pl.pallas_call(
        _kernel,
        out_shape=[sds((D, S), bf16), sds((D, S), bf16),
                   sds((KF, S), bf16), sds((KF, S), bf16),
                   sds((D, F), bf16), sds((D, F), bf16), sds((D, F), bf16)],
        in_specs=[hbm] * 10,
        out_specs=[hbm] * 7,
        scratch_shapes=[
            V((D, S), bf16), V((D, S), bf16), V((2, KF, S), bf16),
            V((D, F), bf16), V((D, F), bf16), V((D, F), bf16),
            V((D, 2 * KP), bf16), V((2 * KP, D), bf16), V((R1, 2 * R2, 2 * R2), bf16),
            V((R1, KP, 2 * R2), bf16), V((2 * KP, S), f32), V((R1, KP, 2 * R2), f32),
            V((R1, KP, 2 * R2), f32),
            V((D, S), f32), V((S, D), bf16), V((D, S), bf16), V((S, D), bf16),
            V((S, FT), bf16), V((S, FT), bf16), V((S, FT), bf16),
            V((D, S), f32), V((D, S), f32),
            V((D, F), bf16), V((D, F), bf16), V((D, F), bf16), V((D, S), bf16),
            pltpu.SemaphoreType.DMA((S // TC + 9,)),
            pltpu.SemaphoreType.DMA((3 * (F // FT) + 3 + S // TC,)),
        ],
        compiler_params=pltpu.CompilerParams(vmem_limit_bytes=124 * 2**20),
    )(A_x[0].T, A_w_r.T, A_w_i.T, B_w_gate, B_w_up, B_w_down.T, grad_out[0].T,
      _FD, _FDT, _G)
    return out.T[None], dx.T[None], dwr.T, dwi.T, dwg, dwu, dwd.T
```

```python
import itertools
import math

import jax
import jax.numpy as jnp
import ml_dtypes
import numpy as np
from jax import lax
from jax.experimental import pallas as pl
from jax.experimental.pallas import tpu as pltpu

S, D, F = 2048, 576, 4608
KF = D // 2 + 1
KP = 304
R1, R2 = 16, 128
RD, DB = 9, 64
K0 = 256
EPS = 1e-5
DH, SH = D // 2, S // 2
KS = 256
TS = 256
TF = 256
EW = 16
WIN = 80
TC = 256

bf16 = jnp.bfloat16
f32 = jnp.float32
V = pltpu.VMEM
NN = (((1,), (0,)), ((), ()))
NT = (((1,), (1,)), ((), ()))


_C1, _C2, _C4 = (math.cos(2 * math.pi * e / RD) for e in (1, 2, 4))
_S1, _S2, _S3, _S4 = (math.sin(2 * math.pi * e / RD) for e in (1, 2, 3, 4))


def _cyc(m, a, b, c, k1, k2, k3):
    e1, e2 = a - c, b - c
    p, q = k1 * e1 + k2 * e2, k2 * e1 + k3 * e2
    return m + p, m + q, m - (p + q)


def _cyc_t(o1, o2, o3, k1, k2, k3):
    p, q = o1 - o3, o2 - o3
    e1, e2 = k1 * p + k2 * q, k2 * p + k3 * q
    return o1 + o2 + o3, e1, e2, -(e1 + e2)


def _rfft9(x):
    s1, s2, s3, s4 = (x[a] + x[RD - a] for a in (1, 2, 3, 4))
    t1, t2, t3, t4 = x[1] - x[8], x[7] - x[2], x[3] - x[6], x[4] - x[5]
    u, v = x[0] + s3, s1 + s2 + s4
    p1, p2, p4 = _cyc(x[0] - 0.5 * s3, s1, s2, s4, _C1, _C2, _C4)
    q1, q2, q4 = _cyc(_S3 * t3, t1, t2, t4, _S1, -_S2, _S4)
    return [p1, q1, p2, q2, u - 0.5 * v, t1 + t2 + t4, p4, q4, u + v]


def _rfft9_t(y):
    p1, q1, p2, q2, p3, q3, p4, q4, y0 = y
    m, s1, s2, s4 = _cyc_t(p1, p2, p4, _C1, _C2, _C4)
    n, t1, t2, t4 = _cyc_t(q1, q2, q4, _S1, -_S2, _S4)
    u, v = y0 + p3, y0 - 0.5 * p3
    s1, s2, s4, s3 = s1 + v, s2 + v, s4 + v, u - 0.5 * m
    t1, t2, t4, t3 = t1 + q3, t2 + q3, t4 + q3, _S3 * n
    return [u + m, s1 + t1, s2 - t2, s3 + t3, s4 + t4, s4 - t4, s3 - t3, s2 + t2, s1 - t1]


_CLASSES = [(64 * (c - 1) + 32 * h, (c, RD - c)[h], 32) for c in (1, 2, 3, 4) for h in (0, 1)]


def _consts():
    bins = np.full(KP, -1)
    for row, c, n in _CLASSES + [(K0, 0, 33)]:
        bins[row:row + n] = c + RD * np.arange(n)
    ang = 2.0 * np.pi * ((bins[:, None] * np.arange(D)[None, :]) % D) / D
    live = (bins >= 0)[:, None]
    inv = np.kron(np.linalg.inv(np.stack(_rfft9(list(np.eye(RD))))), np.eye(DB))
    re, im = (np.cos(ang) * live) @ inv, (-np.sin(ang) * live) @ inv
    fa = np.zeros((11, R2, R2))
    for c in range(5):
        r0, r1 = 64 * c, min(64 * c + 64, KP)
        m = np.concatenate([re[r0:r1], im[r0:r1]])[:, R2 * c:R2 * c + R2]
        fa[c, :m.shape[0], :m.shape[1]] = m
        fa[5 + c] = fa[c].T
    fa[10] = fa[9]
    fa[10, :, 0] = 0.0
    k1 = np.arange(R1)[:, None, None]
    n2 = np.arange(R2)[None, :, None]
    lane = (np.arange(R2)[None, None, :] - k1) % R2
    k2 = 8 * (lane % 16) + lane // 16
    ang = 2.0 * np.pi * ((n2 * (k1 + R1 * k2)) % S) / S
    gr, gi = np.cos(ang), -np.sin(ang)
    g = np.concatenate([np.concatenate([gr, gi], 2), np.concatenate([-gi, gr], 2)], 1)
    cast = lambda a: np.ascontiguousarray(a).astype(np.float32).astype(ml_dtypes.bfloat16)
    return cast(fa), cast(g)


_FA, _G = _consts()
_ZERO = np.zeros((8, R2), np.int32)


def _dot(a, b, dn=NN):
    return lax.dot_general(a, b, dn, preferred_element_type=f32)


def _fft4(x, sign):
    (ar, ai), (br, bi), (cr, ci), (dr, di) = x
    s0r, s0i, d0r, d0i = ar + cr, ai + ci, ar - cr, ai - ci
    s1r, s1i, d1r, d1i = br + dr, bi + di, br - dr, bi - di
    lo = (d0r + d1i, d0i - d1r)
    hi = (d0r - d1i, d0i + d1r)
    o1, o3 = (lo, hi) if sign < 0 else (hi, lo)
    return [(s0r + s1r, s0i + s1i), o1, (s0r - s1r, s0i - s1i), o3]


def _tw16(v, e, sign):
    r, i = v
    e %= 16
    if e == 0:
        return v
    if e == 4:
        return (i, -r) if sign < 0 else (-i, r)
    c = math.cos(2 * math.pi * e / 16)
    s = sign * math.sin(2 * math.pi * e / 16)
    if e % 2 == 0:
        if c * s > 0:
            return ((r - i) * c, (r + i) * c)
        return ((r + i) * c, (i - r) * c)
    return (r * c - i * s, r * s + i * c)


def _fft16(x, sign):
    cols = [_fft4([x[4 * a + b] for a in range(4)], sign) for b in range(4)]
    out = [None] * 16
    for p in range(4):
        o = _fft4([_tw16(cols[b][p], b * p, sign) for b in range(4)], sign)
        for q in range(4):
            out[p + 4 * q] = o[q]
    return out


def _swap16(tiles):
    lane = lax.broadcasted_iota(jnp.int32, tiles[0].shape, 1)
    tiles = list(tiles)
    for d in (1, 2, 4, 8):
        for lo in range(d):
            low = ((lane - lo) & d) == 0
            for t in range(lo, R1, 2 * d):
                a, b = tiles[t], tiles[t + d]
                tiles[t], tiles[t + d] = jnp.where(low, a, b), jnp.where(low, b, a)
    return tiles


def _rot16(tiles, sign):
    return [pltpu.roll(v, (sign * t) % R2, 1) if t else v for t, v in enumerate(tiles)]


def _act_forms(a11, a12, a21, a22):
    return (a11 + a22, a21 + a22, a11, a22, a11 + a12, a21 - a11, a12 - a22)


def _hid_forms(p11, p12, p21, p22):
    return (p11 + p22, p11, p12 - p22, p21 - p11, p22, p11 + p12, p21 + p22)


def _wgt_forms(w11, w12, w21, w22):
    return (w11 + w22, w21 - w22, w12 + w22, w11 + w21, w12 - w11)


def _act_join(n):
    return (jnp.concatenate([n[0] + n[2] + n[4] - n[5], n[1] + n[5]], axis=0),
            jnp.concatenate([n[4] + n[6], n[0] + n[1] + n[3] - n[6]], axis=0))


def _colmean(x):
    return jnp.sum(x, axis=0, keepdims=True) * (1.0 / D)


def _split9(x):
    return [x[a * DB:(a + 1) * DB] for a in range(RD)]


def _kernel(x_h, wr_h, wi_h, wg_h, wu_h, wd_h, g_h, fa_h, gm_h, zero_h,
            out_h, dx_h, dwr_h, dwi_h, dwg_h, dwu_h, dwd_h,
            x_v, g_v, wb_v, w_v, fa_v, gm_v, zero_v,
            wp_v, xs_v, st_v, h_v, hf_v, gf_v, hk_v, gk_v, hr_v, gr_v,
            acco_v, acch_v, dw_v, sin, sout):
    ntc = S // TC
    nj = F // (2 * TF)
    ni = SH // TS

    def loop(name, n, body, lo=0):
        with jax.named_scope(name):
            lax.fori_loop(lo, n, body, 0)

    def blk(i, n):
        return pl.ds(pl.multiple_of(i * n, n), n)

    def cp(src, dst, sem):
        return pltpu.make_async_copy(src, dst, sem)

    x_cp = lambda i: cp(x_h.at[:, blk(i, TC)], x_v.at[:, blk(i, TC)], sin.at[i])
    fa_cp = cp(fa_h, fa_v, sin.at[ntc])
    gm_cp = cp(gm_h, gm_v, sin.at[ntc + 1])
    w_cp = [cp(wr_h, wb_v.at[0], sin.at[ntc + 3]), cp(wi_h, wb_v.at[1], sin.at[ntc + 4])]
    g_cp = cp(g_h, g_v, sin.at[ntc + 5])
    ffn_cp = [cp(wg_h, w_v.at[0], sin.at[ntc + 6]), cp(wu_h, w_v.at[1], sin.at[ntc + 7]),
              cp(wd_h, w_v.at[2], sin.at[ntc + 8]), cp(zero_h, zero_v, sin.at[ntc + 2])]

    x_cp(0).start()
    fa_cp.start()
    for i in range(1, ntc):
        x_cp(i).start()
    for c in w_cp + [gm_cp, g_cp] + ffn_cp:
        c.start()

    def scale(row0, n):
        k = row0 + lax.broadcasted_iota(jnp.int32, (n, R2), 0)
        return jnp.where((k == K0) | (k == K0 + 32), 1.0 / (S * D), 2.0 / (S * D))

    def dft_d(y):
        out = [_dot(fa_v[c], jnp.concatenate(y[2 * c:2 * c + 2], axis=0).astype(bf16))
               for c in range(4)]
        o0 = _dot(fa_v[4, :2 * (KP - K0), :DB], y[8].astype(bf16))
        return jnp.concatenate([o[:DB] for o in out] + [o0[:KP - K0]]
                               + [o[DB:] for o in out] + [o0[KP - K0:]], axis=0)

    def idft_d(z, last):
        y = []
        for c in range(4):
            zc = jnp.concatenate([z[DB * c:DB * c + DB], z[KP + DB * c:KP + DB * c + DB]], axis=0)
            o = _dot(fa_v[5 + c], zc.astype(bf16))
            y += [o[:DB], o[DB:]]
        zc = jnp.concatenate([z[K0:KP], z[KP + K0:]], axis=0)
        y.append(_dot(fa_v[last, :DB, :2 * (KP - K0)], zc.astype(bf16)))
        return jnp.concatenate(_rfft9_t(y), axis=0)

    def filt(k1):
        rows = [pl.ds(c, n, stride=RD) for _, c, n in _CLASSES + [(K0, 0, KP - K0)]]
        return [jnp.concatenate([wp_v[a, k1, r, :] for r in rows], axis=0) for a in range(2)]

    def radix_fwd(z_v, t_v):
        def body(r, carry):
            re = blk(r, 8)
            im = pl.ds(pl.multiple_of(r * 8 + KP, 8), 8)
            xs = [(z_v[re, n * R2:(n + 1) * R2], z_v[im, n * R2:(n + 1) * R2])
                  for n in range(R1)]
            for k, (a, b) in enumerate(_fft16(xs, -1)):
                t_v[k, re, 0:R2] = a
                t_v[k, re, R2:2 * R2] = b
            return carry
        loop("radix", KP // 8, body)

    def radix_inv(z_v, t_v):
        def body(r, carry):
            re = blk(r, 8)
            im = pl.ds(pl.multiple_of(r * 8 + KP, 8), 8)
            xs = [(t_v[n, re, 0:R2], t_v[n, re, R2:2 * R2]) for n in range(R1)]
            for k, (a, b) in enumerate(_fft16(xs, 1)):
                z_v[re, k * R2:(k + 1) * R2] = a
                z_v[im, k * R2:(k + 1) * R2] = b
            return carry
        loop("radix", KP // 8, body)

    def spectral_fwd(z_v, t_v):
        fa_cp.wait()

        def p1(i, carry):
            x_cp(i).wait()
            c = blk(i, TC)
            y = _rfft9(_split9(x_v[:, c].astype(f32)))
            mu = _colmean(y[8])
            y[8] = y[8] - RD * mu
            sq = [v * v for v in y]
            en = (sq[8] + 1.5 * sq[5]
                  + 2.0 * (sq[0] + sq[1] + sq[2] + sq[3] + sq[4] + sq[6] + sq[7]))
            rstd = 1.0 / jnp.sqrt(_colmean(en) * (1.0 / RD) + EPS)
            st_v[0, :, c] = mu
            st_v[1, :, c] = rstd
            z_v[:, c] = dft_d(y) * rstd
            return carry
        loop("p1", ntc, p1)

        radix_fwd(z_v, t_v)

        for c in w_cp:
            c.wait()

        def put_w(a, rr, w):
            w = pltpu.bitcast(w, jnp.uint32)
            tiles = _swap16(_rot16([w[:, t * R2:(t + 1) * R2] for t in range(R1)], 1))
            for k in range(R1):
                wp_v[a, k, rr, :] = pltpu.bitcast(tiles[k], bf16).astype(f32)

        def pw(r, carry):
            for a in range(2):
                put_w(a, blk(r, 32), wb_v[a, blk(r, 32), :])
            return carry
        loop("pw", (KF - 1) // 32, pw)
        row = lax.broadcasted_iota(jnp.int32, (16, S), 0)
        for a in range(2):
            last = jnp.broadcast_to(wb_v[a, KF - 1:KF, :].astype(f32), (16, S))
            put_w(a, slice(KF - 1, KP), jnp.where(row == 0, last, 0.0).astype(bf16))
            for k in range(R1):
                for m in range(34, KP - K0):
                    wp_v[a, k, RD * m:RD * m + 1, :] = jnp.zeros((1, R2), f32)

        gm_cp.wait()

        def p3(k1, carry):
            xx = _dot(t_v[k1].astype(bf16), gm_v[k1])
            cc = scale(0, KP)
            xr, xi = xx[:, :R2] * cc, xx[:, R2:] * cc
            xs_v[k1, :, :R2] = xr.astype(bf16)
            xs_v[k1, :, R2:] = xi.astype(bf16)
            wr, wi = filt(k1)
            yy = jnp.concatenate([xr * wr - xi * wi, xr * wi + xi * wr], axis=1)
            t_v[k1] = _dot(yy.astype(bf16), gm_v[k1], NT)
            return carry
        loop("p3", R1, p3)

        radix_inv(z_v, t_v)

        g_cp.wait()

        def forms(i, xa, xb, f_v, k_v, r_v):
            c = blk(i, R2)
            for r, v in enumerate(_act_forms(xa[:DH], xb[:DH], xa[DH:], xb[DH:])):
                f_v[r, :, c] = v.astype(bf16)
            for r, v in enumerate(_act_forms(xa[:KS].T, xb[:KS].T,
                                             xa[DH:DH + KS].T, xb[DH:DH + KS].T)):
                k_v[r, c, :] = v.astype(bf16)
            rest = jnp.concatenate([xa[KS:DH], xa[DH + KS:], xb[KS:DH], xb[DH + KS:]], axis=0).T
            r_v[0, c, :] = rest[:, :D - 2 * KS].astype(bf16)
            r_v[1, c, :] = rest[:, D - 2 * KS:].astype(bf16)

        def p5(i, carry):
            ca, cb = blk(i, R2), blk(i + SH // R2, R2)
            hn = []
            for c in (ca, cb):
                h = x_v[:, c].astype(f32) + idft_d(z_v[:, c], 9)
                mu = _colmean(h)
                hc = h - mu
                rstd = 1.0 / jnp.sqrt(_colmean(hc * hc) + EPS)
                st_v[2, :, c] = mu
                st_v[3, :, c] = rstd
                h_v[:, c] = h
                hn.append(hc * rstd)
            forms(i, hn[0], hn[1], hf_v, hk_v, hr_v)
            forms(i, g_v[:, ca].astype(f32), g_v[:, cb].astype(f32), gf_v, gk_v, gr_v)
            return carry
        loop("p5", SH // R2, p5)

    pl.run_scoped(spectral_fwd, V((2 * KP, S), f32), V((R1, KP, 2 * R2), f32))

    def dw_cp(j):
        return [cp(dw_v.at[j % 2, m], o.at[:, blk(j, 2 * TF)], sout.at[3 * (j % 2) + m])
                for m, o in enumerate((dwg_h, dwu_h, dwd_h))]

    def ffn(ws_v, p_v, raw_v, m_v):
        def window(q):
            r0 = pl.multiple_of(jnp.minimum(q * WIN, DH - WIN), 16)
            return pl.ds(r0, WIN), pl.ds(pl.multiple_of(r0 + DH, 16), WIN)

        def wprep(j, q):
            src = jnp.minimum(j, nj - 1)
            f1, f2 = blk(2 * src, TF), blk(2 * src + 1, TF)
            d1, d2 = window(q)
            for m in range(3):
                for r, v in enumerate(_wgt_forms(w_v[m, d1, f1], w_v[m, d1, f2],
                                                 w_v[m, d2, f1], w_v[m, d2, f2])):
                    ws_v[j % 3, m, r, d1, :] = v

        def wform(j, m, r, n):
            if r < 5:
                return ws_v[j % 3, m, r, 0:n, :]
            return w_v[m, DH:DH + n, blk(2 * j + 1, TF)] if r == 5 else w_v[m, 0:n, blk(2 * j, TF)]

        def finalize(j, q):
            d1, d2 = window(q)
            for m in range(3):
                n = [m_v[m][r][j % 2, d1, :] for r in range(7)]
                dw_v[j % 2, m, d1, :TF] = (n[0] + n[3] - n[4] + n[6]).astype(bf16)
                dw_v[j % 2, m, d1, TF:] = (n[2] + n[4]).astype(bf16)
                dw_v[j % 2, m, d2, :TF] = (n[1] + n[3]).astype(bf16)
                dw_v[j % 2, m, d2, TF:] = (n[0] - n[1] + n[2] + n[5]).astype(bf16)

        def stage1(t):
            j, ss = t // ni, blk(t % ni, TS)
            f1, f2 = blk(2 * j, TF), blk(2 * j + 1, TF)
            wprep(j + 1, t % ni)
            for m, (k_v, r_v) in enumerate(((hk_v, hr_v), (hk_v, hr_v), (gk_v, gr_v))):
                t1, t2 = r_v[0, ss, :], r_v[1, ss, :]
                w1, w2 = [jnp.concatenate([w_v[m, KS:DH, f], w_v[m, DH + KS:, f]], axis=0)
                          for f in (f1, f2)]
                q = lambda r: _dot(k_v[r, ss, :], wform(j, m, r, KS))
                q2 = q(2)
                yield q2
                q5 = q(5)
                yield q5
                raw_v[m, 1] = q2 + q5 + _dot(t1, w2)
                q3 = q(3)
                yield q3
                q6 = q(6)
                yield q6
                raw_v[m, 2] = q3 + q6 + _dot(t2, w1)
                q0 = q(0)
                yield q0
                q1 = q(1)
                raw_v[m, 0] = (q0 + q5 - q3) + q1 + _dot(t1, w1)
                yield q1
                q4 = q(4)
                raw_v[m, 3] = (q0 - q2 + q6) + q4 + _dot(t2, w2)
                yield q4

        def gate(t, r0, after):
            rows = slice(r0, r0 + EW)
            res = ([], [], [])
            if after is not None:
                keep = jnp.tile(zero_v[...] == 0, (EW // 8, TF // R2))
                after = jnp.tile(after[:8, :R2], (EW // 8, TF // R2))
            for q in range(4):
                a, u, dp = raw_v[0, q, rows], raw_v[1, q, rows], raw_v[2, q, rows]
                if after is not None:
                    a = jnp.where(keep, a, after)
                sg = jax.nn.sigmoid(a)
                sl = a * sg
                res[0].append(dp * u * (sg + sl * (1.0 - sg)))
                res[1].append(dp * sl)
                res[2].append(sl * u)
            for m in range(3):
                for r, v in enumerate(_hid_forms(*res[m])):
                    p_v[t % 2, m, r, rows, :] = v.astype(bf16)

        def stage2(t):
            j, i = t // ni, t % ni
            ss, b = blk(i, TS), t % 2
            finalize(j + 1, i)
            for r in range(7):
                o = _dot(wform(j, 2, r, DH), p_v[b, 2, r], NT)
                acco_v[r][:, ss] = jnp.where(j == 0, 0.0, acco_v[r][:, ss]) + o
                yield o
                o = (_dot(wform(j, 0, r, DH), p_v[b, 0, r], NT)
                     + _dot(wform(j, 1, r, DH), p_v[b, 1, r], NT))
                acch_v[r][:, ss] = jnp.where(j == 0, 0.0, acch_v[r][:, ss]) + o
                yield o
                for m, f_v in enumerate((hf_v, hf_v, gf_v)):
                    o = _dot(f_v[r, :, ss], p_v[b, m, r])
                    m_v[m][r][j % 2] = jnp.where(i == 0, 0.0, m_v[m][r][j % 2]) + o
                    yield o

        def step(dots, t, ndots):
            nchunk = TS // EW
            done = 0
            for k, o in enumerate(dots):
                while t is not None and done < nchunk and done * ndots <= k * nchunk:
                    gate(t, done * EW, o)
                    done += 1

        for c in ffn_cp:
            c.wait()
        loop("wprep0", ni, lambda q, carry: (wprep(0, q), carry)[1])
        nt = nj * ni
        with jax.named_scope("head"):
            step(stage1(0), None, 0)
            for r0 in range(0, TS, EW):
                gate(0, r0, None)
            step(stage1(1), None, 0)

        def body(t, carry):
            j, i = (t - 1) // ni, (t - 1) % ni

            @pl.when((i == 0) & (j >= 2))
            def _():
                @pl.when(j >= 3)
                def _():
                    for c in dw_cp(j - 3):
                        c.wait()
                for c in dw_cp(j - 2):
                    c.start()
            step(itertools.chain(stage2(t - 1), stage1(t + 1)), t, 35)
            return carry
        loop("ffn", nt - 1, body, 1)
        with jax.named_scope("tail"):
            step(stage2(nt - 2), nt - 1, 35)
            step(stage2(nt - 1), None, 0)
            for c in dw_cp(nj - 2):
                c.start()
            for c in dw_cp(nj - 3):
                c.wait()
        loop("fin", ni, lambda q, carry: (finalize(nj - 1, q), carry)[1])
        for c in dw_cp(nj - 1):
            c.start()

    pl.run_scoped(ffn, V((3, 3, 5, DH, TF), bf16), V((2, 3, 7, TS, TF), bf16),
                  V((3, 4, TS, TF), f32), [[V((2, DH, TF), f32)] * 7] * 3)

    def spectral_bwd(z_v, t_v, ob_v, dx_v):
        o_cp = cp(ob_v, out_h, sout.at[6])

        def p7(i, carry):
            c = blk(i, R2)
            o = _act_join([acco_v[r][:, c] for r in range(7)])
            dn = _act_join([acch_v[r][:, c] for r in range(7)])
            for half, cc in enumerate((c, blk(i + SH // R2, R2))):
                h = h_v[:, cc]
                ob_v[:, cc] = (h + o[half]).astype(bf16)
                rstd = st_v[3, :, cc]
                hn = (h - st_v[2, :, cc]) * rstd
                d = dn[half]
                dh = g_v[:, cc].astype(f32) + rstd * (d - _colmean(d) - hn * _colmean(d * hn))
                h_v[:, cc] = dh
                z_v[:, cc] = dft_d(_rfft9(_split9(dh)))
            return carry
        loop("p7", SH // R2, p7)
        o_cp.start()

        radix_fwd(z_v, t_v)

        def p9(k1, carry):
            dy = _dot(t_v[k1].astype(bf16), gm_v[k1])
            dr, di = dy[:, :R2], dy[:, R2:]
            cc = scale(0, KP)
            wr, wi = (w * cc for w in filt(k1))
            dxx = jnp.concatenate([dr * wr + di * wi, di * wr - dr * wi], axis=1)
            t_v[k1] = _dot(dxx.astype(bf16), gm_v[k1], NT)
            xr, xi = xs_v[k1, :, :R2].astype(f32), xs_v[k1, :, R2:].astype(f32)
            for a, v in enumerate((dr * xr + di * xi, di * xr - dr * xi)):
                for row, c, n in _CLASSES + [(K0, 0, 40)]:
                    wp_v[a, k1, pl.ds(c, n, stride=RD), :] = v[row:row + n]
            return carry
        loop("p9", R1, p9)

        def get_dw(a, rr):
            tiles = [pltpu.bitcast(wp_v[a, k, rr, :].astype(bf16), jnp.uint32) for k in range(R1)]
            return pltpu.bitcast(jnp.concatenate(_rot16(_swap16(tiles), -1), axis=1), bf16)

        def pdw(r, carry):
            for a in range(2):
                wb_v[a, blk(r, 32), :] = get_dw(a, blk(r, 32))
            return carry
        loop("pdw", (KF - 1) // 32, pdw)
        for a in range(2):
            wb_v[a, KF - 1:KF, :] = get_dw(a, slice(KF - 1, KP)).astype(f32)[0:1].astype(bf16)
        dw_out = [cp(wb_v.at[0], dwr_h, sout.at[7]),
                  cp(wb_v.at[1], dwi_h, sout.at[8])]
        for c in dw_out:
            c.start()

        radix_inv(z_v, t_v)

        dx_cp = lambda i: cp(dx_v.at[:, blk(i, TC)], dx_h.at[:, blk(i, TC)],
                             sout.at[9 + i])

        def p11(i, carry):
            c = blk(i, TC)
            dxn = idft_d(z_v[:, c], 10)
            rstd = st_v[1, :, c]
            xn = (x_v[:, c].astype(f32) - st_v[0, :, c]) * rstd
            dx_v[:, c] = (h_v[:, c] + rstd * (dxn - xn * _colmean(dxn * xn))).astype(bf16)
            dx_cp(i).start()
            return carry
        loop("p11", ntc, p11)

        for j in (nj - 2, nj - 1):
            for c in dw_cp(j):
                c.wait()
        o_cp.wait()
        for c in dw_out:
            c.wait()
        for i in range(ntc):
            dx_cp(i).wait()

    pl.run_scoped(spectral_bwd, V((2 * KP, S), f32), V((R1, KP, 2 * R2), f32),
                  V((D, S), bf16), V((D, S), bf16))


@jax.jit
def pallas_sequential_preLN__spectral_gfnet__swiglu_ffn__prompt_kernel(
    A_x: jax.Array,
    A_w_r: jax.Array,
    A_w_i: jax.Array,
    B_x: jax.Array,
    B_w_gate: jax.Array,
    B_w_up: jax.Array,
    B_w_down: jax.Array,
    grad_out: jax.Array,
):
    del B_x
    sds = jax.ShapeDtypeStruct
    hbm = pl.BlockSpec(memory_space=pltpu.HBM)
    out, dx, dwr, dwi, dwg, dwu, dwd = pl.pallas_call(
        _kernel,
        out_shape=[sds((D, S), bf16), sds((D, S), bf16),
                   sds((KF, S), bf16), sds((KF, S), bf16),
                   sds((D, F), bf16), sds((D, F), bf16), sds((D, F), bf16)],
        in_specs=[hbm] * 10,
        out_specs=[hbm] * 7,
        scratch_shapes=[
            V((D, S), bf16), V((D, S), bf16), V((2, KF, S), bf16), V((3, D, F), bf16),
            V((11, R2, R2), bf16), V((R1, 2 * R2, 2 * R2), bf16),
            V((8, R2), jnp.int32),
            V((2, R1, RD * (KP - K0), R2), f32), V((R1, KP, 2 * R2), bf16),
            V((4, 1, S), f32), V((D, S), f32),
            V((7, DH, SH), bf16), V((7, DH, SH), bf16),
            V((7, SH, KS), bf16), V((7, SH, KS), bf16),
            V((2, SH, D - 2 * KS), bf16), V((2, SH, D - 2 * KS), bf16),
            [V((DH, SH), f32)] * 7, [V((DH, SH), f32)] * 7,
            V((2, 3, D, 2 * TF), bf16),
            pltpu.SemaphoreType.DMA((S // TC + 9,)),
            pltpu.SemaphoreType.DMA((9 + S // TC,)),
        ],
        compiler_params=pltpu.CompilerParams(vmem_limit_bytes=124 * 2**20),
    )(A_x[0].T, A_w_r.T, A_w_i.T, B_w_gate, B_w_up, B_w_down.T, grad_out[0].T,
      _FA, _G, _ZERO)
    return out.T[None], dx.T[None], dwr.T, dwi.T, dwg, dwu, dwd.T
```

```python
import functools
import itertools
import math

import jax
import jax.numpy as jnp
import ml_dtypes
import numpy as np
from jax import lax
from jax.experimental import pallas as pl
from jax.experimental.pallas import tpu as pltpu

S, D, F = 2048, 576, 4608
KF = D // 2 + 1
KP = 304
R1, R2 = 16, 128
RD, DB = 9, 64
K0 = 256
EPS = 1e-5
DH, SH = D // 2, S // 2
KA, KS = 192, 256
TS = 256
TF = 256
UN = 2
EW = 16
WIN = 80
TC = 256

bf16 = jnp.bfloat16
f32 = jnp.float32
u32 = jnp.uint32
V = pltpu.VMEM
NN = (((1,), (0,)), ((), ()))
NT = (((1,), (1,)), ((), ()))


_C1, _C2, _C4 = (math.cos(2 * math.pi * e / RD) for e in (1, 2, 4))
_S1, _S2, _S3, _S4 = (math.sin(2 * math.pi * e / RD) for e in (1, 2, 3, 4))


def _cyc(m, a, b, c, k1, k2, k3):
    e1, e2 = a - c, b - c
    p, q = k1 * e1 + k2 * e2, k2 * e1 + k3 * e2
    return m + p, m + q, m - (p + q)


def _cyc_t(o1, o2, o3, k1, k2, k3):
    p, q = o1 - o3, o2 - o3
    e1, e2 = k1 * p + k2 * q, k2 * p + k3 * q
    return o1 + o2 + o3, e1, e2, -(e1 + e2)


def _rfft9(x):
    s1, s2, s3, s4 = (x[a] + x[RD - a] for a in (1, 2, 3, 4))
    t1, t2, t3, t4 = x[1] - x[8], x[7] - x[2], x[3] - x[6], x[4] - x[5]
    u, v = x[0] + s3, s1 + s2 + s4
    p1, p2, p4 = _cyc(x[0] - 0.5 * s3, s1, s2, s4, _C1, _C2, _C4)
    q1, q2, q4 = _cyc(_S3 * t3, t1, t2, t4, _S1, -_S2, _S4)
    return [p1, q1, p2, q2, u - 0.5 * v, t1 + t2 + t4, p4, q4, u + v]


def _rfft9_t(y):
    p1, q1, p2, q2, p3, q3, p4, q4, y0 = y
    m, s1, s2, s4 = _cyc_t(p1, p2, p4, _C1, _C2, _C4)
    n, t1, t2, t4 = _cyc_t(q1, q2, q4, _S1, -_S2, _S4)
    u, v = y0 + p3, y0 - 0.5 * p3
    s1, s2, s4, s3 = s1 + v, s2 + v, s4 + v, u - 0.5 * m
    t1, t2, t4, t3 = t1 + q3, t2 + q3, t4 + q3, _S3 * n
    return [u + m, s1 + t1, s2 - t2, s3 + t3, s4 + t4, s4 - t4, s3 - t3, s2 + t2, s1 - t1]


_CLASSES = [(64 * (c - 1) + 32 * h, (c, RD - c)[h], 32) for c in (1, 2, 3, 4) for h in (0, 1)]


def _consts():
    bins = np.full(KP, -1)
    for row, c, n in _CLASSES + [(K0, 0, 33)]:
        bins[row:row + n] = c + RD * np.arange(n)
    ang = 2.0 * np.pi * ((bins[:, None] * np.arange(D)[None, :]) % D) / D
    live = (bins >= 0)[:, None]
    inv = np.kron(np.linalg.inv(np.stack(_rfft9(list(np.eye(RD))))), np.eye(DB))
    re, im = (np.cos(ang) * live) @ inv, (-np.sin(ang) * live) @ inv
    fa = np.zeros((11, R2, R2))
    for c in range(5):
        r0, r1 = 64 * c, min(64 * c + 64, KP)
        m = np.concatenate([re[r0:r1], im[r0:r1]])[:, R2 * c:R2 * c + R2]
        fa[c, :m.shape[0], :m.shape[1]] = m
        fa[5 + c] = fa[c].T
    fa[10] = fa[9]
    fa[10, :, 0] = 0.0
    k1 = np.arange(R1)[:, None, None]
    n2 = np.arange(R2)[None, :, None]
    lane = (np.arange(R2)[None, None, :] - k1) % R2
    k2 = 8 * (lane % 16) + lane // 16
    ang = 2.0 * np.pi * ((n2 * (k1 + R1 * k2)) % S) / S
    gr, gi = np.cos(ang), -np.sin(ang)
    g = np.concatenate([gr, gi], 2)
    cast = lambda a: np.ascontiguousarray(a).astype(np.float32).astype(ml_dtypes.bfloat16)
    return cast(fa), cast(g)


_FA, _G = _consts()
_ZERO = np.zeros((8, R2), np.int32)


def _dot(a, b, dn=NN):
    return lax.dot_general(a, b, dn, preferred_element_type=f32)


def _fft4(x, sign):
    (ar, ai), (br, bi), (cr, ci), (dr, di) = x
    s0r, s0i, d0r, d0i = ar + cr, ai + ci, ar - cr, ai - ci
    s1r, s1i, d1r, d1i = br + dr, bi + di, br - dr, bi - di
    lo = (d0r + d1i, d0i - d1r)
    hi = (d0r - d1i, d0i + d1r)
    o1, o3 = (lo, hi) if sign < 0 else (hi, lo)
    return [(s0r + s1r, s0i + s1i), o1, (s0r - s1r, s0i - s1i), o3]


def _tw16(v, e, sign):
    r, i = v
    e %= 16
    if e == 0:
        return v
    if e == 4:
        return (i, -r) if sign < 0 else (-i, r)
    c = math.cos(2 * math.pi * e / 16)
    s = sign * math.sin(2 * math.pi * e / 16)
    if e % 2 == 0:
        if c * s > 0:
            return ((r - i) * c, (r + i) * c)
        return ((r + i) * c, (i - r) * c)
    return (r * c - i * s, r * s + i * c)


def _fft16(x, sign):
    cols = [_fft4([x[4 * a + b] for a in range(4)], sign) for b in range(4)]
    out = [None] * 16
    for p in range(4):
        o = _fft4([_tw16(cols[b][p], b * p, sign) for b in range(4)], sign)
        for q in range(4):
            out[p + 4 * q] = o[q]
    return out


def _swap16(tiles):
    lane = lax.broadcasted_iota(jnp.int32, tiles[0].shape, 1)
    tiles = list(tiles)
    for d in (1, 2, 4, 8):
        for lo in range(d):
            low = ((lane - lo) & d) == 0
            for t in range(lo, R1, 2 * d):
                a, b = tiles[t], tiles[t + d]
                tiles[t], tiles[t + d] = jnp.where(low, a, b), jnp.where(low, b, a)
    return tiles


def _rot16(tiles, sign):
    return [pltpu.roll(v, (sign * t) % R2, 1) if t else v for t, v in enumerate(tiles)]


def _act_forms(a11, a12, a21, a22):
    return (a11 + a22, a21 + a22, a11, a22, a11 + a12, a21 - a11, a12 - a22)


def _hid_forms(p11, p12, p21, p22):
    return (p11 + p22, p11, p12 - p22, p21 - p11, p22, p11 + p12, p21 + p22)


def _wgt_forms(w11, w12, w21, w22):
    return (lambda: w11() + w22(), lambda: w21() - w22(), lambda: w12() + w22(),
            lambda: w11() + w21(), lambda: w12() - w11(), w22, w11)


def _act_join(n):
    return (jnp.concatenate([n[0] + n[2] + n[4] - n[5], n[1] + n[5]], axis=0),
            jnp.concatenate([n[4] + n[6], n[0] + n[1] + n[3] - n[6]], axis=0))


def _pk(v):
    return pltpu.bitcast(v.astype(bf16), u32)


def _up(v):
    return pltpu.bitcast(v, bf16)


def _colmean(x):
    return jnp.sum(x, axis=0, keepdims=True) * (1.0 / D)


def _split9(x):
    return [x[a * DB:(a + 1) * DB] for a in range(RD)]


def _overlap(dots, *tasks):
    plan = [(first + s * (last - first + 1) // len(steps), step)
            for steps, first, last in tasks for s, step in enumerate(steps)]
    span = {id(step): -(-(last - first + 1) // len(steps))
            for steps, first, last in tasks for step in steps}
    seen = []
    for k, o in enumerate(dots):
        seen.append(o)
        for at, step in plan:
            if at == k:
                step(seen[-span[id(step)]:])
    assert all(at < len(seen) for at, _ in plan)


def _kernel(x_h, wr_h, wi_h, wg_h, wu_h, wd_h, g_h, fa_h, gm_h, zero_h,
            out_h, dx_h, dwr_h, dwi_h, dwg_h, dwu_h, dwd_h,
            x_v, g_v, wb_v, w_v, fa_v, gm_v, zero_v,
            z_v, t_v, wp_v, xs_v, st_v, h_v, hf_v, gf_v, hk_v, gk_v, hr_v, gr_v,
            ws_v, raw_v, p_v, acco_v, acch_v, m_v, dw_v, sin, sout):
    ntc = S // TC
    nj = F // (2 * TF)
    ni = SH // TS
    nt = nj * ni
    assert ni == 4 and nt % 2 == 0
    part, chain = functools.partial, itertools.chain

    def loop(name, n, body, lo=0):
        with jax.named_scope(name):
            lax.fori_loop(lo, n, lambda i, carry: (body(i), carry)[1], 0)

    def blk(i, n):
        return pl.ds(i * n, n) if isinstance(i, int) else pl.ds(pl.multiple_of(i * n, n), n)

    def pace(vals, after):
        if not after:
            return vals
        keep = zero_v[...] == 0
        marks = [o[r:r + 8, :R2] for o in after for r in range(0, o.shape[0], 8)]
        n = sum(v.size for v in vals) // (8 * R2)
        marks = iter([marks[i * len(marks) // n] for i in range(n)])
        return [jnp.block([[jnp.where(keep, v[r:r + 8, c:c + R2],
                                      pltpu.bitcast(next(marks), v.dtype))
                            for c in range(0, v.shape[1], R2)]
                           for r in range(0, v.shape[0], 8)]) for v in vals]

    def pace16(v, after):
        return _up(pace([_pk(v)], after)[0])

    cp = pltpu.make_async_copy
    x_cp = lambda i: cp(x_h.at[:, blk(i, TC)], x_v.at[:, blk(i, TC)], sin.at[i])
    fa_cp = cp(fa_h, fa_v, sin.at[ntc])
    gm_cp = cp(gm_h, gm_v.at[:, pl.ds(0, R2)], sin.at[ntc + 1])
    zero_cp = cp(zero_h, zero_v, sin.at[ntc + 2])
    w_rows = (pl.ds(0, KF - 1), pl.ds(KF - 1, 1))
    w_cp = [cp(src.at[rows], wb_v.at[a, rows], sin.at[ntc + 12 + 2 * a + n])
            for a, src in enumerate((wr_h, wi_h)) for n, rows in enumerate(w_rows)]
    g_cp = cp(g_h, g_v, sin.at[ntc + 5])
    ffn_cp = [[cp(src.at[:, cols], w_v.at[m, :, cols], sin.at[ntc + 16 + 3 * n + m])
               for m, src in enumerate((wg_h, wu_h, wd_h))]
              for n, cols in enumerate((pl.ds(0, 2 * TF), pl.ds(2 * TF, 2 * TF),
                                        pl.ds(4 * TF, F - 4 * TF)))]
    dw_cp = lambda j: [cp(dw_v.at[j & 1, m], o.at[:, blk(j, 2 * TF)], sout.at[3 * (j & 1) + m])
                       for m, o in enumerate((dwg_h, dwu_h, dwd_h))]
    ob_v = w_v.at[0, :, pl.ds(0, S)]
    o_cp = cp(ob_v, out_h, sout.at[6])
    dwf_cp = [cp(wb_v.at[0], dwr_h, sout.at[7]), cp(wb_v.at[1], dwi_h, sout.at[8])]
    dx_cp = lambda i: cp(g_v.at[:, blk(i, TC)], dx_h.at[:, blk(i, TC)], sout.at[9 + i])

    def dft_d(y):
        out = [_dot(fa_v[c], jnp.concatenate(y[2 * c:2 * c + 2], axis=0).astype(bf16))
               for c in range(4)]
        o0 = _dot(fa_v[4, :2 * (KP - K0), :DB], y[8].astype(bf16))
        return jnp.concatenate([o[:DB] for o in out] + [o0[:KP - K0]]
                               + [o[DB:] for o in out] + [o0[KP - K0:]], axis=0)

    def idft_d(z, last):
        y = []
        for c in range(4):
            zc = jnp.concatenate([z[DB * c:DB * c + DB], z[KP + DB * c:KP + DB * c + DB]], axis=0)
            o = _dot(fa_v[5 + c], zc.astype(bf16))
            y += [o[:DB], o[DB:]]
        zc = jnp.concatenate([z[K0:KP], z[KP + K0:]], axis=0)
        y.append(_dot(fa_v[last, :DB, :2 * (KP - K0)], zc.astype(bf16)))
        return y

    def radix_fwd(r, after=None):
        re, im = blk(r, 8), blk(r + KP // 8, 8)
        a = pace([z_v[re, n * R2:(n + 1) * R2] for n in range(R1)]
                 + [z_v[im, n * R2:(n + 1) * R2] for n in range(R1)], after)
        for k, (vr, vi) in enumerate(_fft16(list(zip(a[:R1], a[R1:])), -1)):
            t_v[k, re, :R2] = vr
            t_v[k, re, R2:] = vi

    def radix_inv(r, after=None):
        re, im = blk(r, 8), blk(r + KP // 8, 8)
        a = pace([t_v[n, re, :R2] for n in range(R1)]
                 + [t_v[n, re, R2:] for n in range(R1)], after)
        for k, (vr, vi) in enumerate(_fft16(list(zip(a[:R1], a[R1:])), 1)):
            z_v[re, k * R2:(k + 1) * R2] = vr
            z_v[im, k * R2:(k + 1) * R2] = vi

    def scale():
        k = lax.broadcasted_iota(jnp.int32, (KP, R2), 0)
        return jnp.where((k == K0) | (k == K0 + 32), 1.0 / (S * D), 2.0 / (S * D))

    def filt(k1):
        rows = [pl.ds(c, n, stride=RD) for _, c, n in _CLASSES + [(K0, 0, KP - K0)]]
        return [jnp.concatenate([wp_v[a, k1, r, :] for r in rows], axis=0) for a in range(2)]

    def spectrum(mix, first=False):
        prev = None
        for k1 in range(R1 + 1):
            if k1 < R1:
                if first:
                    gm_v[k1, R2:, :R2] = -gm_v[k1, :R2, R2:]
                    gm_v[k1, R2:, R2:] = gm_v[k1, :R2, :R2]
                cur = _dot(t_v[k1].astype(bf16), gm_v[k1])
                yield cur
            if prev is not None:
                y = jnp.concatenate(mix(k1 - 1, prev[:, :R2], prev[:, R2:]), axis=1)
                o = _dot(y.astype(bf16), gm_v[k1 - 1], NT)
                t_v[k1 - 1] = o
                yield o
            prev = cur

    def mix_fwd(k1, xr, xi):
        cc = scale()
        xr, xi = xr * cc, xi * cc
        xs_v[k1, :, :R2] = _pk(xr)
        xs_v[k1, :, R2:] = _pk(xi)
        wr, wi = filt(k1)
        return [xr * wr - xi * wi, xr * wi + xi * wr]

    def mix_bwd(k1, dr, di):
        cc = scale()
        wr, wi = (w * cc for w in filt(k1))
        xr, xi = _up(xs_v[k1, :, :R2]).astype(f32), _up(xs_v[k1, :, R2:]).astype(f32)
        for a, v in enumerate((dr * xr + di * xi, di * xr - dr * xi)):
            for row, c, n in _CLASSES + [(K0, 0, 40)]:
                wp_v[a, k1, pl.ds(c, n, stride=RD), :] = v[row:row + n]
        return [dr * wr + di * wi, di * wr - dr * wi]

    def put_w(a, rr, w):
        w = _pk(w)
        tiles = _swap16(_rot16([w[:, t * R2:(t + 1) * R2] for t in range(R1)], 1))
        for k in range(R1):
            wp_v[a, k, rr, :] = _up(tiles[k]).astype(f32)

    def get_dw(a, rr):
        tiles = [_pk(wp_v[a, k, rr, :]) for k in range(R1)]
        return _up(jnp.concatenate(_rot16(_swap16(tiles), -1), axis=1))

    def pair(i):
        return blk(i, R2), blk(i + SH // R2, R2)

    def put_f(i, xa, xb, f_v):
        for r, v in enumerate(_act_forms(xa[:DH], xb[:DH], xa[DH:], xb[DH:])):
            f_v[r, :, blk(i, R2)] = _pk(v)

    def put_k(i, xa, xb, k_v, r_v):
        rows = blk(i, R2 // 2)
        f = list(_act_forms(xa[:KS].T, xb[:KS].T, xa[DH:DH + KS].T, xb[DH:DH + KS].T))
        ta, tb = [jnp.concatenate([x[KS:DH], x[DH + KS:]] * 2, axis=0).T for x in (xa, xb)]
        low = lax.broadcasted_iota(jnp.int32, (R2, R2), 1) < KA - R2
        hi = [v[:, R2:] for v in f]
        for r, v in ((1, ta), (2, -hi[3]), (3, -hi[2]), (4, tb)):
            f[r] = jnp.concatenate([f[r][:, :R2], jnp.where(low, hi[r], v)], axis=1)
        for r, v in enumerate(f):
            k_v[r, rows, :] = _pk(v)
        r_v[0, rows, :] = _pk(jnp.where(low, ta, -hi[1]))
        r_v[1, rows, :] = _pk(jnp.where(low, tb, -hi[4]))

    def grad_forms(i):
        ld = lambda after: [pace16(g_v[:, c], after).astype(f32) for c in pair(i)]
        return [lambda after: put_f(i, *ld(after), gf_v),
                lambda after: put_k(i, *ld(after), gk_v, gr_v)]

    def ffn_input(i):
        y = []

        def dots(after):
            y.extend(idft_d(jnp.concatenate([z_v[:, c] for c in pair(i)], axis=1), 9))

        def residual(half, after):
            c = pair(i)[half]
            yy = pace([v[:, half * R2:(half + 1) * R2] for v in y], after)
            h = x_v[:, c].astype(f32) + jnp.concatenate(_rfft9_t(yy), axis=0)
            h_v[:, c] = h
            mu = _colmean(h)
            st_v[2, :, c] = mu
            st_v[3, :, c] = 1.0 / jnp.sqrt(_colmean((h - mu) * (h - mu)) + EPS)

        hn = lambda after: [(pace([h_v[:, c]], after)[0] - st_v[2, :, c]) * st_v[3, :, c]
                            for c in pair(i)]
        return [dots, part(residual, 0), part(residual, 1),
                lambda after: put_f(i, *hn(after), hf_v),
                lambda after: put_k(i, *hn(after), hk_v, hr_v)]

    def ffn_output(i):
        keep, y = {}, []

        def join(acc, after):
            n = [acc[r][:, blk(i, R2)] for r in range(7)]
            n[0], n[1], n[4] = pace([n[0], n[1], n[4]], after)
            return _act_join(n)

        def out(after):
            for o, c in zip(join(acco_v, after), pair(i)):
                ob_v[:, c] = (h_v[:, c] + o).astype(bf16)

        def stats(after):
            for half, (d, c) in enumerate(zip(join(acch_v, after), pair(i))):
                hn = (pace([h_v[:, c]], after)[0] - st_v[2, :, c]) * st_v[3, :, c]
                keep[half] = (d, hn, _colmean(d), _colmean(d * hn))

        def grad(half, after):
            c = pair(i)[half]
            d, hn, m1, m2 = keep[half]
            d, hn = pace([d], after)[0], pace([hn], after)[0]
            dh = g_v[:, c].astype(f32) + st_v[3, :, c] * (d - m1 - hn * m2)
            h_v[:, c] = dh
            y.append([v.astype(bf16) for v in _rfft9(_split9(dh))])

        def dots(after):
            z = dft_d([jnp.concatenate(v, axis=1) for v in zip(*y)])
            for half, c in enumerate(pair(i)):
                z_v[:, c] = z[:, half * R2:(half + 1) * R2]

        return [out, stats, part(grad, 0), part(grad, 1), dots]

    def window(q):
        r0 = (min if isinstance(q, int) else jnp.minimum)(q * (WIN // 16), (DH - WIN) // 16)
        hint = (lambda v, n: v) if isinstance(q, int) else pl.multiple_of
        return (pl.ds(hint(r0 * 16, 16), WIN), pl.ds(hint(r0 * 16 + DH, 16), WIN),
                pl.ds(hint(r0 * 8, 8), WIN // 2))

    def mod3(j):
        return j % 3 if isinstance(j, int) else lax.rem(j, 3)

    def wprep(j, q, r, after=None):
        src = j if isinstance(j, int) else jnp.minimum(j, nj - 1)
        f1, f2 = blk(2 * src, TF), blk(2 * src + 1, TF)
        d1, d2, dst = window(q)
        for m in range(3):
            ld = lambda d, f: lambda: pace16(w_v[m, d, f], after)
            form = _wgt_forms(ld(d1, f1), ld(d1, f2), ld(d2, f1), ld(d2, f2))[r]
            ws_v[m][r][mod3(j), dst, :] = _pk(form())

    def wform(j, m, r, n):
        return _up(ws_v[m][r][mod3(j), 0:n // 2, :])

    def finalize(j, q, m, after=None):
        d1, d2, _ = window(q)
        n = [pace([m_v[m][r][j & 1, d1, :]], after if r < 4 else None)[0] for r in range(7)]
        dw_v[j & 1, m, d1, :TF] = (n[0] + n[3] - n[4] + n[6]).astype(bf16)
        dw_v[j & 1, m, d1, TF:] = (n[2] + n[4]).astype(bf16)
        dw_v[j & 1, m, d2, :TF] = (n[1] + n[3]).astype(bf16)
        dw_v[j & 1, m, d2, TF:] = (n[0] - n[1] + n[2] + n[5]).astype(bf16)

    def stage1(t, b, ms):
        j, ss = t >> 2, blk(t & 3, TS // 2)
        f1, f2 = blk(2 * j, TF), blk(2 * j + 1, TF)
        rows = part(jnp.concatenate, axis=0)
        zero = jnp.zeros((KS - KA, TF), bf16)
        for m in ms:
            k_v, r_v = (gk_v, gr_v) if m == 2 else (hk_v, hr_v)
            v1, v2 = [[w_v[m, KS:DH, f], w_v[m, DH + KS:, f]] for f in (f1, f2)]
            w12, w21 = w_v[m, KA:KS, f2], w_v[m, DH + KA:DH + KS, f1]
            q = lambda r, tail: _dot(_up(k_v[r, ss, :]), rows([wform(j, m, r, KA)] + tail))
            mid = lambda r: [_up(ws_v[m][r][mod3(j), KA // 2:KS // 2, :])]
            q2 = q(2, mid(2))
            yield q2
            q5 = q(5, [w21])
            yield q5
            a7, w7 = _up(k_v[0, ss, R2:]), rows([zero, w12 + w21])
            if m == ms[-1] and len(ms) % 2:
                q7 = rows([_dot(a7[:TS // 2], w7), _dot(a7[TS // 2:], w7)])
            else:
                q7 = _dot(a7, w7)
            raw_v[b][m, 1] = q2 + q5 + q7 + _dot(_up(r_v[0, ss, :]), rows(v2 + mid(1)))
            q3 = q(3, mid(3))
            yield q3
            q6 = q(6, [w12])
            yield q6
            raw_v[b][m, 2] = q3 + q7 + q6 + _dot(_up(r_v[1, ss, :]), rows(v1 + mid(4)))
            q0 = q(0, [zero])
            yield q0
            q1 = q(1, v1)
            raw_v[b][m, 0] = (q0 + q5 - q3) + q1
            yield q1
            q4 = q(4, v2)
            raw_v[b][m, 3] = (q0 - q2 + q6) + q4
            yield q4

    def gate(b, r0, after):
        rows, prows = slice(r0, r0 + EW), slice(r0 // 2, (r0 + EW) // 2)
        res = ([], [], [])
        pre = pace([raw_v[b][0, q, rows] for q in range(4)], after)
        for q in range(4):
            a, u, dp = pre[q], raw_v[b][1, q, rows], raw_v[b][2, q, rows]
            sg = jax.nn.sigmoid(a)
            sl = a * sg
            res[0].append(dp * u * (sg + sl * (1.0 - sg)))
            res[1].append(dp * sl)
            res[2].append(sl * u)
        for m in range(3):
            for r, v in enumerate(_hid_forms(*res[m])):
                p_v[b][m, r, prows, :] = _pk(v)

    gates = lambda b: [part(gate, b, r0) for r0 in range(0, TS, EW)]

    def stage2(t, b, acts=True, wgts=True):
        j, i = t >> 2, t & 3
        ss = blk(i, TS)
        for r in range(7):
            if acts:
                o = _dot(wform(j, 2, r, DH), _up(p_v[b][2, r]), NT)
                acco_v[r][:, ss] = jnp.where(j == 0, 0.0, acco_v[r][:, ss]) + o
                yield o
                o = (_dot(wform(j, 0, r, DH), _up(p_v[b][0, r]), NT)
                     + _dot(wform(j, 1, r, DH), _up(p_v[b][1, r]), NT))
                acch_v[r][:, ss] = jnp.where(j == 0, 0.0, acch_v[r][:, ss]) + o
                yield o
            if wgts:
                for m, f_v in enumerate((hf_v, hf_v, gf_v)):
                    o = _dot(_up(f_v[r, :, ss]), _up(p_v[b][m, r]))
                    m_v[m][r][j & 1] = jnp.where(i == 0, 0.0, m_v[m][r][j & 1]) + o
                    yield o

    fins = lambda j, q: [part(finalize, j, q, m) for m in range(3)]
    preps = lambda j, q: [part(wprep, j, q, r) for r in range(7)]
    cat = lambda lists: list(chain(*lists))

    x_cp(0).start()
    fa_cp.start()
    for i in range(1, ntc):
        x_cp(i).start()
    for c in w_cp + [zero_cp]:
        c.start()
    for a in range(2):
        for k in range(R1):
            wp_v[a, k, pl.ds(RD * 34, KP - K0 - 34, stride=RD), :] = jnp.zeros(
                (KP - K0 - 34, R2), f32)
    fa_cp.wait()

    def p1(i):
        c = blk(i, TC)
        y = _rfft9(_split9(x_v[:, c].astype(f32)))
        mu = _colmean(y[8])
        y[8] = y[8] - RD * mu
        sq = [v * v for v in y]
        en = (sq[8] + 1.5 * sq[5]
              + 2.0 * (sq[0] + sq[1] + sq[2] + sq[3] + sq[4] + sq[6] + sq[7]))
        rstd = 1.0 / jnp.sqrt(_colmean(en) * (1.0 / RD) + EPS)
        st_v[0, :, c] = mu
        st_v[1, :, c] = rstd
        z_v[:, c] = dft_d(y) * rstd

    def p1s(n):
        for i in range(UN):
            x_cp(UN * n + i).wait()
        for i in range(UN):
            p1(UN * n + i)
    loop("p1", ntc // UN, p1s)

    for c in w_cp:
        c.wait()
    gm_cp.start()

    def pw(r):
        pl.when(r == 5)(g_cp.start)
        for a in range(2):
            put_w(a, blk(r, 32), wb_v[a, blk(r, 32), :])
            radix_fwd(4 * r + 2 * a)
            radix_fwd(4 * r + 2 * a + 1)
    loop("pw", (KF - 1) // 32, pw)
    row = lax.broadcasted_iota(jnp.int32, (16, S), 0)
    for a in range(2):
        last = jnp.broadcast_to(wb_v[a, KF - 1:KF, :].astype(f32), (16, S))
        put_w(a, slice(KF - 1, KP), jnp.where(row == 0, last, 0.0))
        radix_fwd((KF - 1) // 8 + a)

    for c in (zero_cp, gm_cp):
        c.wait()

    def fetch(after):
        g_cp.wait()
        for c in ffn_cp[0]:
            c.start()
    with jax.named_scope("p3"):
        _overlap(spectrum(mix_fwd, True),
                 ([fetch] + cat(grad_forms(i) for i in range(7)), 5, 31))
    loop("radix", KP // 16, lambda r: (radix_inv(2 * r), radix_inv(2 * r + 1)))
    for c in ffn_cp[0]:
        c.wait()
    for c in ffn_cp[1] + ffn_cp[2]:
        c.start()
    loop("wprep0", ni, lambda q: [step() for step in preps(0, q)])

    with jax.named_scope("head"):
        _overlap(chain(stage1(0, 0, (2,)), stage1(1, 1, (2,))),
                 (cat(ffn_input(i) for i in (0, 1)), 0, 12))
        _overlap(stage1(0, 0, (0, 1)), (cat(ffn_input(i) for i in (2, 3)), 0, 13))
        for c in ffn_cp[1]:
            c.wait()
        _overlap(stage1(1, 1, (0, 1)), (gates(0), 0, 12),
                 (preps(1, 0) + preps(1, 1), 0, 13))

    def step(t, b, *tasks):
        if not tasks:
            tasks = ((fins(((t - 1) >> 2) + 1, (t - 1) & 3), 49, 55),
                     (preps(((t + 1) >> 2) + 1, (t + 1) & 3), 35, 48))
        _overlap(chain(stage2(t - 1, 1 - b), stage1(t + 1, 1 - b, (0, 1, 2))),
                 (gates(b), 1, 32), *tasks)

    with jax.named_scope("head2"):
        step(1, 1, (ffn_input(4) + ffn_input(5), 1, 28),
             (ffn_input(6) + ffn_input(7) + preps(1, 2) + grad_forms(7), 30, 54))
    for c in ffn_cp[2]:
        c.wait()

    def body(n):
        j = n >> 1

        @pl.when(((n & 1) == 0) & (j >= 3))
        def _():
            for c in dw_cp(j - 3):
                c.wait()

        @pl.when(((n & 1) == 1) & (j >= 2))
        def _():
            for c in dw_cp(j - 2):
                c.start()
        step(2 * n, 0)
        step(2 * n + 1, 1)
    loop("ffn", nt // 2 - 1, body, 1)
    for c in dw_cp(nj - 3):
        c.start()

    with jax.named_scope("tail"):
        step(nt - 2, 0, (ffn_output(0), 1, 30), (ffn_output(1) + fins(nj - 2, 1), 33, 54))
        _overlap(stage2(nt - 2, 0), (gates(1), 1, 32),
                 (cat(ffn_output(i) for i in (2, 3)), 0, 32), (fins(nj - 2, 2), 29, 34))
        _overlap(stage2(nt - 1, 1, wgts=False), (cat(ffn_output(i) for i in (4, 5)), 0, 13),
                 (fins(nj - 2, 3), 0, 13))
        _overlap(stage2(nt - 1, 1, acts=False), (cat(ffn_output(i) for i in (6, 7)), 0, 10),
                 ([part(radix_fwd, r) for r in range(KP // 8)], 12, 20))
    for c in dw_cp(nj - 2) + [o_cp]:
        c.start()
    for c in dw_cp(nj - 3):
        c.wait()

    with jax.named_scope("p9"):
        _overlap(spectrum(mix_bwd), (cat(fins(nj - 1, q) for q in range(ni)), 0, 31))
    for c in dw_cp(nj - 1):
        c.start()

    def pdw(r):
        for a in range(2):
            wb_v[a, blk(r, 32), :] = get_dw(a, blk(r, 32))
            radix_inv(4 * r + 2 * a)
            radix_inv(4 * r + 2 * a + 1)
    loop("pdw", (KF - 1) // 32, pdw)
    for a in range(2):
        wb_v[a, KF - 1:KF, :] = get_dw(a, slice(KF - 1, KP)).astype(f32)[0:1].astype(bf16)
        radix_inv((KF - 1) // 8 + a)
    for c in dwf_cp:
        c.start()

    def p11(i):
        c = blk(i, R2)
        dxn = jnp.concatenate(_rfft9_t(idft_d(z_v[:, c], 10)), axis=0)
        rstd = st_v[1, :, c]
        xc = x_v[:, c].astype(f32) - st_v[0, :, c]
        proj = _colmean(dxn * xc) * (rstd * rstd)
        g_v[:, c] = (h_v[:, c] + rstd * (dxn - xc * proj)).astype(bf16)

    def p11s(n):
        for i in range(UN * TC // R2):
            p11(UN * TC // R2 * n + i)
        for i in range(UN):
            dx_cp(UN * n + i).start()
    loop("p11", ntc // UN, p11s)

    for c in dw_cp(nj - 2) + dw_cp(nj - 1) + [o_cp] + dwf_cp + [dx_cp(i) for i in range(ntc)]:
        c.wait()


@jax.jit
def pallas_sequential_preLN__spectral_gfnet__swiglu_ffn__prompt_kernel(
    A_x: jax.Array,
    A_w_r: jax.Array,
    A_w_i: jax.Array,
    B_x: jax.Array,
    B_w_gate: jax.Array,
    B_w_up: jax.Array,
    B_w_down: jax.Array,
    grad_out: jax.Array,
):
    del B_x
    sds = jax.ShapeDtypeStruct
    hbm = pl.BlockSpec(memory_space=pltpu.HBM)
    out, dx, dwr, dwi, dwg, dwu, dwd = pl.pallas_call(
        _kernel,
        out_shape=[sds((D, S), bf16), sds((D, S), bf16),
                   sds((KF, S), bf16), sds((KF, S), bf16),
                   sds((D, F), bf16), sds((D, F), bf16), sds((D, F), bf16)],
        in_specs=[hbm] * 10,
        out_specs=[hbm] * 7,
        scratch_shapes=[
            V((D, S), bf16), V((D, S), bf16), V((2, KF, S), bf16), V((3, D, F), bf16),
            V((11, R2, R2), bf16), V((R1, 2 * R2, 2 * R2), bf16),
            V((8, R2), jnp.int32),
            V((2 * KP, S), f32), V((R1, KP, 2 * R2), f32),
            V((2, R1, RD * (KP - K0), R2), f32), V((R1, KP // 2, 2 * R2), u32),
            V((4, 1, S), f32), V((D, S), f32),
            V((7, DH // 2, SH), u32), V((7, DH // 2, SH), u32),
            V((7, SH // 2, KS), u32), V((7, SH // 2, KS), u32),
            V((2, SH // 2, R2), u32), V((2, SH // 2, R2), u32),
            [[V((3, DH // 2, TF), u32)] * 7] * 3, [V((3, 4, TS, TF), f32)] * 2,
            [V((3, 7, TS // 2, TF), u32)] * 2,
            [V((DH, SH), f32)] * 7, [V((DH, SH), f32)] * 7, [[V((2, DH, TF), f32)] * 7] * 3,
            V((2, 3, D, 2 * TF), bf16),
            pltpu.SemaphoreType.DMA((S // TC + 25,)),
            pltpu.SemaphoreType.DMA((9 + S // TC,)),
        ],
        compiler_params=pltpu.CompilerParams(vmem_limit_bytes=127 * 2**20),
    )(A_x[0].T, A_w_r.T, A_w_i.T, B_w_gate, B_w_up, B_w_down.T, grad_out[0].T,
      _FA, _G, _ZERO)
    return out.T[None], dx.T[None], dwr.T, dwi.T, dwg, dwu, dwd.T
```

```python
import functools
import itertools
import math

import jax
import jax.numpy as jnp
import ml_dtypes
import numpy as np
from jax import lax
from jax.experimental import pallas as pl
from jax.experimental.pallas import tpu as pltpu

S, D, F = 2048, 576, 4608
KF = D // 2 + 1
KP = 304
R1, R2 = 16, 128
RD, DB = 9, 64
K0 = 256
EPS = 1e-5
DH, SH = D // 2, S // 2
KA, KS = 192, 256
TS = 256
TF = 256
UN = 2
EW = 16
WIN = 80
TC = 256

bf16 = jnp.bfloat16
f32 = jnp.float32
u32 = jnp.uint32
V = pltpu.VMEM
NN = (((1,), (0,)), ((), ()))
NT = (((1,), (1,)), ((), ()))


_C1, _C2, _C4 = (math.cos(2 * math.pi * e / RD) for e in (1, 2, 4))
_S1, _S2, _S3, _S4 = (math.sin(2 * math.pi * e / RD) for e in (1, 2, 3, 4))


def _cyc(m, a, b, c, k1, k2, k3):
    e1, e2 = a - c, b - c
    p, q = k1 * e1 + k2 * e2, k2 * e1 + k3 * e2
    return m + p, m + q, m - (p + q)


def _cyc_t(o1, o2, o3, k1, k2, k3):
    p, q = o1 - o3, o2 - o3
    e1, e2 = k1 * p + k2 * q, k2 * p + k3 * q
    return o1 + o2 + o3, e1, e2, -(e1 + e2)


def _rfft9(x):
    s1, s2, s3, s4 = (x[a] + x[RD - a] for a in (1, 2, 3, 4))
    t1, t2, t3, t4 = x[1] - x[8], x[7] - x[2], x[3] - x[6], x[4] - x[5]
    u, v = x[0] + s3, s1 + s2 + s4
    p1, p2, p4 = _cyc(x[0] - 0.5 * s3, s1, s2, s4, _C1, _C2, _C4)
    q1, q2, q4 = _cyc(_S3 * t3, t1, t2, t4, _S1, -_S2, _S4)
    return [p1, q1, p2, q2, u - 0.5 * v, t1 + t2 + t4, p4, q4, u + v]


def _rfft9_t(y):
    p1, q1, p2, q2, p3, q3, p4, q4, y0 = y
    m, s1, s2, s4 = _cyc_t(p1, p2, p4, _C1, _C2, _C4)
    n, t1, t2, t4 = _cyc_t(q1, q2, q4, _S1, -_S2, _S4)
    u, v = y0 + p3, y0 - 0.5 * p3
    s1, s2, s4, s3 = s1 + v, s2 + v, s4 + v, u - 0.5 * m
    t1, t2, t4, t3 = t1 + q3, t2 + q3, t4 + q3, _S3 * n
    return [u + m, s1 + t1, s2 - t2, s3 + t3, s4 + t4, s4 - t4, s3 - t3, s2 + t2, s1 - t1]


_CLASSES = [(64 * (c - 1) + 32 * h, (c, RD - c)[h], 32) for c in (1, 2, 3, 4) for h in (0, 1)]


def _consts():
    root = lambda e, n: np.exp(-2j * np.pi * (e % n) / n)
    bins = np.full(KP, -1)
    for row, c, n in _CLASSES + [(K0, 0, 33)]:
        bins[row:row + n] = c + RD * np.arange(n)
    r9 = np.stack(_rfft9(list(np.eye(RD))))
    r9 = r9 / (r9 * r9).sum(1, keepdims=True)
    coef = (root(bins[:, None, None] * np.arange(RD), RD) * r9).sum(-1)
    full = coef[:, :, None] * root(bins[:, None, None] * np.arange(DB), D)
    full = full.reshape(KP, D) * (bins >= 0)[:, None]
    fa = np.zeros((11, R2, R2))
    for c in range(5):
        blk = full[DB * c:min(DB * c + DB, KP), R2 * c:R2 * c + R2]
        fa[c, :2 * blk.shape[0], :blk.shape[1]] = np.concatenate([blk.real, blk.imag])
        fa[5 + c] = fa[c].T
    fa[10] = fa[9]
    fa[10, :, 0] = 0.0
    k1 = np.arange(R1)[:, None, None]
    lane = (np.arange(R2) - k1) % R2
    k2 = 8 * (lane % 16) + lane // 16
    g = root(np.arange(R2)[:, None] * (k1 + R1 * k2), S)
    g = np.stack([g.real, g.real + g.imag, g.imag - g.real], 1)
    cast = lambda a: (np.round(a, 9) + 0.0).astype(np.float32).astype(ml_dtypes.bfloat16)
    return cast(fa), cast(g)


_FA, _G = _consts()


def _dot(a, b, dn=NN):
    return lax.dot_general(a, b, dn, preferred_element_type=f32)


def _fft4(x, sign):
    (ar, ai), (br, bi), (cr, ci), (dr, di) = x
    s0r, s0i, d0r, d0i = ar + cr, ai + ci, ar - cr, ai - ci
    s1r, s1i, d1r, d1i = br + dr, bi + di, br - dr, bi - di
    lo = (d0r + d1i, d0i - d1r)
    hi = (d0r - d1i, d0i + d1r)
    o1, o3 = (lo, hi) if sign < 0 else (hi, lo)
    return [(s0r + s1r, s0i + s1i), o1, (s0r - s1r, s0i - s1i), o3]


def _tw16(v, e, sign):
    r, i = v
    e %= 16
    if e == 0:
        return v
    if e == 4:
        return (i, -r) if sign < 0 else (-i, r)
    c = math.cos(2 * math.pi * e / 16)
    s = sign * math.sin(2 * math.pi * e / 16)
    if e % 2 == 0:
        if c * s > 0:
            return ((r - i) * c, (r + i) * c)
        return ((r + i) * c, (i - r) * c)
    return (r * c - i * s, r * s + i * c)


def _fft16(x, sign):
    cols = [_fft4([x[4 * a + b] for a in range(4)], sign) for b in range(4)]
    out = [None] * 16
    for p in range(4):
        o = _fft4([_tw16(cols[b][p], b * p, sign) for b in range(4)], sign)
        for q in range(4):
            out[p + 4 * q] = o[q]
    return out


def _swap16(tiles):
    lane = lax.broadcasted_iota(jnp.int32, tiles[0].shape, 1)
    tiles = list(tiles)
    for d in (1, 2, 4, 8):
        for lo in range(d):
            low = ((lane - lo) & d) == 0
            for t in range(lo, R1, 2 * d):
                a, b = tiles[t], tiles[t + d]
                tiles[t], tiles[t + d] = jnp.where(low, a, b), jnp.where(low, b, a)
    return tiles


def _rot16(tiles, sign):
    return [pltpu.roll(v, (sign * t) % R2, 1) if t else v for t, v in enumerate(tiles)]


def _act_forms(a11, a12, a21, a22):
    return (a11 + a22, a21 + a22, a11, a22, a11 + a12, a21 - a11, a12 - a22)


def _hid_forms(p11, p12, p21, p22):
    return (p11 + p22, p11, p12 - p22, p21 - p11, p22, p11 + p12, p21 + p22)


def _wgt_forms(w11, w12, w21, w22):
    return (lambda: w11() + w22(), lambda: w21() - w22(), lambda: w12() + w22(),
            lambda: w11() + w21(), lambda: w12() - w11(), w22, w11)


def _act_join(n):
    return (jnp.concatenate([n[0] + n[2] + n[4] - n[5], n[1] + n[5]], axis=0),
            jnp.concatenate([n[4] + n[6], n[0] + n[1] + n[3] - n[6]], axis=0))


def _pk(v):
    return pltpu.bitcast(v.astype(bf16), u32)


def _up(v):
    return pltpu.bitcast(v, bf16)


def _colmean(x):
    return jnp.sum(x, axis=0, keepdims=True) * (1.0 / D)


def _overlap(dots, *tasks):
    plan = [(first + s * (last - first + 1) // len(steps),
             -(-(last - first + 1) // len(steps)), step)
            for steps, first, last in tasks for s, step in enumerate(steps)]
    seen = []
    for k, o in enumerate(dots):
        seen.append(o)
        for at, span, step in plan:
            if at == k:
                step(seen[-span:])
    assert all(at < len(seen) for at, _, _ in plan)


def _kernel(x_h, wr_h, wi_h, wg_h, wu_h, wd_h, g_h, fa_h, gm_h,
            out_h, dx_h, dwr_h, dwi_h, dwg_h, dwu_h, dwd_h,
            x_v, g_v, wb_v, w_v, fa_v, gm_v,
            z_v, t_v, wp_v, xs_v, st_v, h_v, hf_v, gf_v, hk_v, gk_v, hr_v, gr_v,
            ws_v, raw_v, p_v, acco_v, acch_v, m_v, dw_v, sin, sout):
    ntc = S // TC
    nj = F // (2 * TF)
    ni = SH // TS
    nt = nj * ni
    assert ni == 4 and nt % 2 == 0
    part, chain = functools.partial, itertools.chain

    def loop(name, n, body, lo=0):
        with jax.named_scope(name):
            lax.fori_loop(lo, n, lambda i, carry: (body(i), carry)[1], 0)

    def blk(i, n):
        return pl.ds(i * n, n) if isinstance(i, int) else pl.ds(pl.multiple_of(i * n, n), n)

    def pace(vals, after):
        if not after:
            return vals
        keep = _pk(fa_v[4, R2 - 16:, :]) == 0
        marks = [o[r:r + 8, :R2] for o in after for r in range(0, o.shape[0], 8)]
        n = sum(v.size for v in vals) // (8 * R2)
        marks = iter([marks[i * len(marks) // n] for i in range(n)])
        return [jnp.block([[jnp.where(keep, v[r:r + 8, c:c + R2],
                                      pltpu.bitcast(next(marks), v.dtype))
                            for c in range(0, v.shape[1], R2)]
                           for r in range(0, v.shape[0], 8)]) for v in vals]

    def pace16(v, after):
        return _up(pace([_pk(v)], after)[0])

    cp = pltpu.make_async_copy
    x_cp = lambda i: cp(x_h.at[:, blk(i, TC)], x_v.at[:, blk(i, TC)], sin.at[i])
    fa_cp = cp(fa_h, fa_v, sin.at[ntc])
    gm_cp = cp(gm_h, gm_v, sin.at[ntc + 1])
    g_cp = cp(g_h, g_v, sin.at[ntc + 2])
    w_cp = [cp(src.at[rows], wb_v.at[a, rows], sin.at[ntc + 3 + 2 * a + n])
            for a, src in enumerate((wr_h, wi_h))
            for n, rows in enumerate((pl.ds(0, KF - 1), pl.ds(KF - 1, 1)))]
    ffn_cp = [[cp(src.at[:, cols], w_v.at[m, :, cols], sin.at[ntc + 7 + 3 * n + m])
               for m, src in enumerate((wg_h, wu_h, wd_h))]
              for n, cols in enumerate((pl.ds(0, 2 * TF), pl.ds(2 * TF, 2 * TF),
                                        pl.ds(4 * TF, F - 4 * TF)))]
    dw_cp = lambda j: [cp(dw_v.at[j & 1, m], o.at[:, blk(j, 2 * TF)], sout.at[3 * (j & 1) + m])
                       for m, o in enumerate((dwg_h, dwu_h, dwd_h))]
    ob_v = w_v.at[0, :, pl.ds(0, S)]
    o_cp = [cp(w_v.at[0, :, blk(q, SH // 2)], out_h.at[:, blk(q, SH // 2)], sout.at[6 + q])
            for q in range(4)]
    dwf_cp = lambda rows, n: [cp(wb_v.at[a, rows], o.at[rows], sout.at[10 + ntc + 2 * n + a])
                              for a, o in enumerate((dwr_h, dwi_h))]
    dx_cp = lambda i: cp(g_v.at[:, blk(i, TC)], dx_h.at[:, blk(i, TC)], sout.at[10 + i])

    def dft_d(y):
        out = [_dot(fa_v[c], jnp.concatenate(y[2 * c:2 * c + 2], axis=0).astype(bf16))
               for c in range(4)]
        o0 = _dot(fa_v[4, :2 * (KP - K0), :DB], y[8].astype(bf16))
        return jnp.concatenate([o[:DB] for o in out] + [o0[:KP - K0]]
                               + [o[DB:] for o in out] + [o0[KP - K0:]], axis=0)

    def idft_d(z, last):
        y = []
        for c in range(4):
            zc = jnp.concatenate([z[DB * c:DB * c + DB], z[KP + DB * c:KP + DB * c + DB]], axis=0)
            o = _dot(fa_v[5 + c], zc.astype(bf16))
            y += [o[:DB], o[DB:]]
        zc = jnp.concatenate([z[K0:KP], z[KP + K0:]], axis=0)
        y.append(_dot(fa_v[last, :DB, :2 * (KP - K0)], zc.astype(bf16)))
        return y

    def radix_fwd(r, after=None):
        re, im = blk(r, 8), blk(r + KP // 8, 8)
        a = pace([z_v[re, n * R2:(n + 1) * R2] for n in range(R1)]
                 + [z_v[im, n * R2:(n + 1) * R2] for n in range(R1)], after)
        for k, (vr, vi) in enumerate(_fft16(list(zip(a[:R1], a[R1:])), -1)):
            t_v[k, re, :R2] = vr
            t_v[k, re, R2:] = vi

    def radix_inv(r, after=None):
        re, im = blk(r, 8), blk(r + KP // 8, 8)
        a = pace([t_v[n, re, :R2] for n in range(R1)]
                 + [t_v[n, re, R2:] for n in range(R1)], after)
        for k, (vr, vi) in enumerate(_fft16(list(zip(a[:R1], a[R1:])), 1)):
            z_v[re, k * R2:(k + 1) * R2] = vr
            z_v[im, k * R2:(k + 1) * R2] = vi

    def scale():
        k = lax.broadcasted_iota(jnp.int32, (KP, R2), 0)
        return jnp.where((k == K0) | (k == K0 + 32), 1.0 / (S * D), 2.0 / (S * D))

    def filt(k1):
        rows = [pl.ds(c, n, stride=RD) for _, c, n in _CLASSES + [(K0, 0, KP - K0)]]
        return [jnp.concatenate([wp_v[a, k1, r, :] for r in rows], axis=0) for a in range(2)]

    def spectrum(mix):
        prev = None
        for k1 in range(R1 + 1):
            if k1 < R1:
                a, b = t_v[k1, :, :R2], t_v[k1, :, R2:]
                n = [_dot(v.astype(bf16), gm_v[k1, e]) for e, v in enumerate((a + b, b, a))]
                cur = (n[0] - n[1], n[0] + n[2])
                yield n[2]
            if prev is not None:
                a, b = mix(k1 - 1, *prev)
                n = [_dot(v.astype(bf16), gm_v[k1 - 1, e], NT)
                     for e, v in enumerate((a + b, a, b))]
                t_v[k1 - 1, :, :R2] = n[0] + n[2]
                t_v[k1 - 1, :, R2:] = n[0] - n[1]
                yield n[2]
            prev = cur

    def mix_fwd(k1, xr, xi):
        cc = scale()
        xr, xi = xr * cc, xi * cc
        xs_v[k1, :, :R2] = _pk(xr)
        xs_v[k1, :, R2:] = _pk(xi)
        wr, wi = filt(k1)
        return [xr * wr - xi * wi, xr * wi + xi * wr]

    def mix_bwd(k1, dr, di):
        cc = scale()
        wr, wi = (w * cc for w in filt(k1))
        xr, xi = _up(xs_v[k1, :, :R2]).astype(f32), _up(xs_v[k1, :, R2:]).astype(f32)
        for a, v in enumerate((dr * xr + di * xi, di * xr - dr * xi)):
            for row, c, n in _CLASSES + [(K0, 0, 40)]:
                wp_v[a, k1, pl.ds(c, n, stride=RD), :] = v[row:row + n]
        return [dr * wr + di * wi, di * wr - dr * wi]

    def put_w(a, rr, w):
        w = _pk(w)
        tiles = _swap16(_rot16([w[:, t * R2:(t + 1) * R2] for t in range(R1)], 1))
        for k in range(R1):
            wp_v[a, k, rr, :] = _up(tiles[k]).astype(f32)

    def get_dw(a, rr):
        tiles = [_pk(wp_v[a, k, rr, :]) for k in range(R1)]
        return _up(jnp.concatenate(_rot16(_swap16(tiles), -1), axis=1))

    def pair(i):
        return blk(i, R2), blk(i + SH // R2, R2)

    def put_f(i, xa, xb, f_v):
        for r, v in enumerate(_act_forms(xa[:DH], xb[:DH], xa[DH:], xb[DH:])):
            f_v[r, :, blk(i, R2)] = _pk(v)

    def put_k(i, xa, xb, k_v, r_v):
        rows = blk(i, R2 // 2)
        f = list(_act_forms(xa[:KS].T, xb[:KS].T, xa[DH:DH + KS].T, xb[DH:DH + KS].T))
        ta, tb = [jnp.concatenate([x[KS:DH], x[DH + KS:]] * 2, axis=0).T for x in (xa, xb)]
        low = lax.broadcasted_iota(jnp.int32, (R2, R2), 1) < KA - R2
        hi = [v[:, R2:] for v in f]
        for r, v in ((1, ta), (2, -hi[3]), (3, -hi[2]), (4, tb)):
            f[r] = jnp.concatenate([f[r][:, :R2], jnp.where(low, hi[r], v)], axis=1)
        for r, v in enumerate(f):
            k_v[r, rows, :] = _pk(v)
        r_v[0, rows, :] = _pk(jnp.where(low, ta, -hi[1]))
        r_v[1, rows, :] = _pk(jnp.where(low, tb, -hi[4]))

    def grad_forms(i):
        ld = lambda after: [pace16(g_v[:, c], after).astype(f32) for c in pair(i)]
        return [lambda after: put_f(i, *ld(after), gf_v),
                lambda after: put_k(i, *ld(after), gk_v, gr_v)]

    def ffn_input(i):
        y = []

        def dots(after):
            y.extend(idft_d(jnp.concatenate([z_v[:, c] for c in pair(i)], axis=1), 9))

        def residual(half, after):
            c = pair(i)[half]
            groups = range(0, DB, 16)
            yy = pace([v[b:b + 16, half * R2:(half + 1) * R2] for b in groups for v in y], after)
            hs, mu, var = [], 0.0, 0.0
            for n, b in enumerate(groups):
                for a, d in enumerate(_rfft9_t(yy[RD * n:RD * n + RD])):
                    rows = slice(a * DB + b, a * DB + b + 16)
                    hs.append(x_v[rows, c].astype(f32) + d)
                    h_v[rows, c] = hs[-1]
                    mu = mu + hs[-1]
            mu = _colmean(mu)
            for h in hs:
                var = var + (h - mu) * (h - mu)
            st_v[2, :, c] = mu
            st_v[3, :, c] = 1.0 / jnp.sqrt(_colmean(var) + EPS)

        hn = lambda after: [(pace([h_v[:, c]], after)[0] - st_v[2, :, c]) * st_v[3, :, c]
                            for c in pair(i)]
        return [dots, part(residual, 0), part(residual, 1),
                lambda after: put_f(i, *hn(after), hf_v),
                lambda after: put_k(i, *hn(after), hk_v, hr_v)]

    def ffn_output(i):
        keep, y = {}, []

        def join(acc, after):
            n = [acc[r][:, blk(i, R2)] for r in range(7)]
            n[0], n[1], n[4] = pace([n[0], n[1], n[4]], after)
            return _act_join(n)

        def out(after):
            for o, c in zip(join(acco_v, after), pair(i)):
                ob_v[:, c] = (h_v[:, c] + o).astype(bf16)

        def stats(after):
            for half, (d, c) in enumerate(zip(join(acch_v, after), pair(i))):
                hn = (pace([h_v[:, c]], after)[0] - st_v[2, :, c]) * st_v[3, :, c]
                keep[half] = (d, hn, _colmean(d), _colmean(d * hn))

        def grad(half, after):
            c = pair(i)[half]
            d, hn, m1, m2 = keep[half]
            rows = [slice(a * DB + b, a * DB + b + 16) for b in range(0, DB, 16) for a in range(RD)]
            d, hn = pace([d[r] for r in rows], after), pace([hn[r] for r in rows], after)
            rstd, ys = st_v[3, :, c], []
            for n in range(0, len(rows), RD):
                dh = [g_v[rows[k], c].astype(f32) + rstd * (d[k] - m1 - hn[k] * m2)
                      for k in range(n, n + RD)]
                for r, v in zip(rows[n:n + RD], dh):
                    h_v[r, c] = v
                ys.append([v.astype(bf16) for v in _rfft9(dh)])
            y.append([jnp.concatenate(v, axis=0) for v in zip(*ys)])

        def dots(after):
            z = dft_d([jnp.concatenate(v, axis=1) for v in zip(*y)])
            for half, c in enumerate(pair(i)):
                z_v[:, c] = z[:, half * R2:(half + 1) * R2]

        return [out, stats, part(grad, 0), part(grad, 1), dots]

    def window(q):
        r0 = (min if isinstance(q, int) else jnp.minimum)(q * (WIN // 16), (DH - WIN) // 16)
        hint = (lambda v, n: v) if isinstance(q, int) else pl.multiple_of
        return (pl.ds(hint(r0 * 16, 16), WIN), pl.ds(hint(r0 * 16 + DH, 16), WIN),
                pl.ds(hint(r0 * 8, 8), WIN // 2))

    def mod3(j):
        return j % 3 if isinstance(j, int) else lax.rem(j, 3)

    def wprep(j, q, r, after=None):
        src = j if isinstance(j, int) else jnp.minimum(j, nj - 1)
        f1, f2 = blk(2 * src, TF), blk(2 * src + 1, TF)
        d1, d2, dst = window(q)
        for m in range(3):
            ld = lambda d, f: lambda: pace16(w_v[m, d, f], after)
            form = _wgt_forms(ld(d1, f1), ld(d1, f2), ld(d2, f1), ld(d2, f2))[r]
            ws_v[m][r][mod3(j), dst, :] = _pk(form())

    def wform(j, m, r, n):
        return _up(ws_v[m][r][mod3(j), 0:n // 2, :])

    def finalize(j, q, m, after=None):
        d1, d2, _ = window(q)
        n = [pace([m_v[m][r][j & 1, d1, :]], after if r < 4 else None)[0] for r in range(7)]
        dw_v[j & 1, m, d1, :TF] = (n[0] + n[3] - n[4] + n[6]).astype(bf16)
        dw_v[j & 1, m, d1, TF:] = (n[2] + n[4]).astype(bf16)
        dw_v[j & 1, m, d2, :TF] = (n[1] + n[3]).astype(bf16)
        dw_v[j & 1, m, d2, TF:] = (n[0] - n[1] + n[2] + n[5]).astype(bf16)

    def stage1(t, b, ms):
        j, ss = t >> 2, blk(t & 3, TS // 2)
        f1, f2 = blk(2 * j, TF), blk(2 * j + 1, TF)
        rows = part(jnp.concatenate, axis=0)
        zero = jnp.zeros((KS - KA, TF), bf16)
        for m in ms:
            k_v, r_v = (gk_v, gr_v) if m == 2 else (hk_v, hr_v)
            v1, v2 = [[w_v[m, KS:DH, f], w_v[m, DH + KS:, f]] for f in (f1, f2)]
            w12, w21 = w_v[m, KA:KS, f2], w_v[m, DH + KA:DH + KS, f1]
            q = lambda r, tail: _dot(_up(k_v[r, ss, :]), rows([wform(j, m, r, KA)] + tail))
            mid = lambda r: [_up(ws_v[m][r][mod3(j), KA // 2:KS // 2, :])]
            q2 = q(2, mid(2))
            yield q2
            q5 = q(5, [w21])
            yield q5
            a7, w7 = _up(k_v[0, ss, R2:]), rows([zero, w12 + w21])
            if m == ms[-1] and len(ms) % 2:
                q7 = rows([_dot(a7[:TS // 2], w7), _dot(a7[TS // 2:], w7)])
            else:
                q7 = _dot(a7, w7)
            raw_v[b][m, 1] = q2 + q5 + q7 + _dot(_up(r_v[0, ss, :]), rows(v2 + mid(1)))
            q3 = q(3, mid(3))
            yield q3
            q6 = q(6, [w12])
            yield q6
            raw_v[b][m, 2] = q3 + q7 + q6 + _dot(_up(r_v[1, ss, :]), rows(v1 + mid(4)))
            q0 = q(0, [zero])
            yield q0
            q1 = q(1, v1)
            raw_v[b][m, 0] = (q0 + q5 - q3) + q1
            yield q1
            q4 = q(4, v2)
            raw_v[b][m, 3] = (q0 - q2 + q6) + q4
            yield q4

    def gate(b, r0, after):
        rows, prows = slice(r0, r0 + EW), slice(r0 // 2, (r0 + EW) // 2)
        res = ([], [], [])
        pre = pace([raw_v[b][0, q, rows] for q in range(4)], after)
        for q in range(4):
            a, u, dp = pre[q], raw_v[b][1, q, rows], raw_v[b][2, q, rows]
            sg = jax.nn.sigmoid(a)
            sl = a * sg
            res[0].append(dp * u * (sg + sl * (1.0 - sg)))
            res[1].append(dp * sl)
            res[2].append(sl * u)
        for m in range(3):
            for r, v in enumerate(_hid_forms(*res[m])):
                p_v[b][m, r, prows, :] = _pk(v)

    gates = lambda b: [part(gate, b, r0) for r0 in range(0, TS, EW)]

    def stage2(t, b, acts=True, wgts=True):
        j, i = t >> 2, t & 3
        ss = blk(i, TS)
        for r in range(7):
            if acts:
                o = _dot(wform(j, 2, r, DH), _up(p_v[b][2, r]), NT)
                acco_v[r][:, ss] = jnp.where(j == 0, 0.0, acco_v[r][:, ss]) + o
                yield o
                o = (_dot(wform(j, 0, r, DH), _up(p_v[b][0, r]), NT)
                     + _dot(wform(j, 1, r, DH), _up(p_v[b][1, r]), NT))
                acch_v[r][:, ss] = jnp.where(j == 0, 0.0, acch_v[r][:, ss]) + o
                yield o
            if wgts:
                for m, f_v in enumerate((hf_v, hf_v, gf_v)):
                    o = _dot(_up(f_v[r, :, ss]), _up(p_v[b][m, r]))
                    m_v[m][r][j & 1] = jnp.where(i == 0, 0.0, m_v[m][r][j & 1]) + o
                    yield o

    fins = lambda j, q: [part(finalize, j, q, m) for m in range(3)]
    preps = lambda j, q: [part(wprep, j, q, r) for r in range(7)]
    cat = lambda lists: list(chain(*lists))

    for c in ([x_cp(0), fa_cp] + [x_cp(i) for i in range(1, ntc)] + w_cp + [gm_cp, g_cp]
              + cat(ffn_cp)):
        c.start()
    for a in range(2):
        for k in range(R1):
            wp_v[a, k, pl.ds(RD * 34, KP - K0 - 34, stride=RD), :] = jnp.zeros(
                (KP - K0 - 34, R2), f32)
    fa_cp.wait()

    def p1(i):
        c = blk(i, TC)
        ys, en = [], 0.0
        for b in range(0, DB, 16):
            y = _rfft9([x_v[a * DB + b:a * DB + b + 16, c].astype(f32) for a in range(RD)])
            sq = [v * v for v in y[:8]]
            en = en + 0.75 * sq[5] + (sq[0] + sq[1] + sq[2] + sq[3] + sq[4] + sq[6] + sq[7])
            ys.append([v.astype(bf16) for v in y[:8]] + [y[8]])
        y = [jnp.concatenate(v, axis=0) for v in zip(*ys)]
        mu = _colmean(y[8])
        y[8] = y[8] - RD * mu
        var = (_colmean(y[8] * y[8]) + 2.0 * _colmean(en)) * (1.0 / RD)
        rstd = 1.0 / jnp.sqrt(var + EPS)
        st_v[0, :, c] = mu
        st_v[1, :, c] = rstd
        z_v[:, c] = dft_d(y) * rstd

    def p1s(n):
        for i in range(UN):
            x_cp(UN * n + i).wait()
        for i in range(UN):
            p1(UN * n + i)
    loop("p1", ntc // UN, p1s)
    loop("radix", KP // 16, lambda r: (radix_fwd(2 * r), radix_fwd(2 * r + 1)))
    for m in range(3):
        for r in range(7):
            m_v[m][r][1] = jnp.zeros((DH, TF), f32)

    for c in w_cp:
        c.wait()

    def pw(r):
        for a in range(2):
            put_w(a, blk(r, 32), wb_v[a, blk(r, 32), :])
    loop("pw", (KF - 1) // 32, pw)
    row = lax.broadcasted_iota(jnp.int32, (16, S), 0)
    for a in range(2):
        last = jnp.broadcast_to(wb_v[a, KF - 1:KF, :].astype(f32), (16, S))
        put_w(a, slice(KF - 1, KP), jnp.where(row == 0, last, 0.0))

    gm_cp.wait()
    with jax.named_scope("p3"):
        _overlap(spectrum(mix_fwd),
                 ([lambda after: g_cp.wait()] + cat(grad_forms(i) for i in range(6)), 7, 31))
    loop("radix", KP // 16, lambda r: (radix_inv(2 * r), radix_inv(2 * r + 1)))
    for c in ffn_cp[0]:
        c.wait()
    for m in range(3):
        for r0 in range(0, DH, 16):
            blocks = [w_v[m, d + r0:d + r0 + 16, f:f + TF].astype(f32)
                      for d in (0, DH) for f in (0, TF)]
            for r, form in enumerate(_wgt_forms(*[lambda v=v: v for v in blocks])):
                ws_v[m][r][0, r0 // 2:r0 // 2 + 8, :] = _pk(form())

    with jax.named_scope("head"):
        _overlap(chain(stage1(0, 0, (2,)), stage1(1, 1, (2,))),
                 (cat(ffn_input(i) for i in (0, 1)), 0, 12))
        _overlap(stage1(0, 0, (0, 1)), (cat(ffn_input(i) for i in (2, 3)), 0, 13))
        for c in ffn_cp[1]:
            c.wait()
        _overlap(stage1(1, 1, (0, 1)), (gates(0), 0, 12),
                 (preps(1, 0) + preps(1, 1), 0, 13))

    def step(t, b, *tasks):
        if not tasks:
            tasks = ((fins(((t - 1) >> 2) + 1, (t - 1) & 3), 49, 55),
                     (preps(((t + 1) >> 2) + 1, (t + 1) & 3), 35, 48))
        _overlap(chain(stage2(t - 1, 1 - b), stage1(t + 1, 1 - b, (0, 1, 2))),
                 (gates(b), 1, 32), *tasks)

    with jax.named_scope("head2"):
        step(1, 1, (ffn_input(4) + ffn_input(5) + ffn_input(6)[:3], 1, 33),
             (ffn_input(6)[3:] + ffn_input(7) + preps(1, 2) + grad_forms(6) + grad_forms(7),
              34, 54))
    for c in ffn_cp[2]:
        c.wait()

    def body(n):
        j = n >> 1

        @pl.when(((n & 1) == 0) & (j >= 3))
        def _():
            for c in dw_cp(j - 3):
                c.wait()

        @pl.when(((n & 1) == 1) & (j >= 2))
        def _():
            for c in dw_cp(j - 2):
                c.start()
        step(2 * n, 0)
        step(2 * n + 1, 1)
    loop("ffn", nt // 2 - 1, body, 1)
    for c in dw_cp(nj - 3):
        c.start()

    with jax.named_scope("tail"):
        step(nt - 2, 0, (ffn_output(0), 1, 30), (ffn_output(1) + fins(nj - 2, 1), 33, 54))
        _overlap(stage2(nt - 2, 0), (gates(1), 1, 32),
                 (cat(ffn_output(i) for i in (2, 3)), 0, 32), (fins(nj - 2, 2), 29, 34))
        o_cp[0].start()
        o_cp[2].start()
        _overlap(stage2(nt - 1, 1, wgts=False), (cat(ffn_output(i) for i in (4, 5)), 0, 13),
                 (fins(nj - 2, 3), 0, 13))
        for c in dw_cp(nj - 2):
            c.start()
        for c in dw_cp(nj - 3):
            c.wait()
        _overlap(stage2(nt - 1, 1, acts=False), (cat(ffn_output(i) for i in (6, 7)), 0, 10),
                 ([part(radix_fwd, r) for r in range(KP // 8)], 12, 20))
    for c in (o_cp[1], o_cp[3]):
        c.start()

    with jax.named_scope("p9"):
        _overlap(spectrum(mix_bwd),
                 (cat(fins(nj - 1, q) for q in range(ni))
                  + [lambda after: [c.start() for c in dw_cp(nj - 1)]], 0, 12))

    def pdw(r):
        for a in range(2):
            wb_v[a, blk(r, 32), :] = get_dw(a, blk(r, 32))
            radix_inv(4 * r + 2 * a)
            radix_inv(4 * r + 2 * a + 1)
        for c in dwf_cp(blk(r, 32), r):
            c.start()
    loop("pdw", (KF - 1) // 32, pdw)
    for a in range(2):
        wb_v[a, KF - 1:KF, :] = get_dw(a, slice(KF - 1, KP)).astype(f32)[0:1].astype(bf16)
        radix_inv((KF - 1) // 8 + a)
    dwf_all = [dwf_cp(blk(r, 32), r) for r in range(9)] + [dwf_cp(pl.ds(KF - 1, 1), 9)]
    for c in dwf_all[-1]:
        c.start()

    def p11(i):
        c = blk(i, R2)
        y = idft_d(z_v[:, c], 10)
        mu, rstd = st_v[0, :, c], st_v[1, :, c]
        proj = 0.0
        for b in range(0, DB, 16):
            for a, d in enumerate(_rfft9_t([v[b:b + 16] for v in y])):
                rows = slice(a * DB + b, a * DB + b + 16)
                proj = proj + d * (x_v[rows, c].astype(f32) - mu)
                h_v[rows, c] += rstd * d
        proj = _colmean(proj) * rstd * rstd * rstd
        for r in range(0, D, 16):
            g_v[r:r + 16, c] = (h_v[r:r + 16, c]
                                - (x_v[r:r + 16, c].astype(f32) - mu) * proj).astype(bf16)

    for lo, hi in ((0, 2), (2, 4), (4, 6), (6, 7), (7, 8)):
        with jax.named_scope("p11"):
            for i in range(lo * TC // R2, hi * TC // R2):
                p11(i)
        for i in range(lo, hi):
            dx_cp(i).start()

    for c in (dw_cp(nj - 2) + dw_cp(nj - 1) + o_cp + cat(dwf_all)
              + [dx_cp(i) for i in range(ntc)]):
        c.wait()


@jax.jit
def pallas_sequential_preLN__spectral_gfnet__swiglu_ffn__prompt_kernel(
    A_x: jax.Array,
    A_w_r: jax.Array,
    A_w_i: jax.Array,
    B_x: jax.Array,
    B_w_gate: jax.Array,
    B_w_up: jax.Array,
    B_w_down: jax.Array,
    grad_out: jax.Array,
):
    del B_x
    sds = jax.ShapeDtypeStruct
    hbm = pl.BlockSpec(memory_space=pltpu.HBM)
    out, dx, dwr, dwi, dwg, dwu, dwd = pl.pallas_call(
        _kernel,
        out_shape=[sds((D, S), bf16), sds((D, S), bf16),
                   sds((KF, S), bf16), sds((KF, S), bf16),
                   sds((D, F), bf16), sds((D, F), bf16), sds((D, F), bf16)],
        in_specs=[hbm] * 9,
        out_specs=[hbm] * 7,
        scratch_shapes=[
            V((D, S), bf16), V((D, S), bf16), V((2, KF, S), bf16), V((3, D, F), bf16),
            V((11, R2, R2), bf16), V((R1, 3, R2, R2), bf16),
            V((2 * KP, S), f32), V((R1, KP, 2 * R2), f32),
            V((2, R1, RD * (KP - K0), R2), f32), V((R1, KP // 2, 2 * R2), u32),
            V((4, 1, S), f32), V((D, S), f32),
            V((7, DH // 2, SH), u32), V((7, DH // 2, SH), u32),
            V((7, SH // 2, KS), u32), V((7, SH // 2, KS), u32),
            V((2, SH // 2, R2), u32), V((2, SH // 2, R2), u32),
            [[V((3, DH // 2, TF), u32)] * 7] * 3, [V((3, 4, TS, TF), f32)] * 2,
            [V((3, 7, TS // 2, TF), u32)] * 2,
            [V((DH, SH), f32)] * 7, [V((DH, SH), f32)] * 7, [[V((2, DH, TF), f32)] * 7] * 3,
            V((2, 3, D, 2 * TF), bf16),
            pltpu.SemaphoreType.DMA((S // TC + 16,)),
            pltpu.SemaphoreType.DMA((30 + S // TC,)),
        ],
        compiler_params=pltpu.CompilerParams(vmem_limit_bytes=127 * 2**20),
    )(A_x[0].T, A_w_r.T, A_w_i.T, B_w_gate, B_w_up, B_w_down.T, grad_out[0].T,
      _FA, _G)
    return out.T[None], dx.T[None], dwr.T, dwi.T, dwg, dwu, dwd.T
```

```python
import functools
import itertools
import math

import jax
import jax.numpy as jnp
import ml_dtypes
import numpy as np
from jax import lax
from jax.experimental import pallas as pl
from jax.experimental.pallas import tpu as pltpu

S, D, F = 2048, 576, 4608
KF = D // 2 + 1
KP = 304
R1, R2 = 16, 128
RD, DB = 9, 64
K0 = 256
EPS = 1e-5
DH, SH = D // 2, S // 2
KA, KS = 192, 256
TS = 256
TF = 256
UN = 2
EW = 16
WIN = 80
TC = 256

bf16 = jnp.bfloat16
f32 = jnp.float32
u32 = jnp.uint32
V = pltpu.VMEM
NN = (((1,), (0,)), ((), ()))
NT = (((1,), (1,)), ((), ()))


_C1, _C2, _C4 = (math.cos(2 * math.pi * e / RD) for e in (1, 2, 4))
_S1, _S2, _S3, _S4 = (math.sin(2 * math.pi * e / RD) for e in (1, 2, 3, 4))


def _cyc(m, a, b, c, k1, k2, k3):
    e1, e2 = a - c, b - c
    p, q = k1 * e1 + k2 * e2, k2 * e1 + k3 * e2
    return m + p, m + q, m - (p + q)


def _cyc_t(o1, o2, o3, k1, k2, k3):
    p, q = o1 - o3, o2 - o3
    e1, e2 = k1 * p + k2 * q, k2 * p + k3 * q
    return o1 + o2 + o3, e1, e2, -(e1 + e2)


def _rfft9(x):
    s1, s2, s3, s4 = (x[a] + x[RD - a] for a in (1, 2, 3, 4))
    t1, t2, t3, t4 = x[1] - x[8], x[7] - x[2], x[3] - x[6], x[4] - x[5]
    u, v = x[0] + s3, s1 + s2 + s4
    p1, p2, p4 = _cyc(x[0] - 0.5 * s3, s1, s2, s4, _C1, _C2, _C4)
    q1, q2, q4 = _cyc(_S3 * t3, t1, t2, t4, _S1, -_S2, _S4)
    return [p1, q1, p2, q2, u - 0.5 * v, t1 + t2 + t4, p4, q4, u + v]


def _rfft9_t(y):
    p1, q1, p2, q2, p3, q3, p4, q4, y0 = y
    m, s1, s2, s4 = _cyc_t(p1, p2, p4, _C1, _C2, _C4)
    n, t1, t2, t4 = _cyc_t(q1, q2, q4, _S1, -_S2, _S4)
    u, v = y0 + p3, y0 - 0.5 * p3
    s1, s2, s4, s3 = s1 + v, s2 + v, s4 + v, u - 0.5 * m
    t1, t2, t4, t3 = t1 + q3, t2 + q3, t4 + q3, _S3 * n
    return [u + m, s1 + t1, s2 - t2, s3 + t3, s4 + t4, s4 - t4, s3 - t3, s2 + t2, s1 - t1]


_CLASSES = [(64 * (c - 1) + 32 * h, (c, RD - c)[h], 32) for c in (1, 2, 3, 4) for h in (0, 1)]


def _consts():
    root = lambda e, n: np.exp(-2j * np.pi * (e % n) / n)
    bins = np.full(KP, -1)
    for row, c, n in _CLASSES + [(K0, 0, 33)]:
        bins[row:row + n] = c + RD * np.arange(n)
    r9 = np.stack(_rfft9(list(np.eye(RD))))
    r9 = r9 / (r9 * r9).sum(1, keepdims=True)
    coef = (root(bins[:, None, None] * np.arange(RD), RD) * r9).sum(-1)
    full = coef[:, :, None] * root(bins[:, None, None] * np.arange(DB), D)
    full = full.reshape(KP, D) * (bins >= 0)[:, None]
    fa = np.zeros((11, R2, R2))
    for c in range(5):
        blk = full[DB * c:min(DB * c + DB, KP), R2 * c:R2 * c + R2]
        fa[c, :2 * blk.shape[0], :blk.shape[1]] = np.concatenate([blk.real, blk.imag])
        fa[5 + c] = fa[c].T
    fa[10] = fa[9]
    fa[10, :, 0] = 0.0
    k1 = np.arange(R1)[:, None, None]
    lane = (np.arange(R2) - k1) % R2
    k2 = 8 * (lane % 16) + lane // 16
    g = root(np.arange(R2)[:, None] * (k1 + R1 * k2), S)
    g = np.stack([g.real, g.real + g.imag, g.imag - g.real], 1)
    cast = lambda a: (np.round(a, 9) + 0.0).astype(np.float32).astype(ml_dtypes.bfloat16)
    return cast(fa), cast(g)


_FA, _G = _consts()


def _dot(a, b, dn=NN):
    return lax.dot_general(a, b, dn, preferred_element_type=f32)


def _fft4(x, sign):
    (ar, ai), (br, bi), (cr, ci), (dr, di) = x
    s0r, s0i, d0r, d0i = ar + cr, ai + ci, ar - cr, ai - ci
    s1r, s1i, d1r, d1i = br + dr, bi + di, br - dr, bi - di
    lo = (d0r + d1i, d0i - d1r)
    hi = (d0r - d1i, d0i + d1r)
    o1, o3 = (lo, hi) if sign < 0 else (hi, lo)
    return [(s0r + s1r, s0i + s1i), o1, (s0r - s1r, s0i - s1i), o3]


def _tw16(v, e, sign):
    r, i = v
    e %= 16
    if e == 0:
        return v
    if e == 4:
        return (i, -r) if sign < 0 else (-i, r)
    c = math.cos(2 * math.pi * e / 16)
    s = sign * math.sin(2 * math.pi * e / 16)
    if e % 2 == 0:
        if c * s > 0:
            return ((r - i) * c, (r + i) * c)
        return ((r + i) * c, (i - r) * c)
    return (r * c - i * s, r * s + i * c)


def _fft16(x, sign):
    cols = [_fft4([x[4 * a + b] for a in range(4)], sign) for b in range(4)]
    out = [None] * 16
    for p in range(4):
        o = _fft4([_tw16(cols[b][p], b * p, sign) for b in range(4)], sign)
        for q in range(4):
            out[p + 4 * q] = o[q]
    return out


def _swap16(tiles):
    lane = lax.broadcasted_iota(jnp.int32, tiles[0].shape, 1)
    tiles = list(tiles)
    for d in (1, 2, 4, 8):
        for lo in range(d):
            low = ((lane - lo) & d) == 0
            for t in range(lo, R1, 2 * d):
                a, b = tiles[t], tiles[t + d]
                tiles[t], tiles[t + d] = jnp.where(low, a, b), jnp.where(low, b, a)
    return tiles


def _rot16(tiles, sign):
    return [pltpu.roll(v, (sign * t) % R2, 1) if t else v for t, v in enumerate(tiles)]


def _act_forms(a11, a12, a21, a22):
    return (a11 + a22, a21 + a22, a11, a22, a11 + a12, a21 - a11, a12 - a22)


def _hid_forms(p11, p12, p21, p22):
    return (p11 + p22, p11, p12 - p22, p21 - p11, p22, p11 + p12, p21 + p22)


def _wgt_forms(w11, w12, w21, w22):
    return (lambda: w11() + w22(), lambda: w21() - w22(), lambda: w12() + w22(),
            lambda: w11() + w21(), lambda: w12() - w11(), w22, w11)


def _act_join(n):
    return (jnp.concatenate([n[0] + n[2] + n[4] - n[5], n[1] + n[5]], axis=0),
            jnp.concatenate([n[4] + n[6], n[0] + n[1] + n[3] - n[6]], axis=0))


def _pk(v):
    return pltpu.bitcast(v.astype(bf16), u32)


def _up(v):
    return pltpu.bitcast(v, bf16)


def _colmean(x):
    return jnp.sum(x, axis=0, keepdims=True) * (1.0 / D)


def _overlap(dots, *tasks):
    plan = [(first + s * (last - first + 1) // len(steps),
             -(-(last - first + 1) // len(steps)), step)
            for steps, first, last in tasks for s, step in enumerate(steps)]
    seen = []
    for k, o in enumerate(dots):
        seen.append(o)
        for at, span, step in plan:
            if at == k:
                step(seen[-span:])
    assert all(at < len(seen) for at, _, _ in plan)


def _kernel(x_h, wr_h, wi_h, wg_h, wu_h, wd_h, g_h, fa_h, gm_h,
            out_h, dx_h, dwr_h, dwi_h, dwg_h, dwu_h, dwd_h,
            x_v, g_v, wb_v, w_v, fa_v, gm_v,
            z_v, t_v, wp_v, xs_v, st_v, h_v, hf_v, gf_v, hk_v, gk_v, hr_v, gr_v,
            ws_v, raw_v, p_v, acco_v, acch_v, m_v, dw_v, sin, sout):
    ntc = S // TC
    nj = F // (2 * TF)
    ni = SH // TS
    nt = nj * ni
    assert ni == 4 and nt % 2 == 0
    part, chain = functools.partial, itertools.chain

    def loop(name, n, body, lo=0):
        with jax.named_scope(name):
            lax.fori_loop(lo, n, lambda i, carry: (body(i), carry)[1], 0)

    def blk(i, n):
        return pl.ds(i * n, n) if isinstance(i, int) else pl.ds(pl.multiple_of(i * n, n), n)

    def pace(vals, after):
        if not after:
            return vals
        keep = _pk(fa_v[4, R2 - 16:, :]) == 0
        marks = [o[r:r + 8, :R2] for o in after for r in range(0, o.shape[0], 8)]
        n = sum(v.size for v in vals) // (8 * R2)
        marks = iter([marks[i * len(marks) // n] for i in range(n)])
        return [jnp.block([[jnp.where(keep, v[r:r + 8, c:c + R2],
                                      pltpu.bitcast(next(marks), v.dtype))
                            for c in range(0, v.shape[1], R2)]
                           for r in range(0, v.shape[0], 8)]) for v in vals]

    def pace16(v, after):
        return _up(pace([_pk(v)], after)[0])

    cp = pltpu.make_async_copy
    x_cp = lambda i: cp(x_h.at[:, blk(i, TC)], x_v.at[:, blk(i, TC)], sin.at[i])
    fa_cp = cp(fa_h, fa_v, sin.at[ntc])
    gm_cp = cp(gm_h, gm_v, sin.at[ntc + 1])
    g_cp = cp(g_h, g_v, sin.at[ntc + 2])
    w_cp = [cp(src.at[rows], wb_v.at[a, rows], sin.at[ntc + 3 + 2 * a + n])
            for a, src in enumerate((wr_h, wi_h))
            for n, rows in enumerate((pl.ds(0, KF - 1), pl.ds(KF - 1, 1)))]
    ffn_cp = [[cp(src.at[:, cols], w_v.at[m, :, cols], sin.at[ntc + 7 + 3 * n + m])
               for m, src in enumerate((wg_h, wu_h, wd_h))]
              for n, cols in enumerate((pl.ds(0, 2 * TF), pl.ds(2 * TF, 2 * TF),
                                        pl.ds(4 * TF, F - 4 * TF)))]
    dw_cp = lambda j: [cp(dw_v.at[j & 1, m], o.at[:, blk(j, 2 * TF)], sout.at[3 * (j & 1) + m])
                       for m, o in enumerate((dwg_h, dwu_h, dwd_h))]
    ob_v = w_v.at[0, :, pl.ds(0, S)]
    o_cp = [cp(w_v.at[0, :, blk(q, SH // 2)], out_h.at[:, blk(q, SH // 2)], sout.at[6 + q])
            for q in range(4)]
    dwf_cp = lambda rows, n: [cp(wb_v.at[a, rows], o.at[rows], sout.at[10 + ntc + 2 * n + a])
                              for a, o in enumerate((dwr_h, dwi_h))]
    dx_cp = lambda i: cp(g_v.at[:, blk(i, TC)], dx_h.at[:, blk(i, TC)], sout.at[10 + i])

    def dft_d(y):
        out = [_dot(fa_v[c], jnp.concatenate(y[2 * c:2 * c + 2], axis=0).astype(bf16))
               for c in range(4)]
        o0 = _dot(fa_v[4, :2 * (KP - K0), :DB], y[8].astype(bf16))
        return jnp.concatenate([o[:DB] for o in out] + [o0[:KP - K0]]
                               + [o[DB:] for o in out] + [o0[KP - K0:]], axis=0)

    def idft_d(z, last):
        y = []
        for c in range(4):
            zc = jnp.concatenate([z[DB * c:DB * c + DB], z[KP + DB * c:KP + DB * c + DB]], axis=0)
            o = _dot(fa_v[5 + c], zc.astype(bf16))
            y += [o[:DB], o[DB:]]
        zc = jnp.concatenate([z[K0:KP], z[KP + K0:]], axis=0)
        y.append(_dot(fa_v[last, :DB, :2 * (KP - K0)], zc.astype(bf16)))
        return y

    def radix_fwd(r, after=None):
        re, im = blk(r, 8), blk(r + KP // 8, 8)
        a = pace([z_v[re, n * R2:(n + 1) * R2] for n in range(R1)]
                 + [z_v[im, n * R2:(n + 1) * R2] for n in range(R1)], after)
        for k, (vr, vi) in enumerate(_fft16(list(zip(a[:R1], a[R1:])), -1)):
            t_v[k, re, :R2] = vr
            t_v[k, re, R2:] = vi

    def radix_inv(r, after=None):
        re, im = blk(r, 8), blk(r + KP // 8, 8)
        a = pace([t_v[n, re, :R2] for n in range(R1)]
                 + [t_v[n, re, R2:] for n in range(R1)], after)
        for k, (vr, vi) in enumerate(_fft16(list(zip(a[:R1], a[R1:])), 1)):
            z_v[re, k * R2:(k + 1) * R2] = vr
            z_v[im, k * R2:(k + 1) * R2] = vi

    def scale():
        k = lax.broadcasted_iota(jnp.int32, (KP, R2), 0)
        return jnp.where((k == K0) | (k == K0 + 32), 1.0 / (S * D), 2.0 / (S * D))

    def filt(k1):
        rows = [pl.ds(c, n, stride=RD) for _, c, n in _CLASSES + [(K0, 0, KP - K0)]]
        return [jnp.concatenate([wp_v[a, k1, r, :] for r in rows], axis=0) for a in range(2)]

    def spectrum(mix):
        prev = None
        for k1 in range(R1 + 1):
            if k1 < R1:
                a, b = t_v[k1, :, :R2], t_v[k1, :, R2:]
                n = [_dot(v.astype(bf16), gm_v[k1, e]) for e, v in enumerate((a + b, b, a))]
                cur = (n[0] - n[1], n[0] + n[2])
                yield n[2]
            if prev is not None:
                a, b = mix(k1 - 1, *prev)
                n = [_dot(v.astype(bf16), gm_v[k1 - 1, e], NT)
                     for e, v in enumerate((a + b, a, b))]
                t_v[k1 - 1, :, :R2] = n[0] + n[2]
                t_v[k1 - 1, :, R2:] = n[0] - n[1]
                yield n[2]
            prev = cur

    def mix_fwd(k1, xr, xi):
        cc = scale()
        xr, xi = xr * cc, xi * cc
        xs_v[k1, :, :R2] = _pk(xr)
        xs_v[k1, :, R2:] = _pk(xi)
        wr, wi = filt(k1)
        return [xr * wr - xi * wi, xr * wi + xi * wr]

    def mix_bwd(k1, dr, di):
        cc = scale()
        wr, wi = (w * cc for w in filt(k1))
        xr, xi = _up(xs_v[k1, :, :R2]).astype(f32), _up(xs_v[k1, :, R2:]).astype(f32)
        for a, v in enumerate((dr * xr + di * xi, di * xr - dr * xi)):
            for row, c, n in _CLASSES + [(K0, 0, 40)]:
                wp_v[a, k1, pl.ds(c, n, stride=RD), :] = v[row:row + n]
        return [dr * wr + di * wi, di * wr - dr * wi]

    def put_w(a, rr, w):
        w = _pk(w)
        tiles = _swap16(_rot16([w[:, t * R2:(t + 1) * R2] for t in range(R1)], 1))
        for k in range(R1):
            wp_v[a, k, rr, :] = _up(tiles[k]).astype(f32)

    def get_dw(a, rr):
        tiles = [_pk(wp_v[a, k, rr, :]) for k in range(R1)]
        return _up(jnp.concatenate(_rot16(_swap16(tiles), -1), axis=1))

    def pair(i):
        return blk(i, R2), blk(i + SH // R2, R2)

    def put_f(i, xa, xb, f_v):
        for r, v in enumerate(_act_forms(xa[:DH], xb[:DH], xa[DH:], xb[DH:])):
            f_v[r, :, blk(i, R2)] = _pk(v)

    def put_k(i, xa, xb, k_v, r_v):
        rows = blk(i, R2 // 2)
        f = list(_act_forms(xa[:KS].T, xb[:KS].T, xa[DH:DH + KS].T, xb[DH:DH + KS].T))
        ta, tb = [jnp.concatenate([x[KS:DH], x[DH + KS:]] * 2, axis=0).T for x in (xa, xb)]
        low = lax.broadcasted_iota(jnp.int32, (R2, R2), 1) < KA - R2
        hi = [v[:, R2:] for v in f]
        for r, v in ((1, ta), (2, -hi[3]), (3, -hi[2]), (4, tb)):
            f[r] = jnp.concatenate([f[r][:, :R2], jnp.where(low, hi[r], v)], axis=1)
        for r, v in enumerate(f):
            k_v[r, rows, :] = _pk(v)
        r_v[0, rows, :] = _pk(jnp.where(low, ta, -hi[1]))
        r_v[1, rows, :] = _pk(jnp.where(low, tb, -hi[4]))

    def grad_forms(i):
        ld = lambda after: [pace16(g_v[:, c], after).astype(f32) for c in pair(i)]
        return [lambda after: put_f(i, *ld(after), gf_v),
                lambda after: put_k(i, *ld(after), gk_v, gr_v)]

    def ffn_input(i):
        y = []

        def dots(after):
            y.extend(idft_d(jnp.concatenate([z_v[:, c] for c in pair(i)], axis=1), 9))

        def residual(half, after):
            c = pair(i)[half]
            groups = range(0, DB, 16)
            yy = pace([v[b:b + 16, half * R2:(half + 1) * R2] for b in groups for v in y], after)
            hs, mu, var = [], 0.0, 0.0
            for n, b in enumerate(groups):
                for a, d in enumerate(_rfft9_t(yy[RD * n:RD * n + RD])):
                    rows = slice(a * DB + b, a * DB + b + 16)
                    hs.append(x_v[rows, c].astype(f32) + d)
                    h_v[rows, c] = hs[-1]
                    mu = mu + hs[-1]
            mu = _colmean(mu)
            for h in hs:
                var = var + (h - mu) * (h - mu)
            st_v[2, :, c] = mu
            st_v[3, :, c] = 1.0 / jnp.sqrt(_colmean(var) + EPS)

        hn = lambda after: [(pace([h_v[:, c]], after)[0] - st_v[2, :, c]) * st_v[3, :, c]
                            for c in pair(i)]
        return [dots, part(residual, 0), part(residual, 1),
                lambda after: put_f(i, *hn(after), hf_v),
                lambda after: put_k(i, *hn(after), hk_v, hr_v)]

    def ffn_output(i):
        keep, y = {}, []

        def join(acc, after):
            n = [acc[r][:, blk(i, R2)] for r in range(7)]
            n[0], n[1], n[4] = pace([n[0], n[1], n[4]], after)
            return _act_join(n)

        def out(after):
            for o, c in zip(join(acco_v, after), pair(i)):
                ob_v[:, c] = (h_v[:, c] + o).astype(bf16)

        def stats(after):
            for half, (d, c) in enumerate(zip(join(acch_v, after), pair(i))):
                hn = (pace([h_v[:, c]], after)[0] - st_v[2, :, c]) * st_v[3, :, c]
                keep[half] = (d, hn, _colmean(d), _colmean(d * hn))

        def grad(half, after):
            c = pair(i)[half]
            d, hn, m1, m2 = keep[half]
            rows = [slice(a * DB + b, a * DB + b + 16) for b in range(0, DB, 16) for a in range(RD)]
            d, hn = pace([d[r] for r in rows], after), pace([hn[r] for r in rows], after)
            rstd, ys = st_v[3, :, c], []
            for n in range(0, len(rows), RD):
                dh = [g_v[rows[k], c].astype(f32) + rstd * (d[k] - m1 - hn[k] * m2)
                      for k in range(n, n + RD)]
                for r, v in zip(rows[n:n + RD], dh):
                    h_v[r, c] = v
                ys.append([v.astype(bf16) for v in _rfft9(dh)])
            y.append([jnp.concatenate(v, axis=0) for v in zip(*ys)])

        def dots(after):
            z = dft_d([jnp.concatenate(v, axis=1) for v in zip(*y)])
            for half, c in enumerate(pair(i)):
                z_v[:, c] = z[:, half * R2:(half + 1) * R2]

        return [out, stats, part(grad, 0), part(grad, 1), dots]

    def window(q):
        r0 = (min if isinstance(q, int) else jnp.minimum)(q * (WIN // 16), (DH - WIN) // 16)
        hint = (lambda v, n: v) if isinstance(q, int) else pl.multiple_of
        return (pl.ds(hint(r0 * 16, 16), WIN), pl.ds(hint(r0 * 16 + DH, 16), WIN),
                pl.ds(hint(r0 * 8, 8), WIN // 2))

    def mod3(j):
        return j % 3 if isinstance(j, int) else lax.rem(j, 3)

    def wprep(j, q, r, after=None):
        src = j if isinstance(j, int) else jnp.minimum(j, nj - 1)
        f1, f2 = blk(2 * src, TF), blk(2 * src + 1, TF)
        d1, d2, dst = window(q)
        for m in range(3):
            ld = lambda d, f: lambda: pace16(w_v[m, d, f], after)
            form = _wgt_forms(ld(d1, f1), ld(d1, f2), ld(d2, f1), ld(d2, f2))[r]
            ws_v[m][r][mod3(j), dst, :] = _pk(form())

    def wform(j, m, r, n):
        return _up(ws_v[m][r][mod3(j), 0:n // 2, :])

    def finalize(j, q, m, after=None):
        d1, d2, _ = window(q)
        n = [pace([m_v[m][r][j & 1, d1, :]], after if r < 4 else None)[0] for r in range(7)]
        dw_v[j & 1, m, d1, :TF] = (n[0] + n[3] - n[4] + n[6]).astype(bf16)
        dw_v[j & 1, m, d1, TF:] = (n[2] + n[4]).astype(bf16)
        dw_v[j & 1, m, d2, :TF] = (n[1] + n[3]).astype(bf16)
        dw_v[j & 1, m, d2, TF:] = (n[0] - n[1] + n[2] + n[5]).astype(bf16)

    def stage1(t, b, ms):
        j, ss = t >> 2, blk(t & 3, TS // 2)
        f1, f2 = blk(2 * j, TF), blk(2 * j + 1, TF)
        rows = part(jnp.concatenate, axis=0)
        zero = jnp.zeros((KS - KA, TF), bf16)
        for m in ms:
            k_v, r_v = (gk_v, gr_v) if m == 2 else (hk_v, hr_v)
            v1, v2 = [[w_v[m, KS:DH, f], w_v[m, DH + KS:, f]] for f in (f1, f2)]
            w12, w21 = w_v[m, KA:KS, f2], w_v[m, DH + KA:DH + KS, f1]
            q = lambda r, tail: _dot(_up(k_v[r, ss, :]), rows([wform(j, m, r, KA)] + tail))
            mid = lambda r: [_up(ws_v[m][r][mod3(j), KA // 2:KS // 2, :])]
            q2 = q(2, mid(2))
            yield q2
            q5 = q(5, [w21])
            yield q5
            a7, w7 = _up(k_v[0, ss, R2:]), rows([zero, w12 + w21])
            if m == ms[-1] and len(ms) % 2:
                q7 = rows([_dot(a7[:TS // 2], w7), _dot(a7[TS // 2:], w7)])
            else:
                q7 = _dot(a7, w7)
            raw_v[b][m, 1] = q2 + q5 + q7 + _dot(_up(r_v[0, ss, :]), rows(v2 + mid(1)))
            q3 = q(3, mid(3))
            yield q3
            q6 = q(6, [w12])
            yield q6
            raw_v[b][m, 2] = q3 + q7 + q6 + _dot(_up(r_v[1, ss, :]), rows(v1 + mid(4)))
            q0 = q(0, [zero])
            yield q0
            q1 = q(1, v1)
            raw_v[b][m, 0] = (q0 + q5 - q3) + q1
            yield q1
            q4 = q(4, v2)
            raw_v[b][m, 3] = (q0 - q2 + q6) + q4
            yield q4

    def gate(b, r0, after):
        rows, prows = slice(r0, r0 + EW), slice(r0 // 2, (r0 + EW) // 2)
        res = ([], [], [])
        pre = pace([raw_v[b][0, q, rows] for q in range(4)], after)
        for q in range(4):
            a, u, dp = pre[q], raw_v[b][1, q, rows], raw_v[b][2, q, rows]
            sg = jax.nn.sigmoid(a)
            sl = a * sg
            res[0].append(dp * u * (sg + sl * (1.0 - sg)))
            res[1].append(dp * sl)
            res[2].append(sl * u)
        for m in range(3):
            for r, v in enumerate(_hid_forms(*res[m])):
                p_v[b][m, r, prows, :] = _pk(v)

    gates = lambda b: [part(gate, b, r0) for r0 in range(0, TS, EW)]

    def stage2(t, b, acts=True, wgts=True):
        j, i = t >> 2, t & 3
        ss = blk(i, TS)
        for r in range(7):
            if acts:
                o = _dot(wform(j, 2, r, DH), _up(p_v[b][2, r]), NT)
                acco_v[r][:, ss] = jnp.where(j == 0, 0.0, acco_v[r][:, ss]) + o
                yield o
                o = (_dot(wform(j, 0, r, DH), _up(p_v[b][0, r]), NT)
                     + _dot(wform(j, 1, r, DH), _up(p_v[b][1, r]), NT))
                acch_v[r][:, ss] = jnp.where(j == 0, 0.0, acch_v[r][:, ss]) + o
                yield o
            if wgts:
                for m, f_v in enumerate((hf_v, hf_v, gf_v)):
                    o = _dot(_up(f_v[r, :, ss]), _up(p_v[b][m, r]))
                    m_v[m][r][j & 1] = jnp.where(i == 0, 0.0, m_v[m][r][j & 1]) + o
                    yield o

    fins = lambda j, q: [part(finalize, j, q, m) for m in range(3)]
    preps = lambda j, q: [part(wprep, j, q, r) for r in range(7)]
    cat = lambda lists: list(chain(*lists))

    for c in ([x_cp(0), fa_cp] + [x_cp(i) for i in range(1, ntc)] + w_cp + [gm_cp, g_cp]
              + cat(ffn_cp)):
        c.start()
    for a in range(2):
        for k in range(R1):
            wp_v[a, k, pl.ds(RD * 34, KP - K0 - 34, stride=RD), :] = jnp.zeros(
                (KP - K0 - 34, R2), f32)
    fa_cp.wait()

    def p1(i):
        c = blk(i, TC)
        ys, en = [], 0.0
        for b in range(0, DB, 16):
            y = _rfft9([x_v[a * DB + b:a * DB + b + 16, c].astype(f32) for a in range(RD)])
            sq = [v * v for v in y[:8]]
            en = en + 0.75 * sq[5] + (sq[0] + sq[1] + sq[2] + sq[3] + sq[4] + sq[6] + sq[7])
            ys.append([v.astype(bf16) for v in y[:8]] + [y[8]])
        y = [jnp.concatenate(v, axis=0) for v in zip(*ys)]
        mu = _colmean(y[8])
        y[8] = y[8] - RD * mu
        var = (_colmean(y[8] * y[8]) + 2.0 * _colmean(en)) * (1.0 / RD)
        rstd = 1.0 / jnp.sqrt(var + EPS)
        st_v[0, :, c] = mu
        st_v[1, :, c] = rstd
        z_v[:, c] = dft_d(y) * rstd

    def p1s(n):
        for i in range(UN):
            x_cp(UN * n + i).wait()
        for i in range(UN):
            p1(UN * n + i)
    loop("p1", ntc // UN, p1s)
    loop("radix", KP // 16, lambda r: (radix_fwd(2 * r), radix_fwd(2 * r + 1)))
    for m in range(3):
        for r in range(7):
            m_v[m][r][1] = jnp.zeros((DH, TF), f32)

    for c in w_cp:
        c.wait()

    def pw(r):
        for a in range(2):
            put_w(a, blk(r, 32), wb_v[a, blk(r, 32), :])
    loop("pw", (KF - 1) // 32, pw)
    row = lax.broadcasted_iota(jnp.int32, (16, S), 0)
    for a in range(2):
        last = jnp.broadcast_to(wb_v[a, KF - 1:KF, :].astype(f32), (16, S))
        put_w(a, slice(KF - 1, KP), jnp.where(row == 0, last, 0.0))

    gm_cp.wait()
    with jax.named_scope("p3"):
        _overlap(spectrum(mix_fwd),
                 ([lambda after: g_cp.wait()] + cat(grad_forms(i) for i in range(5)), 11, 31))
    loop("radix", KP // 16, lambda r: (radix_inv(2 * r), radix_inv(2 * r + 1)))
    for c in ffn_cp[0]:
        c.wait()
    for m in range(3):
        for r0 in range(0, DH, 16):
            blocks = [w_v[m, d + r0:d + r0 + 16, f:f + TF].astype(f32)
                      for d in (0, DH) for f in (0, TF)]
            for r, form in enumerate(_wgt_forms(*[lambda v=v: v for v in blocks])):
                ws_v[m][r][0, r0 // 2:r0 // 2 + 8, :] = _pk(form())

    with jax.named_scope("head"):
        _overlap(chain(stage1(0, 0, (2,)), stage1(1, 1, (2,))),
                 (cat(ffn_input(i) for i in (0, 1)), 0, 12))
        _overlap(stage1(0, 0, (0, 1)), (cat(ffn_input(i) for i in (2, 3)), 0, 13))
        for c in ffn_cp[1]:
            c.wait()
        _overlap(stage1(1, 1, (0, 1)), (gates(0), 0, 12),
                 (preps(1, 0) + preps(1, 1), 0, 13))

    def step(t, b, *tasks):
        if not tasks:
            tasks = ((fins(((t - 1) >> 2) + 1, (t - 1) & 3), 49, 55),
                     (preps(((t + 1) >> 2) + 1, (t + 1) & 3), 35, 48))
        _overlap(chain(stage2(t - 1, 1 - b), stage1(t + 1, 1 - b, (0, 1, 2))),
                 (gates(b), 1, 32), *tasks)

    with jax.named_scope("head2"):
        in6 = ffn_input(6)
        step(1, 1, (ffn_input(4) + ffn_input(5) + grad_forms(5) + in6[:1], 1, 33),
             (in6[1:] + ffn_input(7) + preps(1, 2) + grad_forms(6) + grad_forms(7),
              34, 54))
    for c in ffn_cp[2]:
        c.wait()

    def body(n):
        j = n >> 1

        @pl.when(((n & 1) == 0) & (j >= 3))
        def _():
            for c in dw_cp(j - 3):
                c.wait()

        @pl.when(((n & 1) == 1) & (j >= 2))
        def _():
            for c in dw_cp(j - 2):
                c.start()
        step(2 * n, 0)
        step(2 * n + 1, 1)
    loop("ffn", nt // 2 - 1, body, 1)
    for c in dw_cp(nj - 3):
        c.start()

    with jax.named_scope("tail"):
        step(nt - 2, 0, (ffn_output(0) + ffn_output(1), 1, 34),
             (ffn_output(2) + ffn_output(3), 35, 54))
        o_cp[0].start()
        o_cp[2].start()
        _overlap(chain(stage2(nt - 2, 0, wgts=False), stage2(nt - 2, 0, acts=False)),
                 (gates(1), 1, 32), (ffn_output(4) + ffn_output(5), 14, 33),
                 (fins(nj - 2, 1), 0, 13))
        _overlap(chain(stage2(nt - 1, 1, wgts=False), stage2(nt - 1, 1, acts=False)),
                 (fins(nj - 2, 2) + fins(nj - 2, 3)
                  + [lambda after: [c.start() for c in dw_cp(nj - 2)]
                     + [c.wait() for c in dw_cp(nj - 3)]], 0, 13),
                 (ffn_output(6) + ffn_output(7), 14, 25),
                 ([part(radix_fwd, r) for r in range(KP // 8)], 26, 34))
    for c in (o_cp[1], o_cp[3]):
        c.start()

    with jax.named_scope("p9"):
        _overlap(spectrum(mix_bwd),
                 (cat(fins(nj - 1, q) for q in range(ni))
                  + [lambda after: [c.start() for c in dw_cp(nj - 1)]], 0, 12))

    def pdw(r):
        for a in range(2):
            wb_v[a, blk(r, 32), :] = get_dw(a, blk(r, 32))
            radix_inv(4 * r + 2 * a)
            radix_inv(4 * r + 2 * a + 1)
        for c in dwf_cp(blk(r, 32), r):
            c.start()
    loop("pdw", (KF - 1) // 32, pdw)
    for a in range(2):
        wb_v[a, KF - 1:KF, :] = get_dw(a, slice(KF - 1, KP)).astype(f32)[0:1].astype(bf16)
        radix_inv((KF - 1) // 8 + a)
    dwf_all = [dwf_cp(blk(r, 32), r) for r in range(9)] + [dwf_cp(pl.ds(KF - 1, 1), 9)]
    for c in dwf_all[-1]:
        c.start()

    def p11(i):
        c = blk(i, R2)
        y = idft_d(z_v[:, c], 10)
        mu, rstd = st_v[0, :, c], st_v[1, :, c]
        proj = 0.0
        for b in range(0, DB, 16):
            for a, d in enumerate(_rfft9_t([v[b:b + 16] for v in y])):
                rows = slice(a * DB + b, a * DB + b + 16)
                proj = proj + d * (x_v[rows, c].astype(f32) - mu)
                h_v[rows, c] += rstd * d
        proj = _colmean(proj) * rstd * rstd * rstd
        for r in range(0, D, 16):
            g_v[r:r + 16, c] = (h_v[r:r + 16, c]
                                - (x_v[r:r + 16, c].astype(f32) - mu) * proj).astype(bf16)

    for lo, hi in ((0, 2), (2, 4), (4, 6), (6, 7), (7, 8)):
        with jax.named_scope("p11"):
            for i in range(lo * TC // R2, hi * TC // R2):
                p11(i)
        for i in range(lo, hi):
            dx_cp(i).start()

    for c in (dw_cp(nj - 2) + dw_cp(nj - 1) + o_cp + cat(dwf_all)
              + [dx_cp(i) for i in range(ntc)]):
        c.wait()


@jax.jit
def pallas_sequential_preLN__spectral_gfnet__swiglu_ffn__prompt_kernel(
    A_x: jax.Array,
    A_w_r: jax.Array,
    A_w_i: jax.Array,
    B_x: jax.Array,
    B_w_gate: jax.Array,
    B_w_up: jax.Array,
    B_w_down: jax.Array,
    grad_out: jax.Array,
):
    del B_x
    sds = jax.ShapeDtypeStruct
    hbm = pl.BlockSpec(memory_space=pltpu.HBM)
    out, dx, dwr, dwi, dwg, dwu, dwd = pl.pallas_call(
        _kernel,
        out_shape=[sds((D, S), bf16), sds((D, S), bf16),
                   sds((KF, S), bf16), sds((KF, S), bf16),
                   sds((D, F), bf16), sds((D, F), bf16), sds((D, F), bf16)],
        in_specs=[hbm] * 9,
        out_specs=[hbm] * 7,
        scratch_shapes=[
            V((D, S), bf16), V((D, S), bf16), V((2, KF, S), bf16), V((3, D, F), bf16),
            V((11, R2, R2), bf16), V((R1, 3, R2, R2), bf16),
            V((2 * KP, S), f32), V((R1, KP, 2 * R2), f32),
            V((2, R1, RD * (KP - K0), R2), f32), V((R1, KP // 2, 2 * R2), u32),
            V((4, 1, S), f32), V((D, S), f32),
            V((7, DH // 2, SH), u32), V((7, DH // 2, SH), u32),
            V((7, SH // 2, KS), u32), V((7, SH // 2, KS), u32),
            V((2, SH // 2, R2), u32), V((2, SH // 2, R2), u32),
            [[V((3, DH // 2, TF), u32)] * 7] * 3, [V((3, 4, TS, TF), f32)] * 2,
            [V((3, 7, TS // 2, TF), u32)] * 2,
            [V((DH, SH), f32)] * 7, [V((DH, SH), f32)] * 7, [[V((2, DH, TF), f32)] * 7] * 3,
            V((2, 3, D, 2 * TF), bf16),
            pltpu.SemaphoreType.DMA((S // TC + 16,)),
            pltpu.SemaphoreType.DMA((30 + S // TC,)),
        ],
        compiler_params=pltpu.CompilerParams(vmem_limit_bytes=127 * 2**20),
    )(A_x[0].T, A_w_r.T, A_w_i.T, B_w_gate, B_w_up, B_w_down.T, grad_out[0].T,
      _FA, _G)
    return out.T[None], dx.T[None], dwr.T, dwi.T, dwg, dwu, dwd.T
```

```python
import functools
import itertools
import math

import jax
import jax.numpy as jnp
import ml_dtypes
import numpy as np
from jax import lax
from jax.experimental import pallas as pl
from jax.experimental.pallas import tpu as pltpu

S, D, F = 2048, 576, 4608
KF = D // 2 + 1
KP = 304
R1, R2 = 16, 128
RD, DB = 9, 64
K0 = 256
EPS = 1e-5
DH, SH = D // 2, S // 2
KA, KS = 192, 256
TS = 256
TF = 256
UN = 2
EW = 16
WIN = 80
TC = 256

bf16 = jnp.bfloat16
f32 = jnp.float32
u32 = jnp.uint32
V = pltpu.VMEM
NN = (((1,), (0,)), ((), ()))
NT = (((1,), (1,)), ((), ()))


_C1, _C2, _C4 = (math.cos(2 * math.pi * e / RD) for e in (1, 2, 4))
_S1, _S2, _S3, _S4 = (math.sin(2 * math.pi * e / RD) for e in (1, 2, 3, 4))


def _cyc(m, a, b, c, k1, k2, k3):
    e1, e2 = a - c, b - c
    p, q = k1 * e1 + k2 * e2, k2 * e1 + k3 * e2
    return m + p, m + q, m - (p + q)


def _cyc_t(o1, o2, o3, k1, k2, k3):
    p, q = o1 - o3, o2 - o3
    e1, e2 = k1 * p + k2 * q, k2 * p + k3 * q
    return o1 + o2 + o3, e1, e2, -(e1 + e2)


def _rfft9(x):
    s1, s2, s3, s4 = (x[a] + x[RD - a] for a in (1, 2, 3, 4))
    t1, t2, t3, t4 = x[1] - x[8], x[7] - x[2], x[3] - x[6], x[4] - x[5]
    u, v = x[0] + s3, s1 + s2 + s4
    p1, p2, p4 = _cyc(x[0] - 0.5 * s3, s1, s2, s4, _C1, _C2, _C4)
    q1, q2, q4 = _cyc(_S3 * t3, t1, t2, t4, _S1, -_S2, _S4)
    return [p1, q1, p2, q2, u - 0.5 * v, t1 + t2 + t4, p4, q4, u + v]


def _rfft9_t(y):
    p1, q1, p2, q2, p3, q3, p4, q4, y0 = y
    m, s1, s2, s4 = _cyc_t(p1, p2, p4, _C1, _C2, _C4)
    n, t1, t2, t4 = _cyc_t(q1, q2, q4, _S1, -_S2, _S4)
    u, v = y0 + p3, y0 - 0.5 * p3
    s1, s2, s4, s3 = s1 + v, s2 + v, s4 + v, u - 0.5 * m
    t1, t2, t4, t3 = t1 + q3, t2 + q3, t4 + q3, _S3 * n
    return [u + m, s1 + t1, s2 - t2, s3 + t3, s4 + t4, s4 - t4, s3 - t3, s2 + t2, s1 - t1]


_CLASSES = [(64 * (c - 1) + 32 * h, (c, RD - c)[h], 32) for c in (1, 2, 3, 4) for h in (0, 1)]


def _consts():
    root = lambda e, n: np.exp(-2j * np.pi * (e % n) / n)
    bins = np.full(KP, -1)
    for row, c, n in _CLASSES + [(K0, 0, 33)]:
        bins[row:row + n] = c + RD * np.arange(n)
    r9 = np.stack(_rfft9(list(np.eye(RD))))
    r9 = r9 / (r9 * r9).sum(1, keepdims=True)
    coef = (root(bins[:, None, None] * np.arange(RD), RD) * r9).sum(-1)
    full = coef[:, :, None] * root(bins[:, None, None] * np.arange(DB), D)
    full = full.reshape(KP, D) * (bins >= 0)[:, None]
    fa = np.zeros((11, R2, R2))
    for c in range(5):
        blk = full[DB * c:min(DB * c + DB, KP), R2 * c:R2 * c + R2]
        fa[c, :2 * blk.shape[0], :blk.shape[1]] = np.concatenate([blk.real, blk.imag])
        fa[5 + c] = fa[c].T
    fa[10] = fa[9]
    fa[10, :, 0] = 0.0
    k1 = np.arange(R1)[:, None, None]
    lane = (np.arange(R2) - k1) % R2
    k2 = 8 * (lane % 16) + lane // 16
    g = root(np.arange(R2)[:, None] * (k1 + R1 * k2), S)
    g = np.stack([g.real, g.real + g.imag, g.imag - g.real], 1)
    cast = lambda a: (np.round(a, 9) + 0.0).astype(np.float32).astype(ml_dtypes.bfloat16)
    return cast(fa), cast(g)


_FA, _G = _consts()


def _dot(a, b, dn=NN):
    return lax.dot_general(a, b, dn, preferred_element_type=f32)


def _fft4(x, sign):
    (ar, ai), (br, bi), (cr, ci), (dr, di) = x
    s0r, s0i, d0r, d0i = ar + cr, ai + ci, ar - cr, ai - ci
    s1r, s1i, d1r, d1i = br + dr, bi + di, br - dr, bi - di
    lo = (d0r + d1i, d0i - d1r)
    hi = (d0r - d1i, d0i + d1r)
    o1, o3 = (lo, hi) if sign < 0 else (hi, lo)
    return [(s0r + s1r, s0i + s1i), o1, (s0r - s1r, s0i - s1i), o3]


def _tw16(v, e, sign):
    r, i = v
    e %= 16
    if e == 0:
        return v
    if e == 4:
        return (i, -r) if sign < 0 else (-i, r)
    c = math.cos(2 * math.pi * e / 16)
    s = sign * math.sin(2 * math.pi * e / 16)
    if e % 2 == 0:
        if c * s > 0:
            return ((r - i) * c, (r + i) * c)
        return ((r + i) * c, (i - r) * c)
    return (r * c - i * s, r * s + i * c)


def _fft16(x, sign):
    cols = [_fft4([x[4 * a + b] for a in range(4)], sign) for b in range(4)]
    out = [None] * 16
    for p in range(4):
        o = _fft4([_tw16(cols[b][p], b * p, sign) for b in range(4)], sign)
        for q in range(4):
            out[p + 4 * q] = o[q]
    return out


def _swap16(tiles):
    lane = lax.broadcasted_iota(jnp.int32, tiles[0].shape, 1)
    tiles = list(tiles)
    for d in (1, 2, 4, 8):
        for lo in range(d):
            low = ((lane - lo) & d) == 0
            for t in range(lo, R1, 2 * d):
                a, b = tiles[t], tiles[t + d]
                tiles[t], tiles[t + d] = jnp.where(low, a, b), jnp.where(low, b, a)
    return tiles


def _rot16(tiles, sign):
    return [pltpu.roll(v, (sign * t) % R2, 1) if t else v for t, v in enumerate(tiles)]


def _act_forms(a11, a12, a21, a22):
    return (a11 + a22, a21 + a22, a11, a22, a11 + a12, a21 - a11, a12 - a22)


def _hid_forms(p11, p12, p21, p22):
    return (p11 + p22, p11, p12 - p22, p21 - p11, p22, p11 + p12, p21 + p22)


def _wgt_forms(w11, w12, w21, w22):
    return (lambda: w11() + w22(), lambda: w21() - w22(), lambda: w12() + w22(),
            lambda: w11() + w21(), lambda: w12() - w11(), w22, w11)


def _act_join(n):
    return (jnp.concatenate([n[0] + n[2] + n[4] - n[5], n[1] + n[5]], axis=0),
            jnp.concatenate([n[4] + n[6], n[0] + n[1] + n[3] - n[6]], axis=0))


def _pk(v):
    return pltpu.bitcast(v.astype(bf16), u32)


def _up(v):
    return pltpu.bitcast(v, bf16)


def _colmean(x):
    return jnp.sum(x, axis=0, keepdims=True) * (1.0 / D)


def _overlap(dots, *tasks):
    plan = [(first + s * (last - first + 1) // len(steps),
             -(-(last - first + 1) // len(steps)), step)
            for steps, first, last in tasks for s, step in enumerate(steps)]
    seen = []
    for k, o in enumerate(dots):
        seen.append(o)
        for at, span, step in plan:
            if at == k:
                step(seen[-span:])
    assert all(at < len(seen) for at, _, _ in plan)


def _kernel(x_h, wr_h, wi_h, wg_h, wu_h, wd_h, g_h, fa_h, gm_h,
            out_h, dx_h, dwr_h, dwi_h, dwg_h, dwu_h, dwd_h,
            x_v, g_v, wb_v, w_v, fa_v, gm_v,
            z_v, t_v, wp_v, xs_v, st_v, h_v, hf_v, gf_v, hk_v, gk_v, hr_v, gr_v,
            ws_v, raw_v, p_v, acco_v, acch_v, m_v, dw_v, sin, sout):
    ntc = S // TC
    nj = F // (2 * TF)
    ni = SH // TS
    nt = nj * ni
    assert ni == 4 and nt % 2 == 0
    part, chain = functools.partial, itertools.chain

    def loop(name, n, body, lo=0):
        with jax.named_scope(name):
            lax.fori_loop(lo, n, lambda i, carry: (body(i), carry)[1], 0)

    def blk(i, n):
        return pl.ds(i * n, n) if isinstance(i, int) else pl.ds(pl.multiple_of(i * n, n), n)

    def pace(vals, after):
        if not after:
            return vals
        rows, cols = vals[0].shape
        keep = _pk(fa_v[4, R2 - 16:, :]) == 0
        keep = jnp.tile(keep, (rows // 8, cols // R2))
        after = [o if o.shape[1] >= cols else jnp.tile(o, (1, cols // R2)) for o in after]
        marks = [(o, r) for o in after for r in range(0, o.shape[0], 8)]
        n = len(vals) * rows // 8
        marks = [lax.slice(o, (r, 0), (r + 8, cols))
                 for o, r in (marks[i * len(marks) // n] for i in range(n))]
        out = []
        for k, v in enumerate(vals):
            mark = jnp.concatenate(marks[k * rows // 8:(k + 1) * rows // 8], axis=0)
            if v.dtype != f32:
                mark = pltpu.bitcast(mark, v.dtype)
            out.append(lax.select(keep, v, mark))
        return out

    def pace16(v, after):
        return _up(pace([_pk(v)], after)[0])

    cp = pltpu.make_async_copy
    x_cp = lambda i: cp(x_h.at[:, blk(i, TC)], x_v.at[:, blk(i, TC)], sin.at[i])
    fa_cp = cp(fa_h, fa_v, sin.at[ntc])
    gm_cp = cp(gm_h, gm_v, sin.at[ntc + 1])
    g_cp = cp(g_h, g_v, sin.at[ntc + 2])
    w_cp = [cp(src.at[rows], wb_v.at[a, rows], sin.at[ntc + 3 + 2 * a + n])
            for a, src in enumerate((wr_h, wi_h))
            for n, rows in enumerate((pl.ds(0, KF - 1), pl.ds(KF - 1, 1)))]
    ffn_cp = [[cp(src.at[:, cols], w_v.at[m, :, cols], sin.at[ntc + 7 + 3 * n + m])
               for m, src in enumerate((wg_h, wu_h, wd_h))]
              for n, cols in enumerate((pl.ds(0, 2 * TF), pl.ds(2 * TF, 2 * TF),
                                        pl.ds(4 * TF, F - 4 * TF)))]
    dw_cp = lambda j: [cp(dw_v.at[j & 1, m], o.at[:, blk(j, 2 * TF)], sout.at[3 * (j & 1) + m])
                       for m, o in enumerate((dwg_h, dwu_h, dwd_h))]
    ob_v = w_v.at[0, :, pl.ds(0, S)]
    o_cp = [cp(w_v.at[0, :, blk(q, SH // 2)], out_h.at[:, blk(q, SH // 2)], sout.at[6 + q])
            for q in range(4)]
    dwf_cp = lambda rows, n: [cp(wb_v.at[a, rows], o.at[rows], sout.at[10 + ntc + 2 * n + a])
                              for a, o in enumerate((dwr_h, dwi_h))]
    dx_cp = lambda i: cp(g_v.at[:, blk(i, TC)], dx_h.at[:, blk(i, TC)], sout.at[10 + i])

    def dft_d(y):
        out = [_dot(fa_v[c], jnp.concatenate(y[2 * c:2 * c + 2], axis=0).astype(bf16))
               for c in range(4)]
        o0 = _dot(fa_v[4, :2 * (KP - K0), :DB], y[8].astype(bf16))
        return jnp.concatenate([o[:DB] for o in out] + [o0[:KP - K0]]
                               + [o[DB:] for o in out] + [o0[KP - K0:]], axis=0)

    def idft_d(z, last):
        y = []
        for c in range(4):
            zc = jnp.concatenate([z[DB * c:DB * c + DB], z[KP + DB * c:KP + DB * c + DB]], axis=0)
            o = _dot(fa_v[5 + c], zc.astype(bf16))
            y += [o[:DB], o[DB:]]
        zc = jnp.concatenate([z[K0:KP], z[KP + K0:]], axis=0)
        y.append(_dot(fa_v[last, :DB, :2 * (KP - K0)], zc.astype(bf16)))
        return y

    def radix_fwd(r, after=None):
        re, im = blk(r, 8), blk(r + KP // 8, 8)
        a = pace([z_v[re, n * R2:(n + 1) * R2] for n in range(R1)]
                 + [z_v[im, n * R2:(n + 1) * R2] for n in range(R1)], after)
        for k, (vr, vi) in enumerate(_fft16(list(zip(a[:R1], a[R1:])), -1)):
            t_v[k, re, :R2] = vr
            t_v[k, re, R2:] = vi

    def radix_inv(r, after=None):
        re, im = blk(r, 8), blk(r + KP // 8, 8)
        a = pace([t_v[n, re, :R2] for n in range(R1)]
                 + [t_v[n, re, R2:] for n in range(R1)], after)
        for k, (vr, vi) in enumerate(_fft16(list(zip(a[:R1], a[R1:])), 1)):
            z_v[re, k * R2:(k + 1) * R2] = vr
            z_v[im, k * R2:(k + 1) * R2] = vi

    def scale():
        k = lax.broadcasted_iota(jnp.int32, (KP, R2), 0)
        return jnp.where((k == K0) | (k == K0 + 32), 1.0 / (S * D), 2.0 / (S * D))

    def filt(k1):
        rows = [pl.ds(c, n, stride=RD) for _, c, n in _CLASSES + [(K0, 0, KP - K0)]]
        return [jnp.concatenate([wp_v[a, k1, r, :] for r in rows], axis=0) for a in range(2)]

    def spectrum(mix):
        prev = None
        for k1 in range(R1 + 1):
            if k1 < R1:
                a, b = t_v[k1, :, :R2], t_v[k1, :, R2:]
                n = [_dot(v.astype(bf16), gm_v[k1, e]) for e, v in enumerate((a + b, b, a))]
                cur = (n[0] - n[1], n[0] + n[2])
                yield n[2]
            if prev is not None:
                a, b = mix(k1 - 1, *prev)
                n = [_dot(v.astype(bf16), gm_v[k1 - 1, e], NT)
                     for e, v in enumerate((a + b, a, b))]
                t_v[k1 - 1, :, :R2] = n[0] + n[2]
                t_v[k1 - 1, :, R2:] = n[0] - n[1]
                yield n[2]
            prev = cur

    def mix_fwd(k1, xr, xi):
        cc = scale()
        xr, xi = xr * cc, xi * cc
        xs_v[k1, :, :R2] = _pk(xr)
        xs_v[k1, :, R2:] = _pk(xi)
        wr, wi = filt(k1)
        return [xr * wr - xi * wi, xr * wi + xi * wr]

    def mix_bwd(k1, dr, di):
        cc = scale()
        wr, wi = (w * cc for w in filt(k1))
        xr, xi = _up(xs_v[k1, :, :R2]).astype(f32), _up(xs_v[k1, :, R2:]).astype(f32)
        for a, v in enumerate((dr * xr + di * xi, di * xr - dr * xi)):
            for row, c, n in _CLASSES + [(K0, 0, 40)]:
                wp_v[a, k1, pl.ds(c, n, stride=RD), :] = v[row:row + n]
        return [dr * wr + di * wi, di * wr - dr * wi]

    def put_w(a, rr, w):
        w = _pk(w)
        tiles = _swap16(_rot16([w[:, t * R2:(t + 1) * R2] for t in range(R1)], 1))
        for k in range(R1):
            wp_v[a, k, rr, :] = _up(tiles[k]).astype(f32)

    def get_dw(a, rr):
        tiles = [_pk(wp_v[a, k, rr, :]) for k in range(R1)]
        return _up(jnp.concatenate(_rot16(_swap16(tiles), -1), axis=1))

    def pair(i):
        return blk(i, R2), blk(i + SH // R2, R2)

    def put_f(i, xa, xb, f_v):
        for r, v in enumerate(_act_forms(xa[:DH], xb[:DH], xa[DH:], xb[DH:])):
            f_v[r, :, blk(i, R2)] = _pk(v)

    def put_k(i, xa, xb, k_v, r_v):
        rows = blk(i, R2 // 2)
        f = list(_act_forms(xa[:KS].T, xb[:KS].T, xa[DH:DH + KS].T, xb[DH:DH + KS].T))
        ta, tb = [jnp.concatenate([x[KS:DH], x[DH + KS:]] * 2, axis=0).T for x in (xa, xb)]
        low = lax.broadcasted_iota(jnp.int32, (R2, R2), 1) < KA - R2
        hi = [v[:, R2:] for v in f]
        for r, v in ((1, ta), (2, -hi[3]), (3, -hi[2]), (4, tb)):
            f[r] = jnp.concatenate([f[r][:, :R2], jnp.where(low, hi[r], v)], axis=1)
        for r, v in enumerate(f):
            k_v[r, rows, :] = _pk(v)
        r_v[0, rows, :] = _pk(jnp.where(low, ta, -hi[1]))
        r_v[1, rows, :] = _pk(jnp.where(low, tb, -hi[4]))

    def grad_forms(i):
        ld = lambda after: [pace16(g_v[:, c], after).astype(f32) for c in pair(i)]
        return [lambda after: put_f(i, *ld(after), gf_v),
                lambda after: put_k(i, *ld(after), gk_v, gr_v)]

    def ffn_input(i):
        y = []

        def dots(after):
            y.extend(idft_d(jnp.concatenate([z_v[:, c] for c in pair(i)], axis=1), 9))

        def residual(half, after):
            c = pair(i)[half]
            groups = range(0, DB, 16)
            yy = pace([v[b:b + 16, half * R2:(half + 1) * R2] for b in groups for v in y], after)
            hs, mu, var = [], 0.0, 0.0
            for n, b in enumerate(groups):
                for a, d in enumerate(_rfft9_t(yy[RD * n:RD * n + RD])):
                    rows = slice(a * DB + b, a * DB + b + 16)
                    hs.append(x_v[rows, c].astype(f32) + d)
                    h_v[rows, c] = hs[-1]
                    mu = mu + hs[-1]
            mu = _colmean(mu)
            for h in hs:
                var = var + (h - mu) * (h - mu)
            st_v[2, :, c] = mu
            st_v[3, :, c] = 1.0 / jnp.sqrt(_colmean(var) + EPS)

        hn = lambda after: [(pace([h_v[:, c]], after)[0] - st_v[2, :, c]) * st_v[3, :, c]
                            for c in pair(i)]
        return [dots, part(residual, 0), part(residual, 1),
                lambda after: put_f(i, *hn(after), hf_v),
                lambda after: put_k(i, *hn(after), hk_v, hr_v)]

    def ffn_output(i):
        keep, y = {}, []

        def join(acc, after):
            n = [acc[r][:, blk(i, R2)] for r in range(7)]
            n[0], n[1], n[4] = pace([n[0], n[1], n[4]], after)
            return _act_join(n)

        def out(after):
            for o, c in zip(join(acco_v, after), pair(i)):
                ob_v[:, c] = (h_v[:, c] + o).astype(bf16)

        def stats(after):
            for half, (d, c) in enumerate(zip(join(acch_v, after), pair(i))):
                hn = (pace([h_v[:, c]], after)[0] - st_v[2, :, c]) * st_v[3, :, c]
                keep[half] = (d, hn, _colmean(d), _colmean(d * hn))

        def grad(half, after):
            c = pair(i)[half]
            d, hn, m1, m2 = keep[half]
            rows = [slice(a * DB + b, a * DB + b + 16) for b in range(0, DB, 16) for a in range(RD)]
            d, hn = pace([d[r] for r in rows], after), pace([hn[r] for r in rows], after)
            rstd, ys = st_v[3, :, c], []
            for n in range(0, len(rows), RD):
                dh = [g_v[rows[k], c].astype(f32) + rstd * (d[k] - m1 - hn[k] * m2)
                      for k in range(n, n + RD)]
                for r, v in zip(rows[n:n + RD], dh):
                    h_v[r, c] = v
                ys.append([v.astype(bf16) for v in _rfft9(dh)])
            y.append([jnp.concatenate(v, axis=0) for v in zip(*ys)])

        def dots(after):
            z = dft_d([jnp.concatenate(v, axis=1) for v in zip(*y)])
            for half, c in enumerate(pair(i)):
                z_v[:, c] = z[:, half * R2:(half + 1) * R2]

        return [out, stats, part(grad, 0), part(grad, 1), dots]

    def window(q):
        r0 = (min if isinstance(q, int) else jnp.minimum)(q * (WIN // 16), (DH - WIN) // 16)
        hint = (lambda v, n: v) if isinstance(q, int) else pl.multiple_of
        return (pl.ds(hint(r0 * 16, 16), WIN), pl.ds(hint(r0 * 16 + DH, 16), WIN),
                pl.ds(hint(r0 * 8, 8), WIN // 2))

    def mod3(j):
        return j % 3 if isinstance(j, int) else lax.rem(j, 3)

    def wprep(j, q, r, after=None):
        src = j if isinstance(j, int) else jnp.minimum(j, nj - 1)
        f1, f2 = blk(2 * src, TF), blk(2 * src + 1, TF)
        d1, d2, dst = window(q)
        for m in range(3):
            ld = lambda d, f: lambda: pace16(w_v[m, d, f], after)
            form = _wgt_forms(ld(d1, f1), ld(d1, f2), ld(d2, f1), ld(d2, f2))[r]
            ws_v[m][r][mod3(j), dst, :] = _pk(form())

    def wform(j, m, r, n):
        return _up(ws_v[m][r][mod3(j), 0:n // 2, :])

    def finalize(j, q, m, after=None):
        d1, d2, _ = window(q)
        n = [pace([m_v[m][r][j & 1, d1, :]], after if r < 4 else None)[0] for r in range(7)]
        dw_v[j & 1, m, d1, :TF] = (n[0] + n[3] - n[4] + n[6]).astype(bf16)
        dw_v[j & 1, m, d1, TF:] = (n[2] + n[4]).astype(bf16)
        dw_v[j & 1, m, d2, :TF] = (n[1] + n[3]).astype(bf16)
        dw_v[j & 1, m, d2, TF:] = (n[0] - n[1] + n[2] + n[5]).astype(bf16)

    def stage1(t, b, ms):
        j, ss = t >> 2, blk(t & 3, TS // 2)
        f1, f2 = blk(2 * j, TF), blk(2 * j + 1, TF)
        rows = part(jnp.concatenate, axis=0)
        zero = jnp.zeros((KS - KA, TF), bf16)
        for m in ms:
            k_v, r_v = (gk_v, gr_v) if m == 2 else (hk_v, hr_v)
            v1, v2 = [[w_v[m, KS:DH, f], w_v[m, DH + KS:, f]] for f in (f1, f2)]
            w12, w21 = w_v[m, KA:KS, f2], w_v[m, DH + KA:DH + KS, f1]
            q = lambda r, tail: _dot(_up(k_v[r, ss, :]), rows([wform(j, m, r, KA)] + tail))
            mid = lambda r: [_up(ws_v[m][r][mod3(j), KA // 2:KS // 2, :])]
            q2 = q(2, mid(2))
            yield q2
            q5 = q(5, [w21])
            yield q5
            a7, w7 = _up(k_v[0, ss, R2:]), rows([zero, w12 + w21])
            if m == ms[-1] and len(ms) % 2:
                q7 = rows([_dot(a7[:TS // 2], w7), _dot(a7[TS // 2:], w7)])
            else:
                q7 = _dot(a7, w7)
            raw_v[b][m, 1] = q2 + q5 + q7 + _dot(_up(r_v[0, ss, :]), rows(v2 + mid(1)))
            q3 = q(3, mid(3))
            yield q3
            q6 = q(6, [w12])
            yield q6
            raw_v[b][m, 2] = q3 + q7 + q6 + _dot(_up(r_v[1, ss, :]), rows(v1 + mid(4)))
            q0 = q(0, [zero])
            yield q0
            q1 = q(1, v1)
            raw_v[b][m, 0] = (q0 + q5 - q3) + q1
            yield q1
            q4 = q(4, v2)
            raw_v[b][m, 3] = (q0 - q2 + q6) + q4
            yield q4

    def gate(b, r0, after):
        rows, prows = slice(r0, r0 + EW), slice(r0 // 2, (r0 + EW) // 2)
        res = ([], [], [])
        pre = pace([raw_v[b][0, q, rows] for q in range(4)], after)
        for q in range(4):
            a, u, dp = pre[q], raw_v[b][1, q, rows], raw_v[b][2, q, rows]
            sg = jax.nn.sigmoid(a)
            sl = a * sg
            res[0].append(dp * u * (sg + sl * (1.0 - sg)))
            res[1].append(dp * sl)
            res[2].append(sl * u)
        for m in range(3):
            for r, v in enumerate(_hid_forms(*res[m])):
                p_v[b][m, r, prows, :] = _pk(v)

    gates = lambda b: [part(gate, b, r0) for r0 in range(0, TS, EW)]

    def stage2(t, b, acts=True, wgts=True):
        j, i = t >> 2, t & 3
        ss = blk(i, TS)
        for r in range(7):
            if acts:
                o = _dot(wform(j, 2, r, DH), _up(p_v[b][2, r]), NT)
                acco_v[r][:, ss] = jnp.where(j == 0, 0.0, acco_v[r][:, ss]) + o
                yield o
                o = (_dot(wform(j, 0, r, DH), _up(p_v[b][0, r]), NT)
                     + _dot(wform(j, 1, r, DH), _up(p_v[b][1, r]), NT))
                acch_v[r][:, ss] = jnp.where(j == 0, 0.0, acch_v[r][:, ss]) + o
                yield o
            if wgts:
                for m, f_v in enumerate((hf_v, hf_v, gf_v)):
                    o = _dot(_up(f_v[r, :, ss]), _up(p_v[b][m, r]))
                    m_v[m][r][j & 1] = jnp.where(i == 0, 0.0, m_v[m][r][j & 1]) + o
                    yield o

    fins = lambda j, q: [part(finalize, j, q, m) for m in range(3)]
    preps = lambda j, q: [part(wprep, j, q, r) for r in range(7)]
    cat = lambda lists: list(chain(*lists))

    for c in ([x_cp(0), fa_cp] + [x_cp(i) for i in range(1, ntc)] + w_cp + [gm_cp, g_cp]
              + cat(ffn_cp)):
        c.start()
    for a in range(2):
        for k in range(R1):
            wp_v[a, k, pl.ds(RD * 34, KP - K0 - 34, stride=RD), :] = jnp.zeros(
                (KP - K0 - 34, R2), f32)
    fa_cp.wait()

    def p1(i):
        c = blk(i, TC)
        ys, en = [], 0.0
        for b in range(0, DB, 16):
            y = _rfft9([x_v[a * DB + b:a * DB + b + 16, c].astype(f32) for a in range(RD)])
            sq = [v * v for v in y[:8]]
            en = en + 0.75 * sq[5] + (sq[0] + sq[1] + sq[2] + sq[3] + sq[4] + sq[6] + sq[7])
            ys.append([v.astype(bf16) for v in y[:8]] + [y[8]])
        y = [jnp.concatenate(v, axis=0) for v in zip(*ys)]
        mu = _colmean(y[8])
        y[8] = y[8] - RD * mu
        var = (_colmean(y[8] * y[8]) + 2.0 * _colmean(en)) * (1.0 / RD)
        rstd = 1.0 / jnp.sqrt(var + EPS)
        st_v[0, :, c] = mu
        st_v[1, :, c] = rstd
        z_v[:, c] = dft_d(y) * rstd

    def p1s(n):
        for i in range(UN):
            x_cp(UN * n + i).wait()
        for i in range(UN):
            p1(UN * n + i)
    loop("p1", ntc // UN, p1s)
    loop("radix", KP // 16, lambda r: (radix_fwd(2 * r), radix_fwd(2 * r + 1)))
    for m in range(3):
        for r in range(7):
            m_v[m][r][1] = jnp.zeros((DH, TF), f32)

    for c in w_cp:
        c.wait()

    def pw(r):
        for a in range(2):
            put_w(a, blk(r, 32), wb_v[a, blk(r, 32), :])
    loop("pw", (KF - 1) // 32, pw)
    row = lax.broadcasted_iota(jnp.int32, (16, S), 0)
    for a in range(2):
        last = jnp.broadcast_to(wb_v[a, KF - 1:KF, :].astype(f32), (16, S))
        put_w(a, slice(KF - 1, KP), jnp.where(row == 0, last, 0.0))

    gm_cp.wait()
    with jax.named_scope("p3"):
        _overlap(spectrum(mix_fwd),
                 ([lambda after: g_cp.wait()] + cat(grad_forms(i) for i in range(5)), 11, 31))
    loop("radix", KP // 16, lambda r: (radix_inv(2 * r), radix_inv(2 * r + 1)))
    for c in ffn_cp[0]:
        c.wait()
    for m in range(3):
        for r0 in range(0, DH, 16):
            blocks = [w_v[m, d + r0:d + r0 + 16, f:f + TF].astype(f32)
                      for d in (0, DH) for f in (0, TF)]
            for r, form in enumerate(_wgt_forms(*[lambda v=v: v for v in blocks])):
                ws_v[m][r][0, r0 // 2:r0 // 2 + 8, :] = _pk(form())

    with jax.named_scope("head"):
        _overlap(chain(stage1(0, 0, (2,)), stage1(1, 1, (2,))),
                 (cat(ffn_input(i) for i in (0, 1)), 0, 12))
        _overlap(stage1(0, 0, (0, 1)), (cat(ffn_input(i) for i in (2, 3)), 0, 13))
        for c in ffn_cp[1]:
            c.wait()
        _overlap(stage1(1, 1, (0, 1)), (gates(0), 0, 12),
                 (preps(1, 0) + preps(1, 1), 0, 13))

    def step(t, b, *tasks):
        if not tasks:
            tasks = ((fins(((t - 1) >> 2) + 1, (t - 1) & 3), 49, 55),
                     (preps(((t + 1) >> 2) + 1, (t + 1) & 3), 35, 48))
        _overlap(chain(stage2(t - 1, 1 - b), stage1(t + 1, 1 - b, (0, 1, 2))),
                 (gates(b), 1, 32), *tasks)

    with jax.named_scope("head2"):
        in6 = ffn_input(6)
        step(1, 1, (ffn_input(4) + ffn_input(5) + grad_forms(5) + in6[:1], 1, 33),
             (in6[1:] + ffn_input(7) + preps(1, 2) + grad_forms(6) + grad_forms(7),
              34, 54))
    for c in ffn_cp[2]:
        c.wait()

    def body(n):
        j = n >> 1

        @pl.when(((n & 1) == 0) & (j >= 3))
        def _():
            for c in dw_cp(j - 3):
                c.wait()

        @pl.when(((n & 1) == 1) & (j >= 2))
        def _():
            for c in dw_cp(j - 2):
                c.start()
        step(2 * n, 0)
        step(2 * n + 1, 1)
    loop("ffn", nt // 2 - 1, body, 1)
    for c in dw_cp(nj - 3):
        c.start()

    with jax.named_scope("tail"):
        step(nt - 2, 0, (ffn_output(0) + ffn_output(1), 1, 34),
             (ffn_output(2) + ffn_output(3), 35, 54))
        o_cp[0].start()
        o_cp[2].start()
        _overlap(chain(stage2(nt - 2, 0, wgts=False), stage2(nt - 2, 0, acts=False)),
                 (gates(1), 1, 32), (ffn_output(4) + ffn_output(5), 14, 33),
                 (fins(nj - 2, 1), 0, 13))
        _overlap(chain(stage2(nt - 1, 1, wgts=False), stage2(nt - 1, 1, acts=False)),
                 (fins(nj - 2, 2) + fins(nj - 2, 3)
                  + [lambda after: [c.start() for c in dw_cp(nj - 2)]
                     + [c.wait() for c in dw_cp(nj - 3)]], 0, 13),
                 (ffn_output(6) + ffn_output(7), 14, 25),
                 ([part(radix_fwd, r) for r in range(KP // 8)], 26, 34))
    for c in (o_cp[1], o_cp[3]):
        c.start()

    with jax.named_scope("p9"):
        _overlap(spectrum(mix_bwd),
                 (cat(fins(nj - 1, q) for q in range(ni))
                  + [lambda after: [c.start() for c in dw_cp(nj - 1)]], 0, 12))

    def pdw(r):
        for a in range(2):
            wb_v[a, blk(r, 32), :] = get_dw(a, blk(r, 32))
            radix_inv(4 * r + 2 * a)
            radix_inv(4 * r + 2 * a + 1)
        for c in dwf_cp(blk(r, 32), r):
            c.start()
    loop("pdw", (KF - 1) // 32, pdw)
    for a in range(2):
        wb_v[a, KF - 1:KF, :] = get_dw(a, slice(KF - 1, KP)).astype(f32)[0:1].astype(bf16)
        radix_inv((KF - 1) // 8 + a)
    dwf_all = [dwf_cp(blk(r, 32), r) for r in range(9)] + [dwf_cp(pl.ds(KF - 1, 1), 9)]
    for c in dwf_all[-1]:
        c.start()

    def p11(i):
        c = blk(i, R2)
        y = idft_d(z_v[:, c], 10)
        mu, rstd = st_v[0, :, c], st_v[1, :, c]
        proj = 0.0
        for b in range(0, DB, 16):
            for a, d in enumerate(_rfft9_t([v[b:b + 16] for v in y])):
                rows = slice(a * DB + b, a * DB + b + 16)
                proj = proj + d * (x_v[rows, c].astype(f32) - mu)
                h_v[rows, c] += rstd * d
        proj = _colmean(proj) * rstd * rstd * rstd
        for r in range(0, D, 16):
            g_v[r:r + 16, c] = (h_v[r:r + 16, c]
                                - (x_v[r:r + 16, c].astype(f32) - mu) * proj).astype(bf16)

    for lo, hi in ((0, 2), (2, 4), (4, 6), (6, 7), (7, 8)):
        with jax.named_scope("p11"):
            for i in range(lo * TC // R2, hi * TC // R2):
                p11(i)
        for i in range(lo, hi):
            dx_cp(i).start()

    for c in (dw_cp(nj - 2) + dw_cp(nj - 1) + o_cp + cat(dwf_all)
              + [dx_cp(i) for i in range(ntc)]):
        c.wait()


@jax.jit
def pallas_sequential_preLN__spectral_gfnet__swiglu_ffn__prompt_kernel(
    A_x: jax.Array,
    A_w_r: jax.Array,
    A_w_i: jax.Array,
    B_x: jax.Array,
    B_w_gate: jax.Array,
    B_w_up: jax.Array,
    B_w_down: jax.Array,
    grad_out: jax.Array,
):
    del B_x
    sds = jax.ShapeDtypeStruct
    hbm = pl.BlockSpec(memory_space=pltpu.HBM)
    out, dx, dwr, dwi, dwg, dwu, dwd = pl.pallas_call(
        _kernel,
        out_shape=[sds((D, S), bf16), sds((D, S), bf16),
                   sds((KF, S), bf16), sds((KF, S), bf16),
                   sds((D, F), bf16), sds((D, F), bf16), sds((D, F), bf16)],
        in_specs=[hbm] * 9,
        out_specs=[hbm] * 7,
        scratch_shapes=[
            V((D, S), bf16), V((D, S), bf16), V((2, KF, S), bf16), V((3, D, F), bf16),
            V((11, R2, R2), bf16), V((R1, 3, R2, R2), bf16),
            V((2 * KP, S), f32), V((R1, KP, 2 * R2), f32),
            V((2, R1, RD * (KP - K0), R2), f32), V((R1, KP // 2, 2 * R2), u32),
            V((4, 1, S), f32), V((D, S), f32),
            V((7, DH // 2, SH), u32), V((7, DH // 2, SH), u32),
            V((7, SH // 2, KS), u32), V((7, SH // 2, KS), u32),
            V((2, SH // 2, R2), u32), V((2, SH // 2, R2), u32),
            [[V((3, DH // 2, TF), u32)] * 7] * 3, [V((3, 4, TS, TF), f32)] * 2,
            [V((3, 7, TS // 2, TF), u32)] * 2,
            [V((DH, SH), f32)] * 7, [V((DH, SH), f32)] * 7, [[V((2, DH, TF), f32)] * 7] * 3,
            V((2, 3, D, 2 * TF), bf16),
            pltpu.SemaphoreType.DMA((S // TC + 16,)),
            pltpu.SemaphoreType.DMA((30 + S // TC,)),
        ],
        compiler_params=pltpu.CompilerParams(vmem_limit_bytes=127 * 2**20),
    )(A_x[0].T, A_w_r.T, A_w_i.T, B_w_gate, B_w_up, B_w_down.T, grad_out[0].T,
      _FA, _G)
    return out.T[None], dx.T[None], dwr.T, dwi.T, dwg, dwu, dwd.T
```

```python
import functools
import itertools
import math

import jax
import jax.numpy as jnp
import ml_dtypes
import numpy as np
from jax import lax
from jax.experimental import pallas as pl
from jax.experimental.pallas import tpu as pltpu

S, D, F = 2048, 576, 4608
KF = D // 2 + 1
KP = 304
R1, R2 = 16, 128
RD, DB = 9, 64
K0 = 256
EPS = 1e-5
DH, SH = D // 2, S // 2
KA, KS = 192, 256
TS = 256
TF = 256
UN = 2
EW = 16
WIN = 80
TC = 256

bf16 = jnp.bfloat16
f32 = jnp.float32
u32 = jnp.uint32
V = pltpu.VMEM
NN = (((1,), (0,)), ((), ()))
NT = (((1,), (1,)), ((), ()))


_C1, _C2, _C4 = (math.cos(2 * math.pi * e / RD) for e in (1, 2, 4))
_S1, _S2, _S3, _S4 = (math.sin(2 * math.pi * e / RD) for e in (1, 2, 3, 4))


def _cyc(m, a, b, c, k1, k2, k3):
    e1, e2 = a - c, b - c
    p, q = k1 * e1 + k2 * e2, k2 * e1 + k3 * e2
    return m + p, m + q, m - (p + q)


def _cyc_t(o1, o2, o3, k1, k2, k3):
    p, q = o1 - o3, o2 - o3
    e1, e2 = k1 * p + k2 * q, k2 * p + k3 * q
    return o1 + o2 + o3, e1, e2, -(e1 + e2)


def _rfft9(x):
    s1, s2, s3, s4 = (x[a] + x[RD - a] for a in (1, 2, 3, 4))
    t1, t2, t3, t4 = x[1] - x[8], x[7] - x[2], x[3] - x[6], x[4] - x[5]
    u, v = x[0] + s3, s1 + s2 + s4
    p1, p2, p4 = _cyc(x[0] - 0.5 * s3, s1, s2, s4, _C1, _C2, _C4)
    q1, q2, q4 = _cyc(_S3 * t3, t1, t2, t4, _S1, -_S2, _S4)
    return [p1, q1, p2, q2, u - 0.5 * v, t1 + t2 + t4, p4, q4, u + v]


def _rfft9_t(y):
    p1, q1, p2, q2, p3, q3, p4, q4, y0 = y
    m, s1, s2, s4 = _cyc_t(p1, p2, p4, _C1, _C2, _C4)
    n, t1, t2, t4 = _cyc_t(q1, q2, q4, _S1, -_S2, _S4)
    u, v = y0 + p3, y0 - 0.5 * p3
    s1, s2, s4, s3 = s1 + v, s2 + v, s4 + v, u - 0.5 * m
    t1, t2, t4, t3 = t1 + q3, t2 + q3, t4 + q3, _S3 * n
    return [u + m, s1 + t1, s2 - t2, s3 + t3, s4 + t4, s4 - t4, s3 - t3, s2 + t2, s1 - t1]


_CLASSES = [(64 * (c - 1) + 32 * h, (c, RD - c)[h], 32) for c in (1, 2, 3, 4) for h in (0, 1)]


def _consts():
    root = lambda e, n: np.exp(-2j * np.pi * (e % n) / n)
    bins = np.full(KP, -1)
    for row, c, n in _CLASSES + [(K0, 0, 33)]:
        bins[row:row + n] = c + RD * np.arange(n)
    r9 = np.stack(_rfft9(list(np.eye(RD))))
    r9 = r9 / (r9 * r9).sum(1, keepdims=True)
    coef = (root(bins[:, None, None] * np.arange(RD), RD) * r9).sum(-1)
    full = coef[:, :, None] * root(bins[:, None, None] * np.arange(DB), D)
    full = full.reshape(KP, D) * (bins >= 0)[:, None]
    fa = np.zeros((11, R2, R2))
    for c in range(5):
        blk = full[DB * c:min(DB * c + DB, KP), R2 * c:R2 * c + R2]
        fa[c, :2 * blk.shape[0], :blk.shape[1]] = np.concatenate([blk.real, blk.imag])
        fa[5 + c] = fa[c].T
    fa[10] = fa[9]
    fa[10, :, 0] = 0.0
    k1 = np.arange(R1)[:, None, None]
    lane = (np.arange(R2) - k1) % R2
    k2 = 8 * (lane % 16) + lane // 16
    g = root(np.arange(R2)[:, None] * (k1 + R1 * k2), S)
    g = np.stack([g.real, g.real + g.imag, g.imag - g.real], 1)
    cast = lambda a: (np.round(a, 9) + 0.0).astype(np.float32).astype(ml_dtypes.bfloat16)
    return cast(fa), cast(g)


_FA, _G = _consts()


def _dot(a, b, dn=NN):
    return lax.dot_general(a, b, dn, preferred_element_type=f32)


def _fft4(x, sign):
    (ar, ai), (br, bi), (cr, ci), (dr, di) = x
    s0r, s0i, d0r, d0i = ar + cr, ai + ci, ar - cr, ai - ci
    s1r, s1i, d1r, d1i = br + dr, bi + di, br - dr, bi - di
    lo = (d0r + d1i, d0i - d1r)
    hi = (d0r - d1i, d0i + d1r)
    o1, o3 = (lo, hi) if sign < 0 else (hi, lo)
    return [(s0r + s1r, s0i + s1i), o1, (s0r - s1r, s0i - s1i), o3]


def _tw16(v, e, sign):
    r, i = v
    e %= 16
    if e == 0:
        return v
    if e == 4:
        return (i, -r) if sign < 0 else (-i, r)
    c = math.cos(2 * math.pi * e / 16)
    s = sign * math.sin(2 * math.pi * e / 16)
    if e % 2 == 0:
        if c * s > 0:
            return ((r - i) * c, (r + i) * c)
        return ((r + i) * c, (i - r) * c)
    return (r * c - i * s, r * s + i * c)


def _fft16(x, sign):
    cols = [_fft4([x[4 * a + b] for a in range(4)], sign) for b in range(4)]
    out = [None] * 16
    for p in range(4):
        o = _fft4([_tw16(cols[b][p], b * p, sign) for b in range(4)], sign)
        for q in range(4):
            out[p + 4 * q] = o[q]
    return out


def _swap16(tiles):
    lane = lax.broadcasted_iota(jnp.int32, tiles[0].shape, 1)
    tiles = list(tiles)
    for d in (1, 2, 4, 8):
        for lo in range(d):
            low = ((lane - lo) & d) == 0
            for t in range(lo, R1, 2 * d):
                a, b = tiles[t], tiles[t + d]
                tiles[t], tiles[t + d] = jnp.where(low, a, b), jnp.where(low, b, a)
    return tiles


def _rot16(tiles, sign):
    return [pltpu.roll(v, (sign * t) % R2, 1) if t else v for t, v in enumerate(tiles)]


def _act_forms(a11, a12, a21, a22):
    return (a11 + a22, a21 + a22, a11, a22, a11 + a12, a21 - a11, a12 - a22)


def _hid_forms(p11, p12, p21, p22):
    return (p11 + p22, p11, p12 - p22, p21 - p11, p22, p11 + p12, p21 + p22)


def _wgt_forms(w11, w12, w21, w22):
    return (lambda: w11() + w22(), lambda: w21() - w22(), lambda: w12() + w22(),
            lambda: w11() + w21(), lambda: w12() - w11(), w22, w11)


def _act_join(n):
    return (n[0] + n[2] + n[4] - n[5], n[4] + n[6], n[1] + n[5], n[0] + n[1] + n[3] - n[6])


def _pk(v):
    return pltpu.bitcast(v.astype(bf16), u32)


def _up(v):
    return pltpu.bitcast(v, bf16)


def _colmean(x):
    return jnp.sum(x, axis=0, keepdims=True) * (1.0 / D)


def _overlap(dots, *tasks):
    plan = [(first + s * (last - first + 1) // len(steps),
             -(-(last - first + 1) // len(steps)), step)
            for steps, first, last in tasks for s, step in enumerate(steps)]
    seen = []
    for k, o in enumerate(dots):
        seen.append(o)
        for at, span, step in plan:
            if at == k:
                step(seen[-span:])
    assert all(at < len(seen) for at, _, _ in plan)


def _kernel(x_h, wr_h, wi_h, wg_h, wu_h, wd_h, g_h, fa_h, gm_h,
            out_h, dx_h, dwr_h, dwi_h, dwg_h, dwu_h, dwd_h,
            x_v, g_v, wb_v, w_v, fa_v, gm_v,
            z_v, t_v, wp_v, xs_v, st_v, h_v, hf_v, gf_v, hk_v, gk_v, hr_v, gr_v,
            ws_v, raw_v, p_v, acco_v, acch_v, m_v, dw_v, sin, sout):
    ntc = S // TC
    nj = F // (2 * TF)
    ni = SH // TS
    nt = nj * ni
    assert ni == 4 and nt % 2 == 0
    part, chain = functools.partial, itertools.chain

    def loop(name, n, body, lo=0):
        with jax.named_scope(name):
            lax.fori_loop(lo, n, lambda i, carry: (body(i), carry)[1], 0)

    def blk(i, n):
        return pl.ds(i * n, n) if isinstance(i, int) else pl.ds(pl.multiple_of(i * n, n), n)

    def pace(vals, after):
        if not after:
            return vals
        rows, cols = vals[0].shape
        keep = _pk(fa_v[4, R2 - 16:, :]) == 0
        keep = jnp.tile(keep, (rows // 8, cols // R2))
        after = [o if o.shape[1] >= cols else jnp.tile(o, (1, cols // R2)) for o in after]
        marks = [(o, r) for o in after for r in range(0, o.shape[0], 8)]
        n = len(vals) * rows // 8
        marks = [lax.slice(o, (r, 0), (r + 8, cols))
                 for o, r in (marks[i * len(marks) // n] for i in range(n))]
        out = []
        for k, v in enumerate(vals):
            mark = jnp.concatenate(marks[k * rows // 8:(k + 1) * rows // 8], axis=0)
            if v.dtype != f32:
                mark = pltpu.bitcast(mark, v.dtype)
            out.append(lax.select(keep, v, mark))
        return out

    def pace16(v, after):
        return _up(pace([_pk(v)], after)[0])

    cp = pltpu.make_async_copy
    x_cp = lambda i: cp(x_h.at[:, blk(i, TC)], x_v.at[:, blk(i, TC)], sin.at[i])
    fa_cp = cp(fa_h, fa_v, sin.at[ntc])
    gm_cp = cp(gm_h, gm_v, sin.at[ntc + 1])
    g_cp = cp(g_h, g_v, sin.at[ntc + 2])
    w_cp = [cp(src.at[rows], wb_v.at[a, rows], sin.at[ntc + 3 + 2 * a + n])
            for a, src in enumerate((wr_h, wi_h))
            for n, rows in enumerate((pl.ds(0, KF - 1), pl.ds(KF - 1, 1)))]
    ffn_cp = [[cp(src.at[:, cols], w_v.at[m, :, cols], sin.at[ntc + 7 + 3 * n + m])
               for m, src in enumerate((wg_h, wu_h, wd_h))]
              for n, cols in enumerate((pl.ds(0, 2 * TF), pl.ds(2 * TF, 2 * TF),
                                        pl.ds(4 * TF, F - 4 * TF)))]
    dw_cp = lambda j: [cp(dw_v.at[j & 1, m], o.at[:, blk(j, 2 * TF)], sout.at[3 * (j & 1) + m])
                       for m, o in enumerate((dwg_h, dwu_h, dwd_h))]
    ob_v = w_v.at[0, :, pl.ds(0, S)]
    o_cp = [cp(w_v.at[0, :, blk(q, SH // 2)], out_h.at[:, blk(q, SH // 2)], sout.at[6 + q])
            for q in range(4)]
    dwf_cp = lambda rows, n: [cp(wb_v.at[a, rows], o.at[rows], sout.at[10 + ntc + 2 * n + a])
                              for a, o in enumerate((dwr_h, dwi_h))]
    dx_cp = lambda i: cp(g_v.at[:, blk(i, TC)], dx_h.at[:, blk(i, TC)], sout.at[10 + i])

    def dft_d(y):
        out = [_dot(fa_v[c], jnp.concatenate(y[2 * c:2 * c + 2], axis=0).astype(bf16))
               for c in range(4)]
        o0 = _dot(fa_v[4, :2 * (KP - K0), :DB], y[8].astype(bf16))
        return jnp.concatenate([o[:DB] for o in out] + [o0[:KP - K0]]
                               + [o[DB:] for o in out] + [o0[KP - K0:]], axis=0)

    def idft_d(z, last):
        y = []
        for c in range(4):
            zc = jnp.concatenate([z[DB * c:DB * c + DB], z[KP + DB * c:KP + DB * c + DB]], axis=0)
            o = _dot(fa_v[5 + c], zc.astype(bf16))
            y += [o[:DB], o[DB:]]
        zc = jnp.concatenate([z[K0:KP], z[KP + K0:]], axis=0)
        y.append(_dot(fa_v[last, :DB, :2 * (KP - K0)], zc.astype(bf16)))
        return y

    def radix_fwd(r, after=None):
        re, im = blk(r, 8), blk(r + KP // 8, 8)
        a = pace([z_v[re, n * R2:(n + 1) * R2] for n in range(R1)]
                 + [z_v[im, n * R2:(n + 1) * R2] for n in range(R1)], after)
        for k, (vr, vi) in enumerate(_fft16(list(zip(a[:R1], a[R1:])), -1)):
            t_v[k, re, :R2] = vr
            t_v[k, re, R2:] = vi

    def radix_inv(r, after=None):
        re, im = blk(r, 8), blk(r + KP // 8, 8)
        a = pace([t_v[n, re, :R2] for n in range(R1)]
                 + [t_v[n, re, R2:] for n in range(R1)], after)
        for k, (vr, vi) in enumerate(_fft16(list(zip(a[:R1], a[R1:])), 1)):
            z_v[re, k * R2:(k + 1) * R2] = vr
            z_v[im, k * R2:(k + 1) * R2] = vi

    def scale():
        k = lax.broadcasted_iota(jnp.int32, (KP, R2), 0)
        return jnp.where((k == K0) | (k == K0 + 32), 1.0 / (S * D), 2.0 / (S * D))

    def filt(k1):
        rows = [pl.ds(c, n, stride=RD) for _, c, n in _CLASSES + [(K0, 0, KP - K0)]]
        return [jnp.concatenate([wp_v[a, k1, r, :] for r in rows], axis=0) for a in range(2)]

    def spectrum(mix):
        prev = None
        for k1 in range(R1 + 1):
            if k1 < R1:
                a, b = t_v[k1, :, :R2], t_v[k1, :, R2:]
                n = [_dot(v.astype(bf16), gm_v[k1, e]) for e, v in enumerate((a + b, b, a))]
                cur = (n[0] - n[1], n[0] + n[2])
                yield n[2]
            if prev is not None:
                a, b = mix(k1 - 1, *prev)
                n = [_dot(v.astype(bf16), gm_v[k1 - 1, e], NT)
                     for e, v in enumerate((a + b, a, b))]
                t_v[k1 - 1, :, :R2] = n[0] + n[2]
                t_v[k1 - 1, :, R2:] = n[0] - n[1]
                yield n[2]
            prev = cur

    def mix_fwd(k1, xr, xi):
        cc = scale()
        xr, xi = xr * cc, xi * cc
        xs_v[k1, :, :R2] = _pk(xr)
        xs_v[k1, :, R2:] = _pk(xi)
        wr, wi = filt(k1)
        return [xr * wr - xi * wi, xr * wi + xi * wr]

    def mix_bwd(k1, dr, di):
        cc = scale()
        wr, wi = (w * cc for w in filt(k1))
        xr, xi = _up(xs_v[k1, :, :R2]).astype(f32), _up(xs_v[k1, :, R2:]).astype(f32)
        for a, v in enumerate((dr * xr + di * xi, di * xr - dr * xi)):
            for row, c, n in _CLASSES + [(K0, 0, 40)]:
                wp_v[a, k1, pl.ds(c, n, stride=RD), :] = v[row:row + n]
        return [dr * wr + di * wi, di * wr - dr * wi]

    def put_w(a, rr, w):
        w = _pk(w)
        tiles = _swap16(_rot16([w[:, t * R2:(t + 1) * R2] for t in range(R1)], 1))
        for k in range(R1):
            wp_v[a, k, rr, :] = _up(tiles[k]).astype(f32)

    def get_dw(a, rr):
        tiles = [_pk(wp_v[a, k, rr, :]) for k in range(R1)]
        return _up(jnp.concatenate(_rot16(_swap16(tiles), -1), axis=1))

    def pair(i):
        return blk(i, R2), blk(i + SH // R2, R2)

    def put_f(i, load, f_v, after):
        groups = range(0, DH, 16)
        blocks = load([(slice(d + r, d + r + 16), half)
                       for r in groups for d in (0, DH) for half in range(2)], after)
        for n, r0 in enumerate(groups):
            for r, v in enumerate(_act_forms(*blocks[4 * n:4 * n + 4])):
                f_v[r, r0 // 2:r0 // 2 + 8, blk(i, R2)] = _pk(v)

    def put_k(i, xa, xb, k_v, r_v):
        rows = blk(i, R2 // 2)
        f = list(_act_forms(xa[:KS].T, xb[:KS].T, xa[DH:DH + KS].T, xb[DH:DH + KS].T))
        ta, tb = [jnp.concatenate([x[KS:DH], x[DH + KS:]] * 2, axis=0).T for x in (xa, xb)]
        low = lax.broadcasted_iota(jnp.int32, (R2, R2), 1) < KA - R2
        hi = [v[:, R2:] for v in f]
        for r, v in ((1, ta), (2, -hi[3]), (3, -hi[2]), (4, tb)):
            f[r] = jnp.concatenate([f[r][:, :R2], jnp.where(low, hi[r], v)], axis=1)
        for r, v in enumerate(f):
            k_v[r, rows, :] = _pk(v)
        r_v[0, rows, :] = _pk(jnp.where(low, ta, -hi[1]))
        r_v[1, rows, :] = _pk(jnp.where(low, tb, -hi[4]))

    whole = [(slice(0, D), 0), (slice(0, D), 1)]

    def grad_forms(i):
        def load(where, after):
            vals = pace([_pk(g_v[rows, pair(i)[half]]) for rows, half in where], after)
            return [_up(v).astype(f32) for v in vals]
        return [part(put_f, i, load, gf_v),
                lambda after: put_k(i, *load(whole, after), gk_v, gr_v)]

    def ffn_input(i):
        y = []

        def dots(after):
            y.extend(idft_d(jnp.concatenate([z_v[:, c] for c in pair(i)], axis=1), 9))

        def residual(half, after):
            c = pair(i)[half]
            groups = range(0, DB, 16)
            yy = pace([v[b:b + 16, half * R2:(half + 1) * R2] for b in groups for v in y], after)
            hs, mu, var = [], 0.0, 0.0
            for n, b in enumerate(groups):
                for a, d in enumerate(_rfft9_t(yy[RD * n:RD * n + RD])):
                    rows = slice(a * DB + b, a * DB + b + 16)
                    hs.append(x_v[rows, c].astype(f32) + d)
                    h_v[rows, c] = hs[-1]
                    mu = mu + hs[-1]
            mu = _colmean(mu)
            for h in hs:
                var = var + (h - mu) * (h - mu)
            st_v[2, :, c] = mu
            st_v[3, :, c] = 1.0 / jnp.sqrt(_colmean(var) + EPS)

        def load(where, after):
            stat = [(st_v[2, :, c], st_v[3, :, c]) for c in pair(i)]
            vals = pace([h_v[rows, pair(i)[half]] for rows, half in where], after)
            return [(v - stat[half][0]) * stat[half][1] for v, (_, half) in zip(vals, where)]

        return [dots, part(residual, 0), part(residual, 1), part(put_f, i, load, hf_v),
                lambda after: put_k(i, *load(whole, after), hk_v, hr_v)]

    def ffn_output(i):
        dn, sums, y = ({}, {}), [[0.0, 0.0], [0.0, 0.0]], []

        def join(acc, after):
            groups = range(0, DH, 16)
            first = pace([acc[r][r0:r0 + 16, blk(i, R2)] for r0 in groups for r in (0, 1, 4)],
                         after)
            for k, r0 in enumerate(groups):
                n = [acc[r][r0:r0 + 16, blk(i, R2)] for r in (2, 3, 5, 6)]
                n = first[3 * k:3 * k + 2] + n[:2] + first[3 * k + 2:3 * k + 3] + n[2:]
                for (d, half), v in zip(((0, 0), (0, 1), (DH, 0), (DH, 1)), _act_join(n)):
                    yield d + r0, half, v

        def out(after):
            for r, half, o in join(acco_v, after):
                c = pair(i)[half]
                ob_v[r:r + 16, c] = (h_v[r:r + 16, c] + o).astype(bf16)

        def stats(after):
            mu = [st_v[2, :, c] for c in pair(i)]
            for r, half, d in join(acch_v, after):
                dn[half][r] = d
                sums[half][0] += d
                sums[half][1] += d * (h_v[r:r + 16, pair(i)[half]] - mu[half])

        def grad(half, after):
            c = pair(i)[half]
            mu, rstd = st_v[2, :, c], st_v[3, :, c]
            m1, m2 = _colmean(sums[half][0]), _colmean(sums[half][1]) * rstd * rstd
            rows = [a * DB + b for b in range(0, DB, 16) for a in range(RD)]
            d = pace([dn[half][r] for r in rows], after)
            h = pace([h_v[r:r + 16, c] for r in rows], after)
            ys = []
            for n in range(0, len(rows), RD):
                dh = [g_v[rows[k]:rows[k] + 16, c].astype(f32)
                      + rstd * (d[k] - m1 - (h[k] - mu) * m2) for k in range(n, n + RD)]
                for r, v in zip(rows[n:n + RD], dh):
                    h_v[r:r + 16, c] = v
                ys.append([v.astype(bf16) for v in _rfft9(dh)])
            y.append([jnp.concatenate(v, axis=0) for v in zip(*ys)])

        def dots(after):
            z = dft_d([jnp.concatenate(v, axis=1) for v in zip(*y)])
            for half, c in enumerate(pair(i)):
                z_v[:, c] = z[:, half * R2:(half + 1) * R2]

        return [out, stats, part(grad, 0), part(grad, 1), dots]

    def window(q):
        r0 = (min if isinstance(q, int) else jnp.minimum)(q * (WIN // 16), (DH - WIN) // 16)
        hint = (lambda v, n: v) if isinstance(q, int) else pl.multiple_of
        return (pl.ds(hint(r0 * 16, 16), WIN), pl.ds(hint(r0 * 16 + DH, 16), WIN),
                pl.ds(hint(r0 * 8, 8), WIN // 2))

    def mod3(j):
        return j % 3 if isinstance(j, int) else lax.rem(j, 3)

    def wprep(j, q, r, after=None):
        src = j if isinstance(j, int) else jnp.minimum(j, nj - 1)
        f1, f2 = blk(2 * src, TF), blk(2 * src + 1, TF)
        d1, d2, dst = window(q)
        for m in range(3):
            ld = lambda d, f: lambda: pace16(w_v[m, d, f], after)
            form = _wgt_forms(ld(d1, f1), ld(d1, f2), ld(d2, f1), ld(d2, f2))[r]
            ws_v[m][r][mod3(j), dst, :] = _pk(form())

    def wprep_rows(j, r0, after=None):
        for m in range(3):
            blocks = pace([_pk(w_v[m, d + r0:d + r0 + 16, blk(2 * j + f, TF)])
                           for d in (0, DH) for f in range(2)], after)
            blocks = [_up(v).astype(f32) for v in blocks]
            for r, form in enumerate(_wgt_forms(*[lambda v=v: v for v in blocks])):
                ws_v[m][r][j, r0 // 2:r0 // 2 + 8, :] = _pk(form())

    def wform(j, m, r, n):
        return _up(ws_v[m][r][mod3(j), 0:n // 2, :])

    def finalize(j, q, m, after=None):
        d1, d2, _ = window(q)
        n = [pace([m_v[m][r][j & 1, d1, :]], after if r < 4 else None)[0] for r in range(7)]
        dw_v[j & 1, m, d1, :TF] = (n[0] + n[3] - n[4] + n[6]).astype(bf16)
        dw_v[j & 1, m, d1, TF:] = (n[2] + n[4]).astype(bf16)
        dw_v[j & 1, m, d2, :TF] = (n[1] + n[3]).astype(bf16)
        dw_v[j & 1, m, d2, TF:] = (n[0] - n[1] + n[2] + n[5]).astype(bf16)

    def stage1(t, b, ms):
        j, ss = t >> 2, blk(t & 3, TS // 2)
        f1, f2 = blk(2 * j, TF), blk(2 * j + 1, TF)
        rows = part(jnp.concatenate, axis=0)
        zero = jnp.zeros((KS - KA, TF), bf16)
        for m in ms:
            k_v, r_v = (gk_v, gr_v) if m == 2 else (hk_v, hr_v)
            v1, v2 = [[w_v[m, KS:DH, f], w_v[m, DH + KS:, f]] for f in (f1, f2)]
            w12, w21 = w_v[m, KA:KS, f2], w_v[m, DH + KA:DH + KS, f1]
            q = lambda r, tail: _dot(_up(k_v[r, ss, :]), rows([wform(j, m, r, KA)] + tail))
            mid = lambda r: [_up(ws_v[m][r][mod3(j), KA // 2:KS // 2, :])]
            q2 = q(2, mid(2))
            yield q2
            q5 = q(5, [w21])
            yield q5
            a7, w7 = _up(k_v[0, ss, R2:]), rows([zero, w12 + w21])
            if m == ms[-1] and len(ms) % 2:
                q7 = rows([_dot(a7[:TS // 2], w7), _dot(a7[TS // 2:], w7)])
            else:
                q7 = _dot(a7, w7)
            raw_v[b][m, 1] = q2 + q5 + q7 + _dot(_up(r_v[0, ss, :]), rows(v2 + mid(1)))
            q3 = q(3, mid(3))
            yield q3
            q6 = q(6, [w12])
            yield q6
            raw_v[b][m, 2] = q3 + q7 + q6 + _dot(_up(r_v[1, ss, :]), rows(v1 + mid(4)))
            q0 = q(0, [zero])
            yield q0
            q1 = q(1, v1)
            raw_v[b][m, 0] = (q0 + q5 - q3) + q1
            yield q1
            q4 = q(4, v2)
            raw_v[b][m, 3] = (q0 - q2 + q6) + q4
            yield q4

    def gate(b, r0, after):
        rows, prows = slice(r0, r0 + EW), slice(r0 // 2, (r0 + EW) // 2)
        res = ([], [], [])
        pre = pace([raw_v[b][0, q, rows] for q in range(4)], after)
        for q in range(4):
            a, u, dp = pre[q], raw_v[b][1, q, rows], raw_v[b][2, q, rows]
            sg = jax.nn.sigmoid(a)
            sl = a * sg
            res[0].append(dp * u * (sg + sl * (1.0 - sg)))
            res[1].append(dp * sl)
            res[2].append(sl * u)
        for m in range(3):
            for r, v in enumerate(_hid_forms(*res[m])):
                p_v[b][m, r, prows, :] = _pk(v)

    gates = lambda b: [part(gate, b, r0) for r0 in range(0, TS, EW)]

    def stage2(t, b, acts=True, wgts=True, which=range(7)):
        j, i = t >> 2, t & 3
        ss = blk(i, TS)
        for r in which:
            if acts:
                o = _dot(wform(j, 2, r, DH), _up(p_v[b][2, r]), NT)
                acco_v[r][:, ss] = jnp.where(j == 0, 0.0, acco_v[r][:, ss]) + o
                yield o
                o = (_dot(wform(j, 0, r, DH), _up(p_v[b][0, r]), NT)
                     + _dot(wform(j, 1, r, DH), _up(p_v[b][1, r]), NT))
                acch_v[r][:, ss] = jnp.where(j == 0, 0.0, acch_v[r][:, ss]) + o
                yield o
            if wgts:
                for m, f_v in enumerate((hf_v, hf_v, gf_v)):
                    o = _dot(_up(f_v[r, :, ss]), _up(p_v[b][m, r]))
                    m_v[m][r][j & 1] = jnp.where(i == 0, 0.0, m_v[m][r][j & 1]) + o
                    yield o

    fins = lambda j, q: [part(finalize, j, q, m) for m in range(3)]
    preps = lambda j, q: [part(wprep, j, q, r) for r in range(7)]
    cat = lambda lists: list(chain(*lists))

    for c in ([x_cp(0), fa_cp] + [x_cp(i) for i in range(1, ntc)] + w_cp + [gm_cp, g_cp]
              + cat(ffn_cp)):
        c.start()
    for a in range(2):
        for k in range(R1):
            wp_v[a, k, pl.ds(RD * 34, KP - K0 - 34, stride=RD), :] = jnp.zeros(
                (KP - K0 - 34, R2), f32)
    fa_cp.wait()

    def p1(i):
        c = blk(i, TC)
        ys, en = [], 0.0
        for b in range(0, DB, 16):
            y = _rfft9([x_v[a * DB + b:a * DB + b + 16, c].astype(f32) for a in range(RD)])
            sq = [v * v for v in y[:8]]
            en = en + 0.75 * sq[5] + (sq[0] + sq[1] + sq[2] + sq[3] + sq[4] + sq[6] + sq[7])
            ys.append([v.astype(bf16) for v in y[:8]] + [y[8]])
        y = [jnp.concatenate(v, axis=0) for v in zip(*ys)]
        mu = _colmean(y[8])
        y[8] = y[8] - RD * mu
        var = (_colmean(y[8] * y[8]) + 2.0 * _colmean(en)) * (1.0 / RD)
        rstd = 1.0 / jnp.sqrt(var + EPS)
        st_v[0, :, c] = mu
        st_v[1, :, c] = rstd
        z_v[:, c] = dft_d(y) * rstd

    def p1s(n):
        for i in range(UN):
            x_cp(UN * n + i).wait()
        for i in range(UN):
            p1(UN * n + i)
    loop("p1", ntc // UN, p1s)
    loop("radix", KP // 16, lambda r: (radix_fwd(2 * r), radix_fwd(2 * r + 1)))
    for m in range(3):
        for r in range(7):
            m_v[m][r][1] = jnp.zeros((DH, TF), f32)

    for c in w_cp:
        c.wait()

    def pw(r):
        for a in range(2):
            put_w(a, blk(r, 32), wb_v[a, blk(r, 32), :])
    loop("pw", (KF - 1) // 32, pw)
    row = lax.broadcasted_iota(jnp.int32, (16, S), 0)
    for a in range(2):
        last = jnp.broadcast_to(wb_v[a, KF - 1:KF, :].astype(f32), (16, S))
        put_w(a, slice(KF - 1, KP), jnp.where(row == 0, last, 0.0))

    gm_cp.wait()
    with jax.named_scope("p3"):
        _overlap(spectrum(mix_fwd),
                 ([lambda after: g_cp.wait()] + cat(grad_forms(i) for i in range(5)), 11, 31))
    loop("radix", KP // 16, lambda r: (radix_inv(2 * r), radix_inv(2 * r + 1)))
    for c in ffn_cp[0]:
        c.wait()
    for r0 in range(0, DH, 16):
        wprep_rows(0, r0)
    for c in ffn_cp[1]:
        c.wait()

    with jax.named_scope("head"):
        w1 = [part(wprep_rows, 1, r0) for r0 in range(0, DH - WIN, 16)]
        _overlap(chain(stage1(0, 0, (2,)), stage1(1, 1, (2,))),
                 (ffn_input(0) + ffn_input(1), 0, 12), (w1[:6], 0, 13))
        _overlap(stage1(0, 0, (0, 1)), (ffn_input(2) + ffn_input(3), 0, 13), (w1[6:], 0, 13))
        _overlap(stage1(1, 1, (0, 1)), (gates(0), 0, 13))

    def step(t, b, *tasks):
        if not tasks:
            tasks = ((fins(((t - 1) >> 2) + 1, (t - 1) & 3), 49, 55),
                     (preps(((t + 1) >> 2) + 1, (t + 1) & 3), 35, 48))
        _overlap(chain(stage2(t - 1, 1 - b), stage1(t + 1, 1 - b, (0, 1, 2))),
                 (gates(b), 1, 32), *tasks)

    with jax.named_scope("head2"):
        in6 = ffn_input(6)
        step(1, 1, (ffn_input(4) + ffn_input(5) + grad_forms(5) + in6[:1], 1, 33),
             (in6[1:] + ffn_input(7) + grad_forms(6) + grad_forms(7),
              34, 54))
    for c in ffn_cp[2]:
        c.wait()

    def body(n):
        j = n >> 1

        @pl.when(((n & 1) == 0) & (j >= 3))
        def _():
            for c in dw_cp(j - 3):
                c.wait()

        @pl.when(((n & 1) == 1) & (j >= 2))
        def _():
            for c in dw_cp(j - 2):
                c.start()
        step(2 * n, 0)
        step(2 * n + 1, 1)
    loop("ffn", nt // 2 - 1, body, 1)
    for c in dw_cp(nj - 3):
        c.start()

    with jax.named_scope("tail"):
        step(nt - 2, 0, (ffn_output(0) + ffn_output(1), 1, 34),
             (ffn_output(2) + ffn_output(3), 35, 54))
        o_cp[0].start()
        o_cp[2].start()
        _overlap(chain(stage2(nt - 2, 0, wgts=False),
                       stage2(nt - 2, 0, acts=False, which=range(4))),
                 (gates(1), 1, 24),
                 (fins(nj - 2, 1) + fins(nj - 2, 2) + fins(nj - 2, 3), 0, 25))
        for c in dw_cp(nj - 2):
            c.start()
        for c in dw_cp(nj - 3):
            c.wait()
        _overlap(chain(stage2(nt - 1, 1, wgts=False),
                       stage2(nt - 2, 0, acts=False, which=range(4, 7)),
                       stage2(nt - 1, 1, acts=False)),
                 (ffn_output(4) + ffn_output(5), 0, 13),
                 (ffn_output(6) + ffn_output(7), 14, 28),
                 ([part(radix_fwd, r) for r in range(KP // 8)], 28, 43))
    for c in (o_cp[1], o_cp[3]):
        c.start()

    with jax.named_scope("p9"):
        _overlap(spectrum(mix_bwd),
                 (cat(fins(nj - 1, q) for q in range(ni))
                  + [lambda after: [c.start() for c in dw_cp(nj - 1)]], 0, 12))

    def pdw(r):
        for a in range(2):
            wb_v[a, blk(r, 32), :] = get_dw(a, blk(r, 32))
            radix_inv(4 * r + 2 * a)
            radix_inv(4 * r + 2 * a + 1)
        for c in dwf_cp(blk(r, 32), r):
            c.start()
    loop("pdw", (KF - 1) // 32, pdw)
    for a in range(2):
        wb_v[a, KF - 1:KF, :] = get_dw(a, slice(KF - 1, KP)).astype(f32)[0:1].astype(bf16)
        radix_inv((KF - 1) // 8 + a)
    dwf_all = [dwf_cp(blk(r, 32), r) for r in range(9)] + [dwf_cp(pl.ds(KF - 1, 1), 9)]
    for c in dwf_all[-1]:
        c.start()

    def p11(i):
        c = blk(i, R2)
        y = idft_d(z_v[:, c], 10)
        mu, rstd = st_v[0, :, c], st_v[1, :, c]
        proj = 0.0
        for b in range(0, DB, 16):
            for a, d in enumerate(_rfft9_t([v[b:b + 16] for v in y])):
                rows = slice(a * DB + b, a * DB + b + 16)
                proj = proj + d * (x_v[rows, c].astype(f32) - mu)
                h_v[rows, c] += rstd * d
        proj = _colmean(proj) * rstd * rstd * rstd
        for r in range(0, D, 16):
            g_v[r:r + 16, c] = (h_v[r:r + 16, c]
                                - (x_v[r:r + 16, c].astype(f32) - mu) * proj).astype(bf16)

    for lo, hi in ((0, 2), (2, 4), (4, 6), (6, 7), (7, 8)):
        with jax.named_scope("p11"):
            for i in range(lo * TC // R2, hi * TC // R2):
                p11(i)
        for i in range(lo, hi):
            dx_cp(i).start()

    for c in (dw_cp(nj - 2) + dw_cp(nj - 1) + o_cp + cat(dwf_all)
              + [dx_cp(i) for i in range(ntc)]):
        c.wait()


@jax.jit
def pallas_sequential_preLN__spectral_gfnet__swiglu_ffn__prompt_kernel(
    A_x: jax.Array,
    A_w_r: jax.Array,
    A_w_i: jax.Array,
    B_x: jax.Array,
    B_w_gate: jax.Array,
    B_w_up: jax.Array,
    B_w_down: jax.Array,
    grad_out: jax.Array,
):
    del B_x
    sds = jax.ShapeDtypeStruct
    hbm = pl.BlockSpec(memory_space=pltpu.HBM)
    out, dx, dwr, dwi, dwg, dwu, dwd = pl.pallas_call(
        _kernel,
        out_shape=[sds((D, S), bf16), sds((D, S), bf16),
                   sds((KF, S), bf16), sds((KF, S), bf16),
                   sds((D, F), bf16), sds((D, F), bf16), sds((D, F), bf16)],
        in_specs=[hbm] * 9,
        out_specs=[hbm] * 7,
        scratch_shapes=[
            V((D, S), bf16), V((D, S), bf16), V((2, KF, S), bf16), V((3, D, F), bf16),
            V((11, R2, R2), bf16), V((R1, 3, R2, R2), bf16),
            V((2 * KP, S), f32), V((R1, KP, 2 * R2), f32),
            V((2, R1, RD * (KP - K0), R2), f32), V((R1, KP // 2, 2 * R2), u32),
            V((4, 1, S), f32), V((D, S), f32),
            V((7, DH // 2, SH), u32), V((7, DH // 2, SH), u32),
            V((7, SH // 2, KS), u32), V((7, SH // 2, KS), u32),
            V((2, SH // 2, R2), u32), V((2, SH // 2, R2), u32),
            [[V((3, DH // 2, TF), u32)] * 7] * 3, [V((3, 4, TS, TF), f32)] * 2,
            [V((3, 7, TS // 2, TF), u32)] * 2,
            [V((DH, SH), f32)] * 7, [V((DH, SH), f32)] * 7, [[V((2, DH, TF), f32)] * 7] * 3,
            V((2, 3, D, 2 * TF), bf16),
            pltpu.SemaphoreType.DMA((S // TC + 16,)),
            pltpu.SemaphoreType.DMA((30 + S // TC,)),
        ],
        compiler_params=pltpu.CompilerParams(vmem_limit_bytes=127 * 2**20),
    )(A_x[0].T, A_w_r.T, A_w_i.T, B_w_gate, B_w_up, B_w_down.T, grad_out[0].T,
      _FA, _G)
    return out.T[None], dx.T[None], dwr.T, dwi.T, dwg, dwu, dwd.T
```
